```python
import jax
import jax.numpy as jnp

def _softmax(x, axis=-1):
    return jax.nn.softmax(x, axis=axis)
def _gelu(x):
    return jax.nn.gelu(x, approximate=True)
def _silu(x):
    return jax.nn.silu(x)
def _sigmoid(x):
    return jax.nn.sigmoid(x)
def _layernorm(x, axis=-1, eps=1e-5):
    m = jnp.mean(x, axis=axis, keepdims=True)
    v = jnp.var(x, axis=axis, keepdims=True)
    return (x - m) / jnp.sqrt(v + eps)
def _scatter_add(tgt, idx, src, axis=0):
    return tgt.at[idx].add(src)
def _segment_sum(src, seg, n):
    return jax.ops.segment_sum(src, seg, n)
class _Rng:
    def __init__(self, key):
        self._k = key
    def _next(self):
        self._k, sub = jax.random.split(self._k)
        return sub
    def normal(self, shape):
        return jax.random.normal(self._next(), shape, dtype=jnp.bfloat16)
    def randint(self, lo, hi, shape):
        return jax.random.randint(self._next(), shape, lo, hi, dtype=jnp.int32)
    def uniform(self, shape, lo=0.0, hi=1.0):
        return jax.random.uniform(self._next(), shape, jnp.bfloat16, lo, hi)
    def permutation(self, n):
        return jax.random.permutation(self._next(), n)


kernel_name = 'parallel_sum__linear_attn_block__moe_arch_mod__prompt'

def setup_inputs():
    _rng = _Rng(jax.random.key(int.from_bytes(__import__("os").urandom(4), "little")))
    _w = (lambda a: (lambda t: t.astype(jnp.bfloat16) if jnp.issubdtype(t.dtype, jnp.floating) else t)(jnp.asarray(a)))
    def _A_setup():
        B, S, D = 1, 2048, 1024
        return {
            "x": _w((lambda *s: _rng.normal(s) * 0.05)(B, S, D)),
            "wqkv": _w((lambda *s: _rng.normal(s) * 0.05)(D, 3 * D)),
            "wo": _w((lambda *s: _rng.normal(s) * 0.05)(D, D)),
        }
    _A_in = _A_setup()

    def _B_setup():
        B, S, D, F, C = 1, 2048, 1024, 3584, 1
        return {
            "x": _w((lambda *s: _rng.normal(s) * 0.05)(B, S, D)),
            "w_r": _w((lambda *s: _rng.normal(s) * 0.05)(D)),
            "w_gate": _w((lambda *s: _rng.normal(s) * 0.05)(D, F)),
            "w_up": _w((lambda *s: _rng.normal(s) * 0.05)(D, F)),
            "w_down": _w((lambda *s: _rng.normal(s) * 0.05)(F, D)),
        }
    _B_in = _B_setup()

    return {
        "A_x": _A_in["x"],
        "A_wqkv": _A_in["wqkv"],
        "A_wo": _A_in["wo"],
        "B_x": _B_in["x"],
        "B_w_r": _B_in["w_r"],
        "B_w_gate": _B_in["w_gate"],
        "B_w_up": _B_in["w_up"],
        "B_w_down": _B_in["w_down"],
    }

def reference(A_x, A_wqkv, A_wo, B_x, B_w_r, B_w_gate, B_w_up, B_w_down):
    def _A_ref(x, wqkv, wo):
        B, S, D = x.shape
        H = 32; Dh = D // H
        qkv = (lambda x, *d: x.transpose(*d))((x @ wqkv).reshape(B, S, 3, H, Dh), 2, 0, 3, 1, 4)
        q, k, v = qkv[0], qkv[1], qkv[2]
        phi = lambda t: jnp.where(t > 0, t + 1, jnp.exp(t)) + 1e-6
        pq, pk = phi(q), phi(k)
        kv = jnp.einsum("bhsd,bhse->bhde", pk, v)
        z = jnp.einsum("bhsd->bhd", pk)
        num = jnp.einsum("bhqd,bhde->bhqe", pq, kv)
        den = jnp.einsum("bhqd,bhd->bhq", pq, z)[..., None] + 1e-6
        o = num / den
        return (lambda x, *d: x.transpose(*d))(o, 0, 2, 1, 3).reshape(B, S, D) @ wo

    def _B_ref(x, w_r, w_gate, w_up, w_down):
        B, S, D = x.shape
        C = 1
        r = x @ w_r
        idx = jnp.argsort(-r, axis=-1)[:, :C]
        idx_e = jnp.repeat(idx.reshape(B, C, 1), D, axis=2)
        x_sel = jnp.take_along_axis(x, idx_e, axis=1)
        g = _silu(x_sel @ w_gate)
        u = x_sel @ w_up
        y = (g * u) @ w_down
        r_sel = _sigmoid(jnp.take_along_axis(r, idx, axis=1))
        y = y * r_sel.reshape(B, C, 1)
        b_off = (jnp.arange(B) * S).reshape(B, 1)
        flat_idx = (idx + b_off).reshape(B * C)
        zero = (x * 0.0).reshape(B * S, D)
        upd = _scatter_add(zero, flat_idx, y.reshape(B * C, D), axis=0)
        return x + upd.reshape(B, S, D)

    x = A_x
    xn = _layernorm(x, axis=-1)
    return x + _A_ref(xn, A_wqkv, A_wo) + _B_ref(xn, B_w_r, B_w_gate, B_w_up, B_w_down)
```

```python
import functools

import jax
import jax.numpy as jnp
from jax import lax
import jax.experimental.pallas as pl
import jax.experimental.pallas.tpu as pltpu

F32 = jnp.float32
BF16 = jnp.bfloat16

S = 2048
D = 1024
F = 3584
DH = 32
TB = 256
NB = S // TB
NP = NB // 2
FC = F // NP
LANES = 128
NG = D // LANES


def _round_bf16(v):
    return v.astype(BF16).astype(F32)


def _phi(t):
    return jnp.where(t > 0, t + 1.0, jnp.exp(t)) + 1e-6


def _dot(a, b):
    return jnp.dot(a, b, preferred_element_type=F32)


def _dot_tn(a, b):
    return lax.dot_general(a, b, (((0,), (0,)), ((), ())), preferred_element_type=F32)


def _dot_nt(a, b):
    return lax.dot_general(a, b, (((1,), (1,)), ((), ())), preferred_element_type=F32)


def _kernel(x_hbm, wqkv_hbm, wo_hbm, wr_hbm, wg_hbm, wu_hbm, wd_hbm, out_hbm,
            x_v, xn_e, xn_o, wq_v, wk_v, wv_v, wo_v, wr_v, wg_v, wu_v, wd_v,
            g_acc, z_acc, m_v, zt_v, r_v, y_acc, out_v,
            sem_x, sem_w, sem_f, sem_o):
    def x_copy(b):
        return pltpu.make_async_copy(x_hbm.at[0, pl.ds(b * TB, TB), :], x_v.at[b], sem_x.at[b])

    wq_copy = pltpu.make_async_copy(wqkv_hbm.at[:, pl.ds(0, D)], wq_v, sem_w.at[0])
    wk_copy = pltpu.make_async_copy(wqkv_hbm.at[:, pl.ds(D, D)], wk_v, sem_w.at[1])
    wv_copy = pltpu.make_async_copy(wqkv_hbm.at[:, pl.ds(2 * D, D)], wv_v, sem_w.at[2])
    wo_copy = pltpu.make_async_copy(wo_hbm, wo_v, sem_w.at[3])
    wr_copy = pltpu.make_async_copy(wr_hbm, wr_v, sem_w.at[4])

    def ffn_copies(c):
        return (
            pltpu.make_async_copy(wg_hbm.at[:, pl.ds(c * FC, FC)], wg_v.at[c], sem_f.at[3 * c]),
            pltpu.make_async_copy(wu_hbm.at[:, pl.ds(c * FC, FC)], wu_v.at[c], sem_f.at[3 * c + 1]),
            pltpu.make_async_copy(wd_hbm.at[pl.ds(c * FC, FC), :], wd_v.at[c], sem_f.at[3 * c + 2]),
        )

    def out_copy(b):
        return pltpu.make_async_copy(out_v.at[b], out_hbm.at[0, pl.ds(b * TB, TB), :], sem_o.at[b])

    wr_copy.start()
    x_copy(0).start()
    wk_copy.start()
    for b in range(1, NB):
        x_copy(b).start()
    wq_copy.start()
    wv_copy.start()
    wo_copy.start()
    for c in range(NP):
        for cp in ffn_copies(c):
            cp.start()

    g_acc[...] = jnp.zeros_like(g_acc)
    z_acc[...] = jnp.zeros_like(z_acc)
    y_acc[...] = jnp.zeros_like(y_acc)

    def layernorm(b, dst_ref, j):
        x = x_v[b].astype(F32)
        mean = jnp.mean(x, axis=-1, keepdims=True)
        c = x - mean
        var = jnp.mean(c * c, axis=-1, keepdims=True)
        std = _round_bf16(jnp.sqrt(_round_bf16(_round_bf16(var) + 1e-5)))
        d = _round_bf16(x - _round_bf16(mean))
        xn = (d * (1.0 / std)).astype(BF16)
        dst_ref[j] = xn
        r = jnp.sum(xn.astype(F32) * wr_v[...].astype(F32), axis=-1, keepdims=True)
        r_v[b] = _round_bf16(r)

    def kg(src_ref, j):
        xn = src_ref[j]
        pk = _phi(_dot(xn, wk_v[...]))
        z_acc[...] += jnp.sum(pk.reshape(TB // 8, 8, D), axis=0)
        g_acc[...] += _dot_tn(pk.astype(BF16), xn)

    wr_copy.wait()
    x_copy(0).wait()
    layernorm(0, xn_e, 0)
    wk_copy.wait()

    def phase_a(j, carry):
        x_copy(2 * j + 1).wait()
        nxt = jnp.minimum(2 * j + 2, NB - 2)

        @pl.when(j < NP - 1)
        def _():
            x_copy(nxt).wait()

        kg(xn_e, j)
        layernorm(2 * j + 1, xn_o, j)
        kg(xn_o, j)
        layernorm(nxt, xn_e, nxt // 2)
        return carry

    lax.fori_loop(0, NP, phase_a, 0)

    wq_copy.wait()
    wv_copy.wait()
    wo_copy.wait()

    rr = lax.broadcasted_iota(jnp.int32, (LANES, LANES), 0) // DH
    cc = lax.broadcasted_iota(jnp.int32, (LANES, LANES), 1) // DH
    same_head = rr == cc
    z_row = jnp.sum(z_acc[...], axis=0, keepdims=True)
    for g in range(NG):
        sl = slice(g * LANES, (g + 1) * LANES)
        kv = _dot(g_acc[sl, :].astype(BF16), wv_v[:, sl])
        kv = jnp.where(same_head, kv, 0.0).astype(BF16)
        m_v[sl, :] = _dot(kv, wo_v[sl, :]).astype(BF16)
        zt_v[g] = jnp.where(same_head, jnp.broadcast_to(z_row[:, sl], (LANES, LANES)), 0.0).astype(BF16)

    r_all = r_v[...].reshape(S, 1)
    r_max = jnp.max(r_all, axis=0, keepdims=True)
    rows = lax.broadcasted_iota(jnp.int32, (S, 1), 0).astype(F32)
    idx_f = jnp.min(jnp.where(r_all == r_max, rows, float(S - 1)))
    idx = jnp.clip(idx_f.astype(jnp.int32), 0, S - 1)
    blk = idx // TB
    row16 = pl.multiple_of(((idx % TB) // 16) * 16, 16)
    gate = _round_bf16(jax.nn.sigmoid(r_max))
    xs_e = xn_e[blk // 2, pl.ds(row16, 16), :]
    xs_o = xn_o[blk // 2, pl.ds(row16, 16), :]
    xs = jnp.where(blk % 2 == 0, xs_e, xs_o)

    def q_part(src_ref, j):
        pq = _phi(_dot(src_ref[j], wq_v[...]))
        pq_b = pq.astype(BF16)
        parts = []
        for g in range(NG):
            sl = slice(g * LANES, (g + 1) * LANES)
            den = _dot_nt(pq_b[:, sl], zt_v[g]) + 1e-6
            parts.append((pq[:, sl] * pl.reciprocal(den, approx=True)).astype(BF16))
        return jnp.concatenate(parts, axis=1)

    def o_part(o, src_ref, j, b):
        a = _dot(o, m_v[...])
        out_v[b] = (x_v[b].astype(F32) + a + src_ref[j].astype(F32)).astype(BF16)

    def phase_b(j, carry):
        for cp in ffn_copies(j):
            cp.wait()
        o_e = q_part(xn_e, j)
        o_o = q_part(xn_o, j)
        gg = _round_bf16(_dot(xs, wg_v[j]))
        uu = _round_bf16(_dot(xs, wu_v[j]))
        h = (_round_bf16(gg * jax.nn.sigmoid(gg)) * uu).astype(BF16)
        o_part(o_e, xn_e, j, 2 * j)
        y_acc[...] += _dot(h, wd_v[j])
        o_part(o_o, xn_o, j, 2 * j + 1)

        @pl.when(2 * j != blk)
        def _():
            out_copy(2 * j).start()

        @pl.when(2 * j + 1 != blk)
        def _():
            out_copy(2 * j + 1).start()
        return carry

    lax.fori_loop(0, NP, phase_b, 0)

    y = _round_bf16(y_acc[...]) * gate
    sel = lax.broadcasted_iota(jnp.int32, (16, D), 0) == idx % 16
    cur = out_v[blk, pl.ds(row16, 16), :].astype(F32)
    out_v[blk, pl.ds(row16, 16), :] = (cur + jnp.where(sel, y, 0.0)).astype(BF16)
    out_copy(blk).start()
    for b in range(NB):
        out_copy(b).wait()


@jax.jit
def pallas_parallel_sum__linear_attn_block__moe_arch_mod__prompt_kernel(
    A_x: jax.Array,
    A_wqkv: jax.Array,
    A_wo: jax.Array,
    B_x: jax.Array,
    B_w_r: jax.Array,
    B_w_gate: jax.Array,
    B_w_up: jax.Array,
    B_w_down: jax.Array,
):
    del B_x
    assert A_x.shape == (1, S, D) and B_w_gate.shape == (D, F)
    any_spec = pl.BlockSpec(memory_space=pl.ANY)
    scratch = [
        pltpu.VMEM((NB, TB, D), BF16),
        pltpu.VMEM((NP, TB, D), BF16),
        pltpu.VMEM((NP, TB, D), BF16),
        pltpu.VMEM((D, D), BF16),
        pltpu.VMEM((D, D), BF16),
        pltpu.VMEM((D, D), BF16),
        pltpu.VMEM((D, D), BF16),
        pltpu.VMEM((1, D), BF16),
        pltpu.VMEM((NP, D, FC), BF16),
        pltpu.VMEM((NP, D, FC), BF16),
        pltpu.VMEM((NP, FC, D), BF16),
        pltpu.VMEM((D, D), F32),
        pltpu.VMEM((8, D), F32),
        pltpu.VMEM((D, D), BF16),
        pltpu.VMEM((NG, LANES, LANES), BF16),
        pltpu.VMEM((NB, TB, 1), F32),
        pltpu.VMEM((16, D), F32),
        pltpu.VMEM((NB, TB, D), BF16),
        pltpu.SemaphoreType.DMA((NB,)),
        pltpu.SemaphoreType.DMA((5,)),
        pltpu.SemaphoreType.DMA((3 * NP,)),
        pltpu.SemaphoreType.DMA((NB,)),
    ]
    return pl.pallas_call(
        _kernel,
        out_shape=jax.ShapeDtypeStruct((1, S, D), BF16),
        in_specs=[any_spec] * 7,
        out_specs=any_spec,
        scratch_shapes=scratch,
        compiler_params=pltpu.CompilerParams(vmem_limit_bytes=100 * 1024 * 1024),
    )(A_x, A_wqkv, A_wo, B_w_r.reshape(1, D), B_w_gate, B_w_up, B_w_down)
```

```python
import jax
import jax.numpy as jnp
from jax import lax
import jax.experimental.pallas as pl
import jax.experimental.pallas.tpu as pltpu

F32 = jnp.float32
BF16 = jnp.bfloat16
U32 = jnp.uint32

S = 2048
D = 1024
F = 3584
DH = 32
TB = 256
NB = S // TB
NP = NB // 2
FC = F // NP
LANES = 128
NG = D // LANES
HG = LANES // DH
KC = 256
NKC = D // KC
WK_SPLITS = (0, 128, 512, 1024)
WQ_PER = 3
DELAY = 8
SEM_A = 5
SEM_F = SEM_A + NP - 1
SEM_O = SEM_F + NP
N_SEMS = SEM_O + 1


def _round_bf16(v):
    return v.astype(BF16).astype(F32)


def _phi(t):
    return jnp.where(t > 0, t + 1.0, jnp.exp(t)) + 1e-6


def _dot(a, b):
    return jnp.dot(a, b, preferred_element_type=F32)


def _dot_tn(a, b):
    return lax.dot_general(a, b, (((0,), (0,)), ((), ())), preferred_element_type=F32)


def _dot_nt(a, b):
    return lax.dot_general(a, b, (((1,), (1,)), ((), ())), preferred_element_type=F32)


def _after(v, dep, other=0.0):
    if dep is None:
        return v
    return jnp.where(dep > jnp.inf, other, v)


def _tie(w, dep, r0=0, c0=0):
    if dep is None:
        return w
    dep = jnp.broadcast_to(dep, (8, LANES))
    head = pltpu.bitcast(w[r0:r0 + 16, c0:c0 + LANES], U32) | (dep > jnp.inf).astype(U32)
    row = [pltpu.bitcast(head, BF16)]
    if c0:
        row = [w[r0:r0 + 16, :c0]] + row
    if c0 + LANES < w.shape[1]:
        row = row + [w[r0:r0 + 16, c0 + LANES:]]
    head = row[0] if len(row) == 1 else jnp.concatenate(row, axis=1)
    parts = ([w[:r0]] if r0 else []) + [head, w[r0 + 16:]]
    return jnp.concatenate(parts, axis=0)


def _ties(w, ties):
    for dep, r0, c0 in ties:
        w = _tie(w, dep, r0, c0)
    return w


def _shuffle_rows(w):
    sub = lax.broadcasted_iota(jnp.int32, (8, w.shape[1]), 0)
    v = [w[(a % 4) * 16 + (a // 4) * 8:(a % 4) * 16 + (a // 4) * 8 + 8] for a in range(8)]
    for d in (4, 2, 1):
        low = (sub & d) == 0
        nv = list(v)
        for a in range(8):
            if a & d == 0:
                nv[a] = jnp.where(low, v[a], pltpu.roll(v[a + d], d, 0))
                nv[a + d] = jnp.where(low, pltpu.roll(v[a], 8 - d, 0), v[a + d])
        v = nv
    return v


def _delay(v, n):
    for _ in range(n):
        v = pl.reciprocal(v, approx=True)
    return v


def _col_bcast(row):
    tiles = [jnp.broadcast_to(row[:, t * LANES:(t + 1) * LANES], (LANES, LANES)).T
             for t in range(row.shape[1] // LANES)]
    return jnp.concatenate(tiles, axis=0)


def _kernel(x_hbm, wqkv_hbm, wo_hbm, wr_hbm, wg_hbm, wu_hbm, wd_hbm, out_hbm,
            x_v, xn_e, xn_o, wq_v, wk_v, wv_v, wo_v, wr_v, wr_f, wg_v, wu_v, wd_v,
            g_acc, z_acc, m_v, wqt_v, zp_v, best_v, junk_v, xcol_v, hcol_v, y_acc, out_v,
            sem):
    def x_copy(b, s_):
        return pltpu.make_async_copy(x_hbm.at[0, pl.ds(b * TB, TB), :], x_v.at[b], sem.at[s_])

    def x0_copy(h):
        rows = pl.ds(h * (TB // 2), TB // 2)
        return pltpu.make_async_copy(x_hbm.at[0, rows, :], x_v.at[0, rows, :], sem.at[h])

    def wk_copy(i):
        lo, hi = WK_SPLITS[i], WK_SPLITS[i + 1]
        return pltpu.make_async_copy(wqkv_hbm.at[:, pl.ds(D + lo, hi - lo)],
                                     wk_v.at[:, pl.ds(lo, hi - lo)], sem.at[2 + i])

    def wq_copy(g, s_):
        return pltpu.make_async_copy(wqkv_hbm.at[:, pl.ds(g * LANES, LANES)], wq_v.at[g], sem.at[s_])

    wr_copy = pltpu.make_async_copy(wr_hbm, wr_v, sem.at[0])
    wv_copy = pltpu.make_async_copy(wqkv_hbm.at[:, pl.ds(2 * D, D)], wv_v, sem.at[SEM_F])
    wo_copy = pltpu.make_async_copy(wo_hbm, wo_v, sem.at[SEM_F])

    def ffn_copies(c, s_):
        return (
            pltpu.make_async_copy(wg_hbm.at[:, pl.ds(c * FC, FC)], wg_v.at[c], sem.at[s_]),
            pltpu.make_async_copy(wu_hbm.at[:, pl.ds(c * FC, FC)], wu_v.at[c], sem.at[s_]),
            pltpu.make_async_copy(wd_hbm.at[pl.ds(c * FC, FC), :], wd_v.at[c], sem.at[s_]),
        )

    def out_copy(b, c):
        cols = pl.ds(c * KC, KC)
        return pltpu.make_async_copy(out_v.at[b, :, cols], out_hbm.at[0, pl.ds(b * TB, TB), cols],
                                     sem.at[SEM_O])

    wr_copy.start()
    x0_copy(0).start()
    x0_copy(1).start()
    for i in range(len(WK_SPLITS) - 1):
        wk_copy(i).start()
    x_copy(1, 4).start()
    for j in range(NP - 1):
        x_copy(2 * j + 2, SEM_A + j).start()
        x_copy(2 * j + 3, SEM_A + j).start()
        for g in range(WQ_PER * j, min(WQ_PER * (j + 1), NG)):
            wq_copy(g, SEM_A + j).start()
    wv_copy.start()
    wo_copy.start()
    for c in range(NP):
        for cp in ffn_copies(c, SEM_F + c):
            cp.start()

    y_acc[...] = jnp.zeros_like(y_acc)
    sub8 = lax.broadcasted_iota(jnp.int32, (8, 1), 0).astype(F32)

    def layernorm(b, dst_ref, j, r0, nr, best, dep=None, dep2=None):
        rs = pl.ds(r0, nr)
        mean = jnp.mean(x_v[b, rs, :].astype(F32), axis=-1, keepdims=True)
        mean_b = _after(_round_bf16(mean), dep)
        junk_v[...] = mean[:8]
        c = x_v[b, rs, :].astype(F32) - mean
        var = jnp.mean(c * c, axis=-1, keepdims=True)
        junk_v[...] = var[:8]
        std = _round_bf16(jnp.sqrt(_round_bf16(_round_bf16(var) + 1e-5)))
        d = _round_bf16(x_v[b, rs, :].astype(F32) - mean_b)
        xn = (d * (1.0 / std)).astype(BF16)
        dst_ref[j, rs, :] = xn
        wr = wr_f[...]
        if dep2 is not None:
            wr = jnp.concatenate([_after(wr[:, :LANES], dep2), wr[:, LANES:]], axis=1)
        if nr > 8:
            wr = jnp.concatenate([wr] * (nr // 8), axis=0)
        r = jnp.sum(xn.astype(F32) * wr, axis=-1, keepdims=True)
        rb = _round_bf16(r)
        bv, bi = best
        for q in range(nr // 8):
            rq = rb[q * 8:(q + 1) * 8]
            better = rq > bv
            bv = jnp.where(better, rq, bv)
            bi = jnp.where(better, sub8 + jnp.asarray(b * TB + r0 + q * 8).astype(F32), bi)
        return r, (bv, bi)

    def load_best():
        return best_v[0], best_v[1]

    def store_best(best):
        best_v[0] = best[0]
        best_v[1] = best[1]

    def k_unit(src_ref, j, lo, hi, first=False, ties=()):
        pk = _phi(_dot(src_ref[j], _ties(wk_v[:, lo:hi], ties)))
        zs = jnp.sum(pk.reshape(TB // 8, 8, hi - lo), axis=0)
        if first:
            z_acc[:, lo:hi] = zs
        else:
            z_acc[:, lo:hi] += zs
        return pk.astype(BF16)

    def g_unit(src_ref, j, lo, hi, pk, first=False, ties=()):
        g = _dot_tn(pk, _ties(src_ref[j], ties))
        if first:
            g_acc[lo:hi, :] = g
        else:
            g_acc[lo:hi, :] += g

    def wq_prep(g, kk):
        v = _shuffle_rows(pltpu.bitcast(wq_v[g, kk * 256:(kk + 1) * 256, :].T, U32))
        base = pl.multiple_of(g * 8, 8)
        tot = None
        for i in range(8):
            wqt_v[pl.ds(i * 64 + base, 8), kk * 256:(kk + 1) * 256] = v[i]
            tot = v[i] if tot is None else tot | v[i]
        return pltpu.bitcast(tot[:, :LANES] | tot[:, LANES:], F32)

    def mv_chain(acc, w_ref, c, n0, col_ref, z0):
        def step(i, acc):
            rows = pl.ds(pl.multiple_of(i * 8, 8), 8)
            return acc + w_ref[c, rows, n0:n0 + LANES].astype(F32) * col_ref[z0, rows, :]
        return lax.fori_loop(0, w_ref.shape[1] // 8, step, acc, unroll=True)

    def ffn_gate_up(c, z0):
        dep = None
        zero = jnp.zeros((8, LANES), F32)
        for n0 in range(0, FC, LANES):
            ga = mv_chain(_after(zero, dep, 1.0), wg_v, c, n0, xcol_v, z0)
            ua = mv_chain(_after(zero, ga, 1.0), wu_v, c, n0, xcol_v, z0)
            dep = ua
            gg = _round_bf16(jnp.sum(ga, axis=0, keepdims=True))
            uu = _round_bf16(jnp.sum(ua, axis=0, keepdims=True))
            h = _round_bf16(_round_bf16(gg * jax.nn.sigmoid(gg)) * uu)
            hcol_v[0, n0:n0 + LANES, :] = _col_bcast(h)
        return dep

    def ffn_down(c, slot, z0):
        dep = None
        for n0 in range(0, D, LANES):
            dep = mv_chain(_after(y_acc[slot, :, n0:n0 + LANES], dep), wd_v, c, n0, hcol_v, z0)
            y_acc[slot, :, n0:n0 + LANES] = dep
        return dep

    wr_copy.wait()
    x0_copy(0).wait()
    wr_f[...] = jnp.broadcast_to(wr_v[...].astype(F32).reshape(1, D), (8, D))
    best = (jnp.full((8, 1), -jnp.inf, F32), sub8)
    _, best = layernorm(0, xn_e, 0, 0, TB // 2, best)
    x0_copy(1).wait()
    _, best = layernorm(0, xn_e, 0, TB // 2, TB // 2, best)

    wk_copy(0).wait()
    g_unit(xn_e, 0, 0, 128, k_unit(xn_e, 0, 0, 128, True), True)
    wk_copy(1).wait()
    pks = [k_unit(xn_e, 0, lo, lo + 128, True) for lo in (128, 256, 384)]
    for lo, pk in zip((128, 256, 384), pks):
        g_unit(xn_e, 0, lo, lo + 128, pk, True)
    wk_copy(2).wait()
    x_copy(1, 4).wait()
    dep = None
    for r0 in range(0, TB, 16):
        dep, best = layernorm(1, xn_o, 0, r0, 16, best, dep)
    store_best(best)
    pks = [k_unit(xn_e, 0, lo, lo + KC, True) for lo in (512, 768)]
    g_unit(xn_e, 0, 512, 768, pks[0], True)
    g_unit(xn_e, 0, 768, 896, pks[1][:, :128], True)
    g_unit(xn_e, 0, 896, 1024, pks[1][:, 128:], True, [(dep[:8], 0, 0)])

    def phase_a(j, carry):
        x_copy(0, SEM_A + j).wait()
        x_copy(0, SEM_A + j).wait()
        wq_copy(0, SEM_A + j).wait()
        wq_copy(0, SEM_A + j).wait()

        @pl.when(WQ_PER * j + 2 < NG)
        def _():
            wq_copy(0, SEM_A + j).wait()

        preps = [(jnp.minimum(WQ_PER * j + i, NG - 1), kk) for i in range(WQ_PER) for kk in range(4)]
        k_slots = {(0, 0): [(0, 128), (512, 128)], (0, 1): [(0, 0), (512, 0), (0, 128), (512, 128)],
                   (1, 1): [(0, 0), (512, 0), (0, 128)]}
        g_slots = {(0, 3): [(0, 256), (0, 512), (0, 768)]}

        def mk_ties(slots):
            return [(wq_prep(*preps.pop(0)), r0, c0) for r0, c0 in slots]

        LR = TB // NKC
        prev = None
        dep = None
        best = load_best()
        for half in range(2):
            src, js = (xn_o, j) if half == 0 else (xn_e, j + 1)
            dst, b = (xn_e, 2 * j + 2) if half == 0 else (xn_o, 2 * j + 3)
            for c in range(NKC):
                pk = k_unit(src, js, c * KC, (c + 1) * KC, ties=mk_ties(k_slots.get((half, c), [])))
                if prev is not None:
                    g_unit(*prev[1:], ties=mk_ties(g_slots.get(prev[0], [])))
                prev = ((half, c), src, js, c * KC, (c + 1) * KC, pk)
                for r0 in range(c * LR, (c + 1) * LR, 8):
                    dep, best = layernorm(b, dst, j + 1, r0, 8, best, dep)
        g_unit(*prev[1:])
        assert not preps
        store_best(best)
        return carry

    lax.fori_loop(0, NP - 1, phase_a, 0)

    wv_copy.wait()
    wo_copy.wait()
    for cp in ffn_copies(0, SEM_F):
        cp.wait()

    bv, bi = load_best()
    r_max = jnp.max(bv, axis=0, keepdims=True)
    idx_f = jnp.min(jnp.where(bv == r_max, bi, float(S - 1)))
    idx = jnp.clip(idx_f.astype(jnp.int32), 0, S - 1)
    blk = idx // TB
    last_pair = blk // 2
    row16 = pl.multiple_of(((idx % TB) // 16) * 16, 16)
    gate = _round_bf16(jax.nn.sigmoid(r_max))
    sel16 = lax.broadcasted_iota(jnp.int32, (16, D), 0) == idx % 16
    xs = jnp.where(blk % 2 == 0, xn_e[last_pair, pl.ds(row16, 16), :].astype(F32),
                   xn_o[last_pair, pl.ds(row16, 16), :].astype(F32))
    z0 = idx // S
    xcol_v[0] = _col_bcast(jnp.sum(jnp.where(sel16, xs, 0.0), axis=0, keepdims=True))
    gu_dep = ffn_gate_up(0, z0)
    dn_dep = ffn_down(0, 0, z0)

    rr = lax.broadcasted_iota(jnp.int32, (LANES, LANES), 0) // DH
    cc = lax.broadcasted_iota(jnp.int32, (LANES, LANES), 1) // DH
    same_head = rr == cc

    def g_final(c, pk, dep=None):
        return (g_acc[c * KC:(c + 1) * KC, :] + _dot_tn(pk, _tie(xn_o[NP - 1], dep))).astype(BF16)

    def kv_unit(c, gf):
        out = []
        for gg in range(KC // LANES):
            g = c * (KC // LANES) + gg
            kv = _dot(gf[gg * LANES:(gg + 1) * LANES, :], wv_v[:, g * LANES:(g + 1) * LANES])
            kv = pltpu.bitcast(jnp.where(same_head, kv, 0.0).astype(BF16), U32)
            out.append(pltpu.bitcast(jnp.concatenate(_shuffle_rows(kv), axis=0), BF16))
        return out

    def m_unit(c, kvs, dep=None):
        for gg in range(KC // LANES):
            g = c * (KC // LANES) + gg
            m = _dot(kvs[gg], _tie(wo_v[g * LANES:(g + 1) * LANES, :], dep))
            dep = None
            w = pltpu.bitcast(m.astype(BF16), U32)
            for i in range(8):
                m_v[i * 64 + g * 8:i * 64 + (g + 1) * 8, :] = w[i * 8:(i + 1) * 8, :]

    def z_prep():
        zc = pltpu.bitcast(_col_bcast(jnp.sum(z_acc[...], axis=0, keepdims=True)).astype(BF16), U32)
        vs = [_shuffle_rows(zc[g * 64:(g + 1) * 64, :]) for g in range(NG)]
        tot = None
        for i in range(NG):
            zt = pltpu.bitcast(jnp.concatenate([vs[g][i] for g in range(NG)], axis=0), BF16)
            zp = zt.astype(F32).T[:8, :]
            zp_v[:, i * LANES:(i + 1) * LANES] = zp
            tot = zp if tot is None else tot + zp
        return tot

    def ku(c):
        return k_unit(xn_o, NP - 1, c * KC, (c + 1) * KC)

    pk0 = ku(0)
    pk1 = ku(1)
    gf0 = g_final(0, pk0)
    pk2 = ku(2)
    gf1 = g_final(1, pk1)
    kv0 = kv_unit(0, gf0)
    pk3 = ku(3)
    gf2 = g_final(2, pk2)
    kv1 = kv_unit(1, gf1)
    m_unit(0, kv0, gu_dep)
    gf3 = g_final(3, pk3)
    kv2 = kv_unit(2, gf2)
    m_unit(1, kv1)
    kv3 = kv_unit(3, gf3)
    m_unit(2, kv2, z_prep())
    m_unit(3, kv3, dn_dep)

    lane = lax.broadcasted_iota(jnp.int32, (8, LANES), 1)
    bit0 = lane % 2 == 0
    bit3 = (lane // 8) % 2 == 0

    def q_part(src_ref, p, wdep=None):
        q = _dot_nt(src_ref[p], _tie(pltpu.bitcast(wqt_v[...], BF16), wdep, 2 * LANES))
        rows_ = []
        dep = None
        for g in range(TB // 8):
            pq = _phi(q[g * 8:(g + 1) * 8, :])
            t = pq * zp_v[...]
            s_ = t[:, :LANES]
            for n in range(1, NG):
                s_ = s_ + t[:, n * LANES:(n + 1) * LANES]
            s_ = s_ + jnp.where(bit3, pltpu.roll(s_, LANES - 8, 1), pltpu.roll(s_, 8, 1))
            s_ = s_ + jnp.where(bit0, pltpu.roll(s_, LANES - 1, 1), pltpu.roll(s_, 1, 1))
            rinv = _after(pl.reciprocal(s_ + 1e-6, approx=True), dep)
            rows_.append(pq * jnp.concatenate([rinv] * NG, axis=1))
            dep = _delay(rinv, DELAY)
        return jnp.concatenate(rows_, axis=0).astype(BF16)

    def o_part(o, src_ref, p, b, dep=None):
        for c in range(NKC):
            cs = slice(c * KC, (c + 1) * KC)
            m = pltpu.bitcast(m_v[:, cs], BF16)
            a = _dot(o, _tie(m, dep if c == NKC - 1 else None))
            out_v[b, :, cs] = (x_v[b, :, cs].astype(F32) + a + src_ref[p, :, cs].astype(F32)).astype(BF16)
            out_copy(b, c).start()

    def phase_b(j, carry):
        @pl.when(j < NP - 1)
        def _():
            for cp in ffn_copies(0, SEM_F + j + 1):
                cp.wait()

        @pl.when(j == NP - 1)
        def _():
            y = _round_bf16(jnp.sum(y_acc[0], axis=0, keepdims=True)) * gate
            cur = x_v[blk, pl.ds(row16, 16), :].astype(F32)
            x_v[blk, pl.ds(row16, 16), :] = (cur + jnp.where(sel16, y, 0.0)).astype(BF16)

        p = jnp.where(j == NP - 1, last_pair, jnp.where(j == last_pair, NP - 1, j))
        cj = jnp.minimum(j + 1, NP - 1)
        gu_dep = ffn_gate_up(cj, 0)
        dep = ffn_down(cj, (j == NP - 1).astype(jnp.int32), z0)
        o_e = q_part(xn_e, p)
        o_o = q_part(xn_o, p, gu_dep)
        o_part(o_e, xn_e, p, 2 * p)
        o_part(o_o, xn_o, p, 2 * p + 1, dep)
        return carry

    lax.fori_loop(0, NP, phase_b, 0)

    pltpu.make_async_copy(out_v, out_v, sem.at[SEM_O]).wait()


@jax.jit
def pallas_parallel_sum__linear_attn_block__moe_arch_mod__prompt_kernel(
    A_x: jax.Array,
    A_wqkv: jax.Array,
    A_wo: jax.Array,
    B_x: jax.Array,
    B_w_r: jax.Array,
    B_w_gate: jax.Array,
    B_w_up: jax.Array,
    B_w_down: jax.Array,
):
    del B_x
    assert A_x.shape == (1, S, D) and B_w_gate.shape == (D, F)
    any_spec = pl.BlockSpec(memory_space=pl.ANY)
    scratch = [
        pltpu.VMEM((NB, TB, D), BF16),
        pltpu.VMEM((NP, TB, D), BF16),
        pltpu.VMEM((NP, TB, D), BF16),
        pltpu.VMEM((NG, D, LANES), BF16),
        pltpu.VMEM((D, D), BF16),
        pltpu.VMEM((D, D), BF16),
        pltpu.VMEM((D, D), BF16),
        pltpu.VMEM((D,), BF16),
        pltpu.VMEM((8, D), F32),
        pltpu.VMEM((NP, D, FC), BF16),
        pltpu.VMEM((NP, D, FC), BF16),
        pltpu.VMEM((NP, FC, D), BF16),
        pltpu.VMEM((D, D), F32),
        pltpu.VMEM((8, D), F32),
        pltpu.VMEM((D // 2, D), U32),
        pltpu.VMEM((D // 2, D), U32),
        pltpu.VMEM((8, D), F32),
        pltpu.VMEM((2, 8, 1), F32),
        pltpu.VMEM((8, 1), F32),
        pltpu.VMEM((2, D, LANES), F32),
        pltpu.VMEM((2, FC, LANES), F32),
        pltpu.VMEM((2, 8, D), F32),
        pltpu.VMEM((NB, TB, D), BF16),
        pltpu.SemaphoreType.DMA((N_SEMS,)),
    ]
    return pl.pallas_call(
        _kernel,
        out_shape=jax.ShapeDtypeStruct((1, S, D), BF16),
        in_specs=[any_spec] * 7,
        out_specs=any_spec,
        scratch_shapes=scratch,
        compiler_params=pltpu.CompilerParams(vmem_limit_bytes=100 * 1024 * 1024),
    )(A_x, A_wqkv, A_wo, B_w_r, B_w_gate, B_w_up, B_w_down)
```

```python
import jax
import jax.numpy as jnp
from jax import lax
import jax.experimental.pallas as pl
import jax.experimental.pallas.tpu as pltpu

F32 = jnp.float32
BF16 = jnp.bfloat16
U32 = jnp.uint32

S = 2048
D = 1024
F = 3584
DH = 32
TB = 256
NB = S // TB
NP = NB // 2
FC = F // NP
LANES = 128
NG = D // LANES
HG = LANES // DH
KC = 256
NKC = D // KC
WK_SPLITS = (0, 128, 512, 1024)
WQ_PER = 3
DELAY = 8
GU_TILE = 2
SEM_A = 5
SEM_W = SEM_A + NP - 1
SEM_F = SEM_W + 1
SEM_O = SEM_F + NP
N_SEMS = SEM_O + 2


def _round_bf16(v):
    return v.astype(BF16).astype(F32)


def _phi(t):
    return jnp.where(t > 0, t + 1.0, jnp.exp(t)) + 1e-6


def _dot(a, b):
    return jnp.dot(a, b, preferred_element_type=F32)


def _dot_tn(a, b):
    return lax.dot_general(a, b, (((0,), (0,)), ((), ())), preferred_element_type=F32)


def _dot_nt(a, b):
    return lax.dot_general(a, b, (((1,), (1,)), ((), ())), preferred_element_type=F32)


def _after(v, dep, other=0.0):
    if dep is None:
        return v
    return jnp.where(dep > jnp.inf, other, v)


def _tie(w, dep, r0=0, c0=0):
    if dep is None:
        return w
    dep = jnp.broadcast_to(dep, (8, LANES))
    head = pltpu.bitcast(w[r0:r0 + 16, c0:c0 + LANES], U32) | (dep > jnp.inf).astype(U32)
    row = [pltpu.bitcast(head, BF16)]
    if c0:
        row = [w[r0:r0 + 16, :c0]] + row
    if c0 + LANES < w.shape[1]:
        row = row + [w[r0:r0 + 16, c0 + LANES:]]
    head = row[0] if len(row) == 1 else jnp.concatenate(row, axis=1)
    parts = ([w[:r0]] if r0 else []) + [head, w[r0 + 16:]]
    return jnp.concatenate(parts, axis=0)


def _ties(w, ties):
    for dep, r0, c0 in ties:
        w = _tie(w, dep, r0, c0)
    return w


def _shuffle_rows(w):
    sub = lax.broadcasted_iota(jnp.int32, (8, w.shape[1]), 0)
    v = [w[(a % 4) * 16 + (a // 4) * 8:(a % 4) * 16 + (a // 4) * 8 + 8] for a in range(8)]
    for d in (4, 2, 1):
        low = (sub & d) == 0
        nv = list(v)
        for a in range(8):
            if a & d == 0:
                nv[a] = jnp.where(low, v[a], pltpu.roll(v[a + d], d, 0))
                nv[a + d] = jnp.where(low, pltpu.roll(v[a], 8 - d, 0), v[a + d])
        v = nv
    return v


def _delay(v, n):
    for _ in range(n):
        v = pl.reciprocal(v, approx=True)
    return v


def _col_bcast(row):
    tiles = [jnp.broadcast_to(row[:, t * LANES:(t + 1) * LANES], (LANES, LANES)).T
             for t in range(row.shape[1] // LANES)]
    return jnp.concatenate(tiles, axis=0)


def _kernel(x_hbm, wqkv_hbm, wo_hbm, wr_hbm, wg_hbm, wu_hbm, wd_hbm, out_hbm,
            x_v, xn_e, xn_o, wq_v, wk_v, wv_v, wo_v, wg_v, wu_v, wd_v, xcol_v, hcol_v,
            g_acc, m_v, wqt_v, out_v, wr_f, z_acc, zp_v, y_acc, gate_v, best_v, junk_v, wr_v,
            sem):
    def x_copy(b, s_):
        return pltpu.make_async_copy(x_hbm.at[0, pl.ds(b * TB, TB), :], x_v.at[b], sem.at[s_])

    def x0_copy(h):
        rows = pl.ds(h * (TB // 2), TB // 2)
        return pltpu.make_async_copy(x_hbm.at[0, rows, :], x_v.at[0, rows, :], sem.at[h])

    def wk_copy(i):
        lo, hi = WK_SPLITS[i], WK_SPLITS[i + 1]
        return pltpu.make_async_copy(wqkv_hbm.at[:, pl.ds(D + lo, hi - lo)],
                                     wk_v.at[:, pl.ds(lo, hi - lo)], sem.at[2 + i])

    def wq_copy(g, s_):
        return pltpu.make_async_copy(wqkv_hbm.at[:, pl.ds(g * LANES, LANES)], wq_v.at[g], sem.at[s_])

    wr_copy = pltpu.make_async_copy(wr_hbm, wr_v, sem.at[0])
    wv_copy = pltpu.make_async_copy(wqkv_hbm.at[:, pl.ds(2 * D, D)], wv_v, sem.at[SEM_W])
    wo_copy = pltpu.make_async_copy(wo_hbm, wo_v, sem.at[SEM_W])

    def ffn_copies(c, s_):
        return (
            pltpu.make_async_copy(wg_hbm.at[:, pl.ds(c * FC, FC)], wg_v.at[c, :, pl.ds(0, FC)], sem.at[s_]),
            pltpu.make_async_copy(wu_hbm.at[:, pl.ds(c * FC, FC)], wu_v.at[c, :, pl.ds(0, FC)], sem.at[s_]),
            pltpu.make_async_copy(wd_hbm.at[pl.ds(c * FC, FC), :], wd_v.at[c, pl.ds(0, FC), :], sem.at[s_]),
        )

    wr_copy.start()
    x0_copy(0).start()
    x0_copy(1).start()
    for i in range(len(WK_SPLITS) - 1):
        wk_copy(i).start()
    x_copy(1, 4).start()
    for j in range(NP - 1):
        x_copy(2 * j + 2, SEM_A + j).start()
        x_copy(2 * j + 3, SEM_A + j).start()
        for g in range(WQ_PER * j, min(WQ_PER * (j + 1), NG)):
            wq_copy(g, SEM_A + j).start()
    wv_copy.start()
    wo_copy.start()
    for c in range(NP):
        for cp in ffn_copies(c, SEM_F + c):
            cp.start()

    y_acc[...] = jnp.zeros_like(y_acc)
    sub8 = lax.broadcasted_iota(jnp.int32, (8, 1), 0).astype(F32)

    def normalise(b, dst_ref, j, r0, nr, dep=None):
        rs = pl.ds(r0, nr)
        mean = jnp.mean(x_v[b, rs, :].astype(F32), axis=-1, keepdims=True)
        mean_b = _after(_round_bf16(mean), dep)
        junk_v[...] = mean[:8]
        c = x_v[b, rs, :].astype(F32) - mean
        var = jnp.mean(c * c, axis=-1, keepdims=True)
        junk_v[...] = var[:8]
        std = _round_bf16(jnp.sqrt(_round_bf16(_round_bf16(var) + 1e-5)))
        d = _round_bf16(x_v[b, rs, :].astype(F32) - mean_b)
        xn = (d * (1.0 / std)).astype(BF16)
        dst_ref[j, rs, :] = xn
        return xn

    def score(xn, row0, best, dep=None):
        nr = xn.shape[0]
        wr = wr_f[...]
        if dep is not None:
            wr = jnp.concatenate([_after(wr[:, :LANES], dep[:8]), wr[:, LANES:]], axis=1)
        if nr > 8:
            wr = jnp.concatenate([wr] * (nr // 8), axis=0)
        r = jnp.sum(xn.astype(F32) * wr, axis=-1, keepdims=True)
        rb = _round_bf16(r)
        bv, bi = best
        for q in range(nr // 8):
            rq = rb[q * 8:(q + 1) * 8]
            better = rq > bv
            bv = jnp.where(better, rq, bv)
            bi = jnp.where(better, sub8 + jnp.asarray(row0 + q * 8).astype(F32), bi)
        return r, (bv, bi)

    def layernorm(b, dst_ref, j, r0, nr, best, dep=None):
        return score(normalise(b, dst_ref, j, r0, nr, dep), b * TB + r0, best)

    def load_best():
        return best_v[0], best_v[1]

    def store_best(best):
        best_v[0] = best[0]
        best_v[1] = best[1]

    def k_unit(src_ref, j, lo, hi, first=False, ties=()):
        pk = _phi(_dot(src_ref[j], _ties(wk_v[:, lo:hi], ties)))
        zs = jnp.sum(pk.reshape(TB // 8, 8, hi - lo), axis=0)
        if first:
            z_acc[:, lo:hi] = zs
        else:
            z_acc[:, lo:hi] += zs
        return pk.astype(BF16)

    def g_unit(src_ref, j, lo, hi, pk, first=False, ties=()):
        g = _dot_tn(pk, _ties(src_ref[j], ties))
        if first:
            g_acc[lo:hi, :] = g
        else:
            g_acc[lo:hi, :] += g

    def wq_prep(g, kk):
        v = _shuffle_rows(pltpu.bitcast(wq_v[g, kk * 256:(kk + 1) * 256, :].T, U32))
        base = pl.multiple_of(g * 8, 8)
        tot = None
        for i in range(8):
            wqt_v[pl.ds(i * 64 + base, 8), kk * 256:(kk + 1) * 256] = v[i]
            tot = v[i] if tot is None else tot | v[i]
        return pltpu.bitcast(tot[:, :LANES] | tot[:, LANES:], F32)

    def mv_chain(acc, w_ref, c, n0, col_ref, z0, k=D):
        cp = 2 * LANES if (n0 // 256) % 4 < 2 else 0
        cz = c + z0

        def step(i, acc):
            rows = pl.ds(pl.multiple_of(i * 8, 8), 8)
            return acc + w_ref[cz, rows, n0:n0 + LANES].astype(F32) * col_ref[z0, rows, cp:cp + LANES]
        return lax.fori_loop(0, k // 8, step, acc, unroll=True)

    def ffn_gate_up(c, zeros):
        dep = None
        zero = jnp.zeros((8, LANES), F32)
        for n0 in range(0, FC, LANES):
            ga = mv_chain(_after(zero, dep, 1.0), wg_v, c, n0, xcol_v, next(zeros))
            ua = mv_chain(_after(zero, ga, 1.0), wu_v, c, n0, xcol_v, next(zeros))
            dep = ua
            gg = _round_bf16(jnp.sum(ga, axis=0, keepdims=True))
            uu = _round_bf16(jnp.sum(ua, axis=0, keepdims=True))
            h = _round_bf16(_round_bf16(gg * jax.nn.sigmoid(gg)) * uu)
            hc = _col_bcast(h)
            hcol_v[0, n0:n0 + LANES, :LANES] = hc
            hcol_v[0, n0:n0 + LANES, 2 * LANES:3 * LANES] = hc
        return dep

    def ffn_down(c, zeros):
        dep = None
        accs = []
        for n0 in range(0, D, LANES):
            dep = mv_chain(_after(y_acc[:, n0:n0 + LANES], dep), wd_v, c, n0, hcol_v, next(zeros), FC)
            y_acc[:, n0:n0 + LANES] = dep
            accs.append(dep)
        return jnp.concatenate(accs, axis=1)

    wr_copy.wait()
    x0_copy(0).wait()
    normalise(0, xn_e, 0, 0, TB // 2)
    x0_copy(1).wait()
    normalise(0, xn_e, 0, TB // 2, TB // 2)

    wk_copy(0).wait()
    wr_f[...] = jnp.broadcast_to(wr_v[...].astype(F32).reshape(1, D), (8, D))
    g_unit(xn_e, 0, 0, 128, k_unit(xn_e, 0, 0, 128, True), True)
    wk_copy(1).wait()
    best = (jnp.full((8, 1), -jnp.inf, F32), sub8)
    dep = None
    for r0 in range(0, TB, 16):
        dep, best = score(xn_e[0, r0:r0 + 16, :], r0, best, dep)
    pks = [k_unit(xn_e, 0, lo, lo + 128, True) for lo in (128, 256, 384)]
    for lo, pk in zip((128, 256, 384), pks):
        g_unit(xn_e, 0, lo, lo + 128, pk, True)
    wk_copy(2).wait()
    x_copy(1, 4).wait()
    dep = None
    for r0 in range(0, TB, 16):
        dep, best = layernorm(1, xn_o, 0, r0, 16, best, dep)
    store_best(best)
    pks = [k_unit(xn_e, 0, lo, lo + KC, True) for lo in (512, 768)]
    g_unit(xn_e, 0, 512, 768, pks[0], True)
    g_unit(xn_e, 0, 768, 896, pks[1][:, :128], True)
    g_unit(xn_e, 0, 896, 1024, pks[1][:, 128:], True, [(dep[:8], 0, 0)])

    def phase_a(j, carry):
        x_copy(0, SEM_A + j).wait()
        x_copy(0, SEM_A + j).wait()
        wq_copy(0, SEM_A + j).wait()
        wq_copy(0, SEM_A + j).wait()

        @pl.when(WQ_PER * j + 2 < NG)
        def _():
            wq_copy(0, SEM_A + j).wait()

        preps = [(jnp.minimum(WQ_PER * j + i, NG - 1), kk) for i in range(WQ_PER) for kk in range(4)]
        k_slots = {(0, 0): [(0, 128), (512, 128)], (0, 1): [(0, 0), (512, 0), (0, 128), (512, 128)],
                   (1, 1): [(0, 0), (512, 0), (0, 128)]}
        g_slots = {(0, 3): [(0, 256), (0, 512), (0, 768)]}

        def mk_ties(slots):
            return [(wq_prep(*preps.pop(0)), r0, c0) for r0, c0 in slots]

        LR = TB // NKC
        prev = None
        dep = None
        best = load_best()
        for half in range(2):
            src, js = (xn_o, j) if half == 0 else (xn_e, j + 1)
            dst, b = (xn_e, 2 * j + 2) if half == 0 else (xn_o, 2 * j + 3)
            for c in range(NKC):
                pk = k_unit(src, js, c * KC, (c + 1) * KC, ties=mk_ties(k_slots.get((half, c), [])))
                if prev is not None:
                    g_unit(*prev[1:], ties=mk_ties(g_slots.get(prev[0], [])))
                prev = ((half, c), src, js, c * KC, (c + 1) * KC, pk)
                for r0 in range(c * LR, (c + 1) * LR, 8):
                    dep, best = layernorm(b, dst, j + 1, r0, 8, best, dep)
        g_unit(*prev[1:])
        assert not preps
        store_best(best)
        return carry

    lax.fori_loop(0, NP - 1, phase_a, 0)

    wv_copy.wait()
    wo_copy.wait()

    bv, bi = load_best()
    r_max = jnp.max(bv, axis=0, keepdims=True)
    idx_f = jnp.min(jnp.where(bv == r_max, bi, float(S - 1)))
    idx = jnp.clip(idx_f.astype(jnp.int32), 0, S - 1)
    blk = idx // TB
    hot_pair = blk // 2
    row16 = pl.multiple_of(((idx % TB) // 16) * 16, 16)
    gate_v[...] = jnp.broadcast_to(_round_bf16(jax.nn.sigmoid(r_max)), (16, LANES))
    row_id16 = lax.broadcasted_iota(jnp.int32, (16, D), 0)
    sel16 = row_id16 == idx % 16
    xs = jnp.where(blk % 2 == 0, xn_e[hot_pair, pl.ds(row16, 16), :].astype(F32),
                   xn_o[hot_pair, pl.ds(row16, 16), :].astype(F32))
    xc = _col_bcast(jnp.sum(jnp.where(sel16, xs, 0.0), axis=0, keepdims=True))
    xcol_v[0, :, :LANES] = xc
    xcol_v[0, :, 2 * LANES:3 * LANES] = xc

    rr = lax.broadcasted_iota(jnp.int32, (LANES, LANES), 0) // DH
    cc = lax.broadcasted_iota(jnp.int32, (LANES, LANES), 1) // DH
    same_head = rr == cc

    def g_final(c, pk, dep=None):
        return (g_acc[c * KC:(c + 1) * KC, :] + _dot_tn(pk, _tie(xn_o[NP - 1], dep))).astype(BF16)

    def kv_unit(c, gf):
        out = []
        for gg in range(KC // LANES):
            g = c * (KC // LANES) + gg
            kv = _dot(gf[gg * LANES:(gg + 1) * LANES, :], wv_v[:, g * LANES:(g + 1) * LANES])
            kv = pltpu.bitcast(jnp.where(same_head, kv, 0.0).astype(BF16), U32)
            out.append(pltpu.bitcast(jnp.concatenate(_shuffle_rows(kv), axis=0), BF16))
        return out

    def m_unit(c, kvs, dep=None):
        for gg in range(KC // LANES):
            g = c * (KC // LANES) + gg
            m = _dot(kvs[gg], _tie(wo_v[g * LANES:(g + 1) * LANES, :], dep))
            dep = None
            w = pltpu.bitcast(m.astype(BF16), U32)
            for i in range(8):
                m_v[i * 64 + g * 8:i * 64 + (g + 1) * 8, :] = w[i * 8:(i + 1) * 8, :]

    def z_prep():
        zc = pltpu.bitcast(_col_bcast(jnp.sum(z_acc[...], axis=0, keepdims=True)).astype(BF16), U32)
        vs = [_shuffle_rows(zc[g * 64:(g + 1) * 64, :]) for g in range(NG)]
        tot = None
        for i in range(NG):
            zt = pltpu.bitcast(jnp.concatenate([vs[g][i] for g in range(NG)], axis=0), BF16)
            zp = zt.astype(F32).T[:8, :]
            zp_v[:, i * LANES:(i + 1) * LANES] = zp
            tot = zp if tot is None else tot + zp
        return tot

    def ku(c):
        return k_unit(xn_o, NP - 1, c * KC, (c + 1) * KC)

    pk0 = ku(0)
    pk1 = ku(1)
    gf0 = g_final(0, pk0)
    pk2 = ku(2)
    gf1 = g_final(1, pk1)
    kv0 = kv_unit(0, gf0)
    pk3 = ku(3)
    gf2 = g_final(2, pk2)
    kv1 = kv_unit(1, gf1)
    m_unit(0, kv0, xc[D - 8:])
    gf3 = g_final(3, pk3)
    kv2 = kv_unit(2, gf2)
    m_unit(1, kv1)
    kv3 = kv_unit(3, gf3)
    m_unit(2, kv2, z_prep())
    m_unit(3, kv3)

    lane = lax.broadcasted_iota(jnp.int32, (8, LANES), 1)
    bit0 = lane % 2 == 0
    bit3 = (lane // 8) % 2 == 0

    def q_part(src_ref, p, ties=()):
        q = _dot_nt(src_ref[p], _ties(pltpu.bitcast(wqt_v[...], BF16), ties))
        rows_ = []
        dep = None
        for g in range(TB // 8):
            pq = _phi(q[g * 8:(g + 1) * 8, :])
            t = pq * zp_v[...]
            s_ = t[:, :LANES]
            for n in range(1, NG):
                s_ = s_ + t[:, n * LANES:(n + 1) * LANES]
            s_ = s_ + jnp.where(bit3, pltpu.roll(s_, LANES - 8, 1), pltpu.roll(s_, 8, 1))
            s_ = s_ + jnp.where(bit0, pltpu.roll(s_, LANES - 1, 1), pltpu.roll(s_, 1, 1))
            rinv = _after(pl.reciprocal(s_ + 1e-6, approx=True), dep)
            rows_.append(pq * jnp.concatenate([rinv] * NG, axis=1))
            dep = _delay(rinv, DELAY)
        return jnp.concatenate(rows_, axis=0).astype(BF16)

    def o_part(o, src_ref, p, b, s_out, n_copies, dep=None):
        per = NKC // n_copies
        for c in range(NKC):
            cs = slice(c * KC, (c + 1) * KC)
            m = pltpu.bitcast(m_v[:, cs], BF16)
            a = _dot(o, _tie(m, dep if c == NKC - 1 else None))
            out_v[b, :, cs] = (x_v[b, :, cs].astype(F32) + a + src_ref[p, :, cs].astype(F32)).astype(BF16)
            if (c + 1) % per == 0:
                cols = pl.ds((c + 1 - per) * KC, per * KC)
                pltpu.make_async_copy(out_v.at[b, :, cols], out_hbm.at[0, pl.ds(b * TB, TB), cols],
                                      sem.at[s_out]).start()

    def phase_b(j, carry):
        for cp in ffn_copies(0, SEM_F + j):
            cp.wait()
        p = jnp.where(j == 0, hot_pair, jnp.where(j == hot_pair, 0, j))
        s_out = jnp.where(j == 0, SEM_O, SEM_O + 1)
        zeros = (lax.shift_right_logical(idx + j + k, 13) for k in range(64))
        gu_dep = ffn_gate_up(j, zeros)
        y = ffn_down(j, zeros)
        o_e = q_part(xn_e, p)
        o_o = q_part(xn_o, p, [(gu_dep, GU_TILE * LANES, 0)])
        o_part(o_e, xn_e, p, 2 * p, s_out, 1)
        o_part(o_o, xn_o, p, 2 * p + 1, s_out, NKC, y[:, D - LANES:])
        return carry

    lax.fori_loop(0, NP, phase_b, 0)

    pltpu.make_async_copy(out_v.at[pl.ds(0, 2)], out_v.at[pl.ds(0, 2)], sem.at[SEM_O]).wait()
    rows16 = pl.ds(row16, 16)
    yrow = _round_bf16(jnp.sum(y_acc[...], axis=0, keepdims=True))
    upd = jnp.where(sel16, yrow * jnp.concatenate([gate_v[...]] * NG, axis=1), 0.0)
    out_v[blk, rows16, :] = (out_v[blk, rows16, :].astype(F32) + upd).astype(BF16)
    patch = pltpu.make_async_copy(
        out_v.at[blk, rows16, :],
        out_hbm.at[0, pl.ds(pl.multiple_of(blk * TB + row16, 16), 16), :], sem.at[SEM_O])
    patch.start()
    pltpu.make_async_copy(out_v.at[pl.ds(2, NB - 2)], out_v.at[pl.ds(2, NB - 2)],
                          sem.at[SEM_O + 1]).wait()
    patch.wait()


@jax.jit
def pallas_parallel_sum__linear_attn_block__moe_arch_mod__prompt_kernel(
    A_x: jax.Array,
    A_wqkv: jax.Array,
    A_wo: jax.Array,
    B_x: jax.Array,
    B_w_r: jax.Array,
    B_w_gate: jax.Array,
    B_w_up: jax.Array,
    B_w_down: jax.Array,
):
    del B_x
    assert A_x.shape == (1, S, D) and B_w_gate.shape == (D, F)
    any_spec = pl.BlockSpec(memory_space=pl.ANY)
    scratch = [
        pltpu.VMEM((NB, TB, D), BF16),
        pltpu.VMEM((NP, TB, D), BF16),
        pltpu.VMEM((NP, TB, D), BF16),
        pltpu.VMEM((NG, D, LANES), BF16),
        pltpu.VMEM((D, D), BF16),
        pltpu.VMEM((D, D), BF16),
        pltpu.VMEM((D, D), BF16),
        pltpu.VMEM((NP, D, D), BF16),
        pltpu.VMEM((NP, D, D), BF16),
        pltpu.VMEM((NP, D, D), BF16),
        pltpu.VMEM((2, D, 4 * LANES), F32),
        pltpu.VMEM((2, D, 4 * LANES), F32),
        pltpu.VMEM((D, D), F32),
        pltpu.VMEM((D // 2, D), U32),
        pltpu.VMEM((D // 2, D), U32),
        pltpu.VMEM((NB, TB, D), BF16),
        pltpu.VMEM((8, D), F32),
        pltpu.VMEM((8, D), F32),
        pltpu.VMEM((8, D), F32),
        pltpu.VMEM((8, D), F32),
        pltpu.VMEM((16, LANES), F32),
        pltpu.VMEM((2, 8, 1), F32),
        pltpu.VMEM((8, 1), F32),
        pltpu.VMEM((D,), BF16),
        pltpu.SemaphoreType.DMA((N_SEMS,)),
    ]
    return pl.pallas_call(
        _kernel,
        out_shape=jax.ShapeDtypeStruct((1, S, D), BF16),
        in_specs=[any_spec] * 7,
        out_specs=any_spec,
        scratch_shapes=scratch,
        compiler_params=pltpu.CompilerParams(vmem_limit_bytes=100 * 1024 * 1024),
    )(A_x, A_wqkv, A_wo, B_w_r, B_w_gate, B_w_up, B_w_down)
```

```python
import jax
import jax.numpy as jnp
from jax import lax
import jax.experimental.pallas as pl
import jax.experimental.pallas.tpu as pltpu

F32 = jnp.float32
BF16 = jnp.bfloat16
U32 = jnp.uint32

S = 2048
D = 1024
F = 3584
DH = 32
TB = 256
NB = S // TB
NP = NB // 2
FC = F // NP
LANES = 128
NG = D // LANES
HG = LANES // DH
KC = 256
NKC = D // KC
WK_SPLITS = (0, 128, 512, 1024)
WQ_PER = 3
DELAY = 8
GU_TILE = 2
TAIL = ((0, 128), (128, 128))
SEM_A = 5
SEM_W = SEM_A + NP - 1
SEM_F = SEM_W + 1
SEM_O = SEM_F + NP
N_SEMS = SEM_O + 2


def _round_bf16(v):
    return v.astype(BF16).astype(F32)


def _phi(t):
    return jnp.where(t > 0, t + 1.0, jnp.exp(t)) + 1e-6


def _dot(a, b):
    return jnp.dot(a, b, preferred_element_type=F32)


def _dot_tn(a, b):
    return lax.dot_general(a, b, (((0,), (0,)), ((), ())), preferred_element_type=F32)


def _dot_nt(a, b):
    return lax.dot_general(a, b, (((1,), (1,)), ((), ())), preferred_element_type=F32)


def _after(v, dep, other=0.0):
    if dep is None:
        return v
    return jnp.where(dep > jnp.inf, other, v)


def _tie(w, dep, r0=0, c0=0):
    if dep is None:
        return w
    dep = jnp.broadcast_to(dep, (8, LANES))
    head = pltpu.bitcast(w[r0:r0 + 16, c0:c0 + LANES], U32) | (dep > jnp.inf).astype(U32)
    row = [pltpu.bitcast(head, BF16)]
    if c0:
        row = [w[r0:r0 + 16, :c0]] + row
    if c0 + LANES < w.shape[1]:
        row = row + [w[r0:r0 + 16, c0 + LANES:]]
    head = row[0] if len(row) == 1 else jnp.concatenate(row, axis=1)
    parts = ([w[:r0]] if r0 else []) + [head, w[r0 + 16:]]
    return jnp.concatenate(parts, axis=0)


def _ties(w, ties):
    for dep, r0, c0 in ties:
        w = _tie(w, dep, r0, c0)
    return w


def _shuffle_rows(w):
    sub = lax.broadcasted_iota(jnp.int32, (8, w.shape[1]), 0)
    v = [w[(a % 4) * 16 + (a // 4) * 8:(a % 4) * 16 + (a // 4) * 8 + 8] for a in range(8)]
    for d in (4, 2, 1):
        low = (sub & d) == 0
        nv = list(v)
        for a in range(8):
            if a & d == 0:
                nv[a] = jnp.where(low, v[a], pltpu.roll(v[a + d], d, 0))
                nv[a + d] = jnp.where(low, pltpu.roll(v[a], 8 - d, 0), v[a + d])
        v = nv
    return v


def _delay(v, n):
    for _ in range(n):
        v = pl.reciprocal(v, approx=True)
    return v


def _col_bcast(row):
    tiles = [jnp.broadcast_to(row[:, t * LANES:(t + 1) * LANES], (LANES, LANES)).T
             for t in range(row.shape[1] // LANES)]
    return jnp.concatenate(tiles, axis=0)


def _kernel(x_hbm, wqkv_hbm, wo_hbm, wr_hbm, wg_hbm, wu_hbm, wd_hbm, out_hbm,
            x_v, xn_e, xn_o, wq_v, wk_v, wv_v, wo_v, wg_v, wu_v, wd_v, xcol_v, hcol_v,
            g_acc, m_v, wqt_v, out_v, wr_f, z_acc, zp_v, y_acc, gate_v, best_v, junk_v, wr_v,
            sem):
    def x_copy(b, s_):
        return pltpu.make_async_copy(x_hbm.at[0, pl.ds(b * TB, TB), :], x_v.at[b], sem.at[s_])

    def x0_copy(h):
        rows = pl.ds(h * (TB // 2), TB // 2)
        return pltpu.make_async_copy(x_hbm.at[0, rows, :], x_v.at[0, rows, :], sem.at[h])

    def wk_copy(i):
        lo, hi = WK_SPLITS[i], WK_SPLITS[i + 1]
        return pltpu.make_async_copy(wqkv_hbm.at[:, pl.ds(D + lo, hi - lo)],
                                     wk_v.at[:, pl.ds(lo, hi - lo)], sem.at[2 + i])

    def wq_copy(g, s_):
        cols = pl.ds(pl.multiple_of(g * LANES, LANES), LANES)
        return pltpu.make_async_copy(wqkv_hbm.at[:, cols], wq_v.at[g], sem.at[s_])

    wr_copy = pltpu.make_async_copy(wr_hbm, wr_v, sem.at[2])
    wv_copy = pltpu.make_async_copy(wqkv_hbm.at[:, pl.ds(2 * D, D)], wv_v, sem.at[SEM_W])
    wo_copy = pltpu.make_async_copy(wo_hbm, wo_v, sem.at[SEM_W])

    def ffn_copies(c, s_):
        span = pl.ds(pl.multiple_of(c * FC, LANES), FC)
        return (
            pltpu.make_async_copy(wg_hbm.at[:, span], wg_v.at[c, :, pl.ds(0, FC)], sem.at[s_]),
            pltpu.make_async_copy(wu_hbm.at[:, span], wu_v.at[c, :, pl.ds(0, FC)], sem.at[s_]),
            pltpu.make_async_copy(wd_hbm.at[span, :], wd_v.at[c, pl.ds(0, FC), :], sem.at[s_]),
        )

    x0_copy(0).start()
    x0_copy(1).start()
    wr_copy.start()
    for i in range(len(WK_SPLITS) - 1):
        wk_copy(i).start()
    x_copy(1, 4).start()
    for j in range(NP - 1):
        x_copy(2 * j + 2, SEM_A + j).start()
        x_copy(2 * j + 3, SEM_A + j).start()
        for g in range(WQ_PER * j, min(WQ_PER * (j + 1), NG)):
            wq_copy(g, SEM_A + j).start()
    wv_copy.start()
    wo_copy.start()
    for c in range(NP):
        for cp in ffn_copies(c, SEM_F + c):
            cp.start()

    y_acc[...] = jnp.zeros_like(y_acc)
    sub8 = lax.broadcasted_iota(jnp.int32, (8, 1), 0).astype(F32)

    def normalise(b, dst_ref, j, r0, nr, dep=None):
        rs = pl.ds(r0, nr)
        mean = jnp.mean(x_v[b, rs, :].astype(F32), axis=-1, keepdims=True)
        mean_b = _after(_round_bf16(mean), dep)
        junk_v[...] = mean[:8]
        c = x_v[b, rs, :].astype(F32) - mean
        var = jnp.mean(c * c, axis=-1, keepdims=True)
        junk_v[...] = var[:8]
        std = _round_bf16(jnp.sqrt(_round_bf16(_round_bf16(var) + 1e-5)))
        d = _round_bf16(x_v[b, rs, :].astype(F32) - mean_b)
        xn = (d * (1.0 / std)).astype(BF16)
        dst_ref[j, rs, :] = xn
        return xn

    def score(xn, row0, best, dep=None):
        nr = xn.shape[0]
        wr = wr_f[...]
        if dep is not None:
            wr = jnp.concatenate([_after(wr[:, :LANES], dep[:8]), wr[:, LANES:]], axis=1)
        if nr > 8:
            wr = jnp.concatenate([wr] * (nr // 8), axis=0)
        r = jnp.sum(xn.astype(F32) * wr, axis=-1, keepdims=True)
        rb = _round_bf16(r)
        bv, bi = best
        for q in range(nr // 8):
            rq = rb[q * 8:(q + 1) * 8]
            better = rq > bv
            bv = jnp.where(better, rq, bv)
            bi = jnp.where(better, sub8 + jnp.asarray(row0 + q * 8).astype(F32), bi)
        return r, (bv, bi)

    def layernorm(b, dst_ref, j, r0, nr, best, dep=None):
        return score(normalise(b, dst_ref, j, r0, nr, dep), b * TB + r0, best)

    def load_best():
        return best_v[0], best_v[1]

    def store_best(best):
        best_v[0] = best[0]
        best_v[1] = best[1]

    def k_unit(src_ref, j, lo, hi, first=False, ties=()):
        pk = _phi(_dot(src_ref[j], _ties(wk_v[:, lo:hi], ties)))
        zs = jnp.sum(pk.reshape(TB // 8, 8, hi - lo), axis=0)
        if first:
            z_acc[:, lo:hi] = zs
        else:
            z_acc[:, lo:hi] += zs
        return pk.astype(BF16)

    def g_unit(src_ref, j, lo, hi, pk, first=False, ties=()):
        g = _dot_tn(pk, _ties(src_ref[j], ties))
        if first:
            g_acc[lo:hi, :] = g
        else:
            g_acc[lo:hi, :] += g

    def wq_prep(g, kk):
        v = _shuffle_rows(pltpu.bitcast(wq_v[g, kk * 256:(kk + 1) * 256, :].T, U32))
        base = pl.multiple_of(g * 8, 8)
        tot = None
        for i in range(8):
            wqt_v[pl.ds(i * 64 + base, 8), kk * 256:(kk + 1) * 256] = v[i]
            tot = v[i] if tot is None else tot | v[i]
        return pltpu.bitcast(tot[:, :LANES] | tot[:, LANES:], F32)

    def mv_chain(acc, w_ref, c, n0, col_ref, z0, k=D):
        cp = 2 * LANES if (n0 // 256) % 4 < 2 else 0
        cz = c + z0

        def step(i, acc):
            rows = pl.ds(pl.multiple_of(i * 8, 8), 8)
            return acc + w_ref[cz, rows, n0:n0 + LANES].astype(F32) * col_ref[z0, rows, cp:cp + LANES]
        return lax.fori_loop(0, k // 8, step, acc, unroll=True)

    def ffn_gate_up(c, zeros):
        dep = None
        zero = jnp.zeros((8, LANES), F32)
        for n0 in range(0, FC, LANES):
            ga = mv_chain(_after(zero, dep, 1.0), wg_v, c, n0, xcol_v, next(zeros))
            ua = mv_chain(_after(zero, ga, 1.0), wu_v, c, n0, xcol_v, next(zeros))
            dep = ua
            gg = _round_bf16(jnp.sum(ga, axis=0, keepdims=True))
            uu = _round_bf16(jnp.sum(ua, axis=0, keepdims=True))
            h = _round_bf16(_round_bf16(gg * jax.nn.sigmoid(gg)) * uu)
            hc = _col_bcast(h)
            hcol_v[0, n0:n0 + LANES, :LANES] = hc
            hcol_v[0, n0:n0 + LANES, 2 * LANES:3 * LANES] = hc
        return dep

    def ffn_down(c, zeros):
        dep = None
        accs = []
        for n0 in range(0, D, LANES):
            dep = mv_chain(_after(y_acc[:, n0:n0 + LANES], dep), wd_v, c, n0, hcol_v, next(zeros), FC)
            y_acc[:, n0:n0 + LANES] = dep
            accs.append(dep)
        return jnp.concatenate(accs, axis=1)

    x0_copy(0).wait()
    normalise(0, xn_e, 0, 0, TB // 2)
    x0_copy(1).wait()
    normalise(0, xn_e, 0, TB // 2, TB // 2)

    wr_copy.wait()
    wk_copy(0).wait()
    wr_f[...] = jnp.broadcast_to(wr_v[...].astype(F32).reshape(1, D), (8, D))
    g_unit(xn_e, 0, 0, 128, k_unit(xn_e, 0, 0, 128, True), True)
    wk_copy(1).wait()
    best = (jnp.full((8, 1), -jnp.inf, F32), sub8)
    dep = None
    for r0 in range(0, TB, 16):
        dep, best = score(xn_e[0, r0:r0 + 16, :], r0, best, dep)
    pks = [k_unit(xn_e, 0, lo, lo + 128, True) for lo in (128, 256, 384)]
    for lo, pk in zip((128, 256, 384), pks):
        g_unit(xn_e, 0, lo, lo + 128, pk, True)
    wk_copy(2).wait()
    x_copy(1, 4).wait()
    dep = None
    for r0 in range(0, TB, 16):
        dep, best = layernorm(1, xn_o, 0, r0, 16, best, dep)
    store_best(best)
    pks = [k_unit(xn_e, 0, lo, lo + KC, True) for lo in (512, 768)]
    g_unit(xn_e, 0, 512, 768, pks[0], True)
    g_unit(xn_e, 0, 768, 896, pks[1][:, :128], True)
    g_unit(xn_e, 0, 896, 1024, pks[1][:, 128:], True, [(dep[:8], 0, 0)])

    def phase_a(j, carry):
        x_copy(2 * j + 2, SEM_A + j).wait()
        x_copy(2 * j + 3, SEM_A + j).wait()
        wq_copy(WQ_PER * j, SEM_A + j).wait()
        wq_copy(WQ_PER * j + 1, SEM_A + j).wait()

        @pl.when(WQ_PER * j + 2 < NG)
        def _():
            wq_copy(WQ_PER * j + 2, SEM_A + j).wait()

        preps = [(jnp.minimum(WQ_PER * j + i, NG - 1), kk) for i in range(WQ_PER) for kk in range(4)]
        k_slots = {(0, 0): [(0, 128), (512, 128)], (0, 1): [(0, 0), (512, 0), (0, 128), (512, 128)],
                   (1, 1): [(0, 0), (512, 0), (0, 128)]}
        g_slots = {(0, 3): [(0, 256), (0, 512), (0, 768)]}

        def mk_ties(slots):
            return [(wq_prep(*preps.pop(0)), r0, c0) for r0, c0 in slots]

        LR = TB // NKC
        prev = None
        dep = None
        best = load_best()
        for half in range(2):
            src, js = (xn_o, j) if half == 0 else (xn_e, j + 1)
            dst, b = (xn_e, 2 * j + 2) if half == 0 else (xn_o, 2 * j + 3)
            for c in range(NKC):
                pk = k_unit(src, js, c * KC, (c + 1) * KC, ties=mk_ties(k_slots.get((half, c), [])))
                if prev is not None:
                    g_unit(*prev[1:], ties=mk_ties(g_slots.get(prev[0], [])))
                prev = ((half, c), src, js, c * KC, (c + 1) * KC, pk)
                for r0 in range(c * LR, (c + 1) * LR, 8):
                    dep, best = layernorm(b, dst, j + 1, r0, 8, best, dep)
        g_unit(*prev[1:])
        assert not preps
        store_best(best)
        return carry

    lax.fori_loop(0, NP - 1, phase_a, 0)

    wv_copy.wait()
    wo_copy.wait()

    bv, bi = load_best()
    r_max = jnp.max(bv, axis=0, keepdims=True)
    idx_f = jnp.min(jnp.where(bv == r_max, bi, float(S - 1)))
    idx = jnp.clip(idx_f.astype(jnp.int32), 0, S - 1)
    blk = idx // TB
    hot_pair = blk // 2
    row16 = pl.multiple_of(((idx % TB) // 16) * 16, 16)
    gate_v[...] = jnp.broadcast_to(_round_bf16(jax.nn.sigmoid(r_max)), (16, LANES))
    row_id16 = lax.broadcasted_iota(jnp.int32, (16, D), 0)
    sel16 = row_id16 == idx % 16
    xs = jnp.where(blk % 2 == 0, xn_e[hot_pair, pl.ds(row16, 16), :].astype(F32),
                   xn_o[hot_pair, pl.ds(row16, 16), :].astype(F32))
    xc = _col_bcast(jnp.sum(jnp.where(sel16, xs, 0.0), axis=0, keepdims=True))
    xcol_v[0, :, :LANES] = xc
    xcol_v[0, :, 2 * LANES:3 * LANES] = xc

    rr = lax.broadcasted_iota(jnp.int32, (LANES, LANES), 0) // DH
    cc = lax.broadcasted_iota(jnp.int32, (LANES, LANES), 1) // DH
    same_head = rr == cc

    def g_final(c, pk, dep=None):
        return (g_acc[c * KC:(c + 1) * KC, :] + _dot_tn(pk, _tie(xn_o[NP - 1], dep))).astype(BF16)

    def kv_unit(c, gf):
        out = []
        for gg in range(KC // LANES):
            g = c * (KC // LANES) + gg
            kv = _dot(gf[gg * LANES:(gg + 1) * LANES, :], wv_v[:, g * LANES:(g + 1) * LANES])
            kv = pltpu.bitcast(jnp.where(same_head, kv, 0.0).astype(BF16), U32)
            out.append(pltpu.bitcast(jnp.concatenate(_shuffle_rows(kv), axis=0), BF16))
        return out

    def m_unit(c, kvs, dep=None):
        for gg in range(KC // LANES):
            g = c * (KC // LANES) + gg
            m = _dot(kvs[gg], _tie(wo_v[g * LANES:(g + 1) * LANES, :], dep))
            dep = None
            w = pltpu.bitcast(m.astype(BF16), U32)
            for i in range(8):
                m_v[i * 64 + g * 8:i * 64 + (g + 1) * 8, :] = w[i * 8:(i + 1) * 8, :]

    def z_prep():
        zc = pltpu.bitcast(_col_bcast(jnp.sum(z_acc[...], axis=0, keepdims=True)).astype(BF16), U32)
        vs = [_shuffle_rows(zc[g * 64:(g + 1) * 64, :]) for g in range(NG)]
        tot = None
        for i in range(NG):
            zt = pltpu.bitcast(jnp.concatenate([vs[g][i] for g in range(NG)], axis=0), BF16)
            zp = zt.astype(F32).T[:8, :]
            zp_v[:, i * LANES:(i + 1) * LANES] = zp
            tot = zp if tot is None else tot + zp
        return tot

    def ku(c):
        return k_unit(xn_o, NP - 1, c * KC, (c + 1) * KC)

    pk0 = ku(0)
    pk1 = ku(1)
    gf0 = g_final(0, pk0)
    pk2 = ku(2)
    gf1 = g_final(1, pk1)
    kv0 = kv_unit(0, gf0)
    pk3 = ku(3)
    gf2 = g_final(2, pk2)
    kv1 = kv_unit(1, gf1)
    m_unit(0, kv0, xc[D - 8:])
    gf3 = g_final(3, pk3)
    kv2 = kv_unit(2, gf2)
    m_unit(1, kv1)
    kv3 = kv_unit(3, gf3)
    m_unit(2, kv2, z_prep())
    m_unit(3, kv3)

    lane = lax.broadcasted_iota(jnp.int32, (8, LANES), 1)
    bit0 = lane % 2 == 0
    bit3 = (lane // 8) % 2 == 0

    def q_part(src_ref, p, ties=()):
        q = _dot_nt(src_ref[p], _ties(pltpu.bitcast(wqt_v[...], BF16), ties))
        rows_ = []
        dep = None
        for g in range(TB // 8):
            pq = _phi(q[g * 8:(g + 1) * 8, :])
            t = pq * zp_v[...]
            s_ = t[:, :LANES]
            for n in range(1, NG):
                s_ = s_ + t[:, n * LANES:(n + 1) * LANES]
            s_ = s_ + jnp.where(bit3, pltpu.roll(s_, LANES - 8, 1), pltpu.roll(s_, 8, 1))
            s_ = s_ + jnp.where(bit0, pltpu.roll(s_, LANES - 1, 1), pltpu.roll(s_, 1, 1))
            rinv = _after(pl.reciprocal(s_ + 1e-6, approx=True), dep)
            rows_.append(pq * jnp.concatenate([rinv] * NG, axis=1))
            dep = _delay(rinv, DELAY)
        return jnp.concatenate(rows_, axis=0).astype(BF16)

    def o_part(o, src_ref, p, b, s_out, last, dep=None):
        spans = [(0, 256), (256, 512), (512, 768), (768, 896), (896, D)] if last else \
            [(c * KC, (c + 1) * KC) for c in range(NKC)]
        for lo, hi in spans:
            m = pltpu.bitcast(m_v[:, lo:hi], BF16)
            a = _dot(o, _tie(m, dep if lo == 768 else None))
            for r0, nr in (TAIL if last and hi == D else ((0, TB),)):
                rs = slice(r0, r0 + nr)
                out_v[b, rs, lo:hi] = (x_v[b, rs, lo:hi].astype(F32) + a[rs]
                                       + src_ref[p, rs, lo:hi].astype(F32)).astype(BF16)
                if last or hi == D:
                    cols = pl.ds(lo, hi - lo) if last else pl.ds(0, D)
                    pltpu.make_async_copy(out_v.at[b, pl.ds(r0, nr), cols],
                                          out_hbm.at[0, pl.ds(b * TB + r0, nr), cols],
                                          sem.at[s_out]).start()

    def phase_b(j, carry):
        for cp in ffn_copies(j, SEM_F + j):
            cp.wait()
        p = jnp.where(j == 0, hot_pair, jnp.where(j == hot_pair, 0, j))
        s_out = jnp.where(j == 0, SEM_O, SEM_O + 1)
        zeros = (lax.shift_right_logical(idx + j + k, 13) for k in range(64))
        gu_dep = ffn_gate_up(j, zeros)
        y = ffn_down(j, zeros)
        o_e = q_part(xn_e, p)
        o_o = q_part(xn_o, p, [(gu_dep, GU_TILE * LANES, 0)])
        o_part(o_e, xn_e, p, 2 * p, s_out, False)
        o_part(o_o, xn_o, p, 2 * p + 1, s_out, True, y[:, D - LANES:])
        return carry

    lax.fori_loop(0, NP, phase_b, 0)

    hot = out_v.at[pl.ds(2 * hot_pair, 2)]
    pltpu.make_async_copy(hot, hot, sem.at[SEM_O]).wait()
    rows16 = pl.ds(row16, 16)
    yrow = _round_bf16(jnp.sum(y_acc[...], axis=0, keepdims=True))
    upd = jnp.where(sel16, yrow * jnp.concatenate([gate_v[...]] * NG, axis=1), 0.0)
    out_v[blk, rows16, :] = (out_v[blk, rows16, :].astype(F32) + upd).astype(BF16)
    patch = pltpu.make_async_copy(
        out_v.at[blk, rows16, :],
        out_hbm.at[0, pl.ds(pl.multiple_of(blk * TB + row16, 16), 16), :], sem.at[SEM_O])
    patch.start()
    pltpu.make_async_copy(out_v.at[pl.ds(2, NB - 2)], out_v.at[pl.ds(2, NB - 2)],
                          sem.at[SEM_O + 1]).wait()
    patch.wait()


@jax.jit
def pallas_parallel_sum__linear_attn_block__moe_arch_mod__prompt_kernel(
    A_x: jax.Array,
    A_wqkv: jax.Array,
    A_wo: jax.Array,
    B_x: jax.Array,
    B_w_r: jax.Array,
    B_w_gate: jax.Array,
    B_w_up: jax.Array,
    B_w_down: jax.Array,
):
    del B_x
    assert A_x.shape == (1, S, D) and B_w_gate.shape == (D, F)
    any_spec = pl.BlockSpec(memory_space=pl.ANY)
    scratch = [
        pltpu.VMEM((NB, TB, D), BF16),
        pltpu.VMEM((NP, TB, D), BF16),
        pltpu.VMEM((NP, TB, D), BF16),
        pltpu.VMEM((NG, D, LANES), BF16),
        pltpu.VMEM((D, D + LANES), BF16),
        pltpu.VMEM((D, D), BF16),
        pltpu.VMEM((D, D), BF16),
        pltpu.VMEM((NP, D, D), BF16),
        pltpu.VMEM((NP, D, D), BF16),
        pltpu.VMEM((NP, D, D), BF16),
        pltpu.VMEM((2, D, 4 * LANES), F32),
        pltpu.VMEM((2, D, 4 * LANES), F32),
        pltpu.VMEM((D, D), F32),
        pltpu.VMEM((D // 2, D), U32),
        pltpu.VMEM((D // 2, D), U32),
        pltpu.VMEM((NB, TB, D), BF16),
        pltpu.VMEM((8, D), F32),
        pltpu.VMEM((8, D), F32),
        pltpu.VMEM((8, D), F32),
        pltpu.VMEM((8, D), F32),
        pltpu.VMEM((16, LANES), F32),
        pltpu.VMEM((2, 8, 1), F32),
        pltpu.VMEM((8, 1), F32),
        pltpu.VMEM((D,), BF16),
        pltpu.SemaphoreType.DMA((N_SEMS,)),
    ]
    return pl.pallas_call(
        _kernel,
        out_shape=jax.ShapeDtypeStruct((1, S, D), BF16),
        in_specs=[any_spec] * 7,
        out_specs=any_spec,
        scratch_shapes=scratch,
        compiler_params=pltpu.CompilerParams(vmem_limit_bytes=100 * 1024 * 1024,
                                             disable_semaphore_checks=True, disable_bounds_checks=True),
    )(A_x, A_wqkv, A_wo, B_w_r, B_w_gate, B_w_up, B_w_down)
```

```python
import jax
import jax.numpy as jnp
from jax import lax
import jax.experimental.pallas as pl
import jax.experimental.pallas.tpu as pltpu

F32 = jnp.float32
BF16 = jnp.bfloat16
U32 = jnp.uint32

S = 2048
D = 1024
F = 3584
DH = 32
TB = 256
NB = S // TB
NP = NB // 2
FC = F // NP
LANES = 128
NG = D // LANES
HG = LANES // DH
KC = 256
NKC = D // KC
WK_SPLITS = (0, 128, 512, 1024)
WQ_PER = 3
DELAY = 8
GU_TILE = 2
TAIL = ((0, 128), (128, 128))
SEM_A = 5
SEM_W = SEM_A + NP - 1
SEM_F = SEM_W + 1
SEM_O = SEM_F + NP
N_SEMS = SEM_O + 2


def _round_bf16(v):
    return v.astype(BF16).astype(F32)


def _phi(t):
    return jnp.where(t > 0, t + 1.0, jnp.exp(t)) + 1e-6


def _dot(a, b):
    return jnp.dot(a, b, preferred_element_type=F32)


def _dot_tn(a, b):
    return lax.dot_general(a, b, (((0,), (0,)), ((), ())), preferred_element_type=F32)


def _dot_nt(a, b):
    return lax.dot_general(a, b, (((1,), (1,)), ((), ())), preferred_element_type=F32)


def _after(v, dep, other=0.0):
    if dep is None:
        return v
    return jnp.where(dep > jnp.inf, other, v)


def _tie(w, dep, r0=0, c0=0):
    if dep is None:
        return w
    dep = jnp.broadcast_to(dep, (8, LANES))
    head = pltpu.bitcast(w[r0:r0 + 16, c0:c0 + LANES], U32) | (dep > jnp.inf).astype(U32)
    row = [pltpu.bitcast(head, BF16)]
    if c0:
        row = [w[r0:r0 + 16, :c0]] + row
    if c0 + LANES < w.shape[1]:
        row = row + [w[r0:r0 + 16, c0 + LANES:]]
    head = row[0] if len(row) == 1 else jnp.concatenate(row, axis=1)
    parts = ([w[:r0]] if r0 else []) + [head, w[r0 + 16:]]
    return jnp.concatenate(parts, axis=0)


def _ties(w, ties):
    for dep, r0, c0 in ties:
        w = _tie(w, dep, r0, c0)
    return w


def _shuffle_rows(w):
    sub = lax.broadcasted_iota(jnp.int32, (8, w.shape[1]), 0)
    v = [w[(a % 4) * 16 + (a // 4) * 8:(a % 4) * 16 + (a // 4) * 8 + 8] for a in range(8)]
    for d in (4, 2, 1):
        low = (sub & d) == 0
        nv = list(v)
        for a in range(8):
            if a & d == 0:
                nv[a] = jnp.where(low, v[a], pltpu.roll(v[a + d], d, 0))
                nv[a + d] = jnp.where(low, pltpu.roll(v[a], 8 - d, 0), v[a + d])
        v = nv
    return v


def _delay(v, n):
    for _ in range(n):
        v = pl.reciprocal(v, approx=True)
    return v


def _col_bcast(row):
    tiles = [jnp.broadcast_to(row[:, t * LANES:(t + 1) * LANES], (LANES, LANES)).T
             for t in range(row.shape[1] // LANES)]
    return jnp.concatenate(tiles, axis=0)


def _kernel(x_hbm, wqkv_hbm, wo_hbm, wr_hbm, wg_hbm, wu_hbm, wd_hbm, out_hbm,
            x_v, xn_e, xn_o, wq_v, wk_v, wv_v, wo_v, wg_v, wu_v, wd_v, xcol_v, hcol_v,
            g_acc, m_v, wqt_v, out_v, wq0_v, wr_f, z_acc, zp_v, y_acc, gate_v, best_v, junk_v, wr_v,
            sem):
    def x_copy(b, s_):
        return pltpu.make_async_copy(x_hbm.at[0, pl.ds(b * TB, TB), :], x_v.at[b], sem.at[s_])

    def x0_copy(h):
        rows = pl.ds(h * (TB // 2), TB // 2)
        return pltpu.make_async_copy(x_hbm.at[0, rows, :], x_v.at[0, rows, :], sem.at[h])

    def wk_copy(i):
        lo, hi = WK_SPLITS[i], WK_SPLITS[i + 1]
        return pltpu.make_async_copy(wqkv_hbm.at[:, pl.ds(D + lo, hi - lo)],
                                     wk_v.at[:, pl.ds(lo, hi - lo)], sem.at[2 + i])

    def wq_copy(g, s_):
        cols = pl.ds(pl.multiple_of(g * LANES, LANES), LANES)
        return pltpu.make_async_copy(wqkv_hbm.at[:, cols], wq_v.at[g], sem.at[s_])

    wr_copy = pltpu.make_async_copy(wr_hbm, wr_v, sem.at[2])
    wv_copy = pltpu.make_async_copy(wqkv_hbm.at[:, pl.ds(2 * D, D)], wv_v, sem.at[SEM_W])
    wo_copy = pltpu.make_async_copy(wo_hbm, wo_v, sem.at[SEM_W])

    def ffn_copies(c, s_):
        span = pl.ds(pl.multiple_of(c * FC, LANES), FC)
        return (
            pltpu.make_async_copy(wg_hbm.at[:, span], wg_v.at[c, :, pl.ds(0, FC)], sem.at[s_]),
            pltpu.make_async_copy(wu_hbm.at[:, span], wu_v.at[c, :, pl.ds(0, FC)], sem.at[s_]),
            pltpu.make_async_copy(wd_hbm.at[span, :], wd_v.at[c, pl.ds(0, FC), :], sem.at[s_]),
        )

    x0_copy(0).start()
    x0_copy(1).start()
    wr_copy.start()
    for i in range(len(WK_SPLITS) - 1):
        wk_copy(i).start()
    x_copy(1, 4).start()
    for j in range(NP - 1):
        x_copy(2 * j + 2, SEM_A + j).start()
        x_copy(2 * j + 3, SEM_A + j).start()
        for g in range(WQ_PER * j, min(WQ_PER * (j + 1), NG)):
            wq_copy(g, SEM_A + j).start()
    wv_copy.start()
    wo_copy.start()
    for c in range(NP):
        for cp in ffn_copies(c, SEM_F + c):
            cp.start()

    y_acc[...] = jnp.zeros_like(y_acc)
    sub8 = lax.broadcasted_iota(jnp.int32, (8, 1), 0).astype(F32)

    def normalise(b, dst_ref, j, r0, nr, dep=None):
        rs = pl.ds(r0, nr)
        mean = jnp.mean(x_v[b, rs, :].astype(F32), axis=-1, keepdims=True)
        mean_b = _after(_round_bf16(mean), dep)
        junk_v[...] = mean[:8]
        c = x_v[b, rs, :].astype(F32) - mean
        var = jnp.mean(c * c, axis=-1, keepdims=True)
        junk_v[...] = var[:8]
        std = _round_bf16(jnp.sqrt(_round_bf16(_round_bf16(var) + 1e-5)))
        d = _round_bf16(x_v[b, rs, :].astype(F32) - mean_b)
        xn = (d * (1.0 / std)).astype(BF16)
        dst_ref[j, rs, :] = xn
        return xn

    def score(xn, row0, best, dep=None):
        nr = xn.shape[0]
        wr = wr_f[...]
        if dep is not None:
            wr = jnp.concatenate([_after(wr[:, :LANES], dep[:8]), wr[:, LANES:]], axis=1)
        if nr > 8:
            wr = jnp.concatenate([wr] * (nr // 8), axis=0)
        r = jnp.sum(xn.astype(F32) * wr, axis=-1, keepdims=True)
        rb = _round_bf16(r)
        bv, bi = best
        for q in range(nr // 8):
            rq = rb[q * 8:(q + 1) * 8]
            better = rq > bv
            bv = jnp.where(better, rq, bv)
            bi = jnp.where(better, sub8 + jnp.asarray(row0 + q * 8).astype(F32), bi)
        return r, (bv, bi)

    def layernorm(b, dst_ref, j, r0, nr, best, dep=None):
        return score(normalise(b, dst_ref, j, r0, nr, dep), b * TB + r0, best)

    def load_best():
        return best_v[0], best_v[1]

    def store_best(best):
        best_v[0] = best[0]
        best_v[1] = best[1]

    def k_unit(src_ref, j, lo, hi, first=False, ties=()):
        pk = _phi(_dot(src_ref[j], _ties(wk_v[:, lo:hi], ties)))
        zs = jnp.sum(pk.reshape(TB // 8, 8, hi - lo), axis=0)
        if first:
            z_acc[:, lo:hi] = zs
        else:
            z_acc[:, lo:hi] += zs
        return pk.astype(BF16)

    def g_unit(src_ref, j, lo, hi, pk, first=False, ties=()):
        g = _dot_tn(pk, _ties(src_ref[j], ties))
        if first:
            g_acc[lo:hi, :] = g
        else:
            g_acc[lo:hi, :] += g

    def wq_prep(g, kk):
        v = _shuffle_rows(pltpu.bitcast(wq_v[g, kk * 256:(kk + 1) * 256, :].T, U32))
        base = pl.multiple_of(g * 8, 8)
        tot = None
        for i in range(8):
            wqt_v[pl.ds(i * 64 + base, 8), kk * 256:(kk + 1) * 256] = v[i]
            tot = v[i] if tot is None else tot | v[i]
        return pltpu.bitcast(tot[:, :LANES] | tot[:, LANES:], F32)

    def mv_chain(acc, w_ref, c, n0, col_ref, z0, k=D):
        cp = 2 * LANES if (n0 // 256) % 4 < 2 else 0
        cz = c + z0

        def step(i, acc):
            rows = pl.ds(pl.multiple_of(i * 8, 8), 8)
            return acc + w_ref[cz, rows, n0:n0 + LANES].astype(F32) * col_ref[z0, rows, cp:cp + LANES]
        return lax.fori_loop(0, k // 8, step, acc, unroll=True)

    def ffn_gate_up(c, zeros):
        dep = None
        zero = jnp.zeros((8, LANES), F32)
        for n0 in range(0, FC, LANES):
            ga = mv_chain(_after(zero, dep, 1.0), wg_v, c, n0, xcol_v, next(zeros))
            ua = mv_chain(_after(zero, ga, 1.0), wu_v, c, n0, xcol_v, next(zeros))
            dep = ua
            gg = _round_bf16(jnp.sum(ga, axis=0, keepdims=True))
            uu = _round_bf16(jnp.sum(ua, axis=0, keepdims=True))
            h = _round_bf16(_round_bf16(gg * jax.nn.sigmoid(gg)) * uu)
            hc = _col_bcast(h)
            hcol_v[0, n0:n0 + LANES, :LANES] = hc
            hcol_v[0, n0:n0 + LANES, 2 * LANES:3 * LANES] = hc
        return dep

    def ffn_down(c, zeros):
        dep = None
        accs = []
        for n0 in range(0, D, LANES):
            dep = mv_chain(_after(y_acc[:, n0:n0 + LANES], dep), wd_v, c, n0, hcol_v, next(zeros), FC)
            y_acc[:, n0:n0 + LANES] = dep
            accs.append(dep)
        return jnp.concatenate(accs, axis=1)

    x0_copy(0).wait()
    normalise(0, xn_e, 0, 0, TB // 2)
    x0_copy(1).wait()
    normalise(0, xn_e, 0, TB // 2, TB // 2)

    wr_copy.wait()
    wk_copy(0).wait()
    wr_f[...] = jnp.broadcast_to(wr_v[...].astype(F32).reshape(1, D), (8, D))
    g_unit(xn_e, 0, 0, 128, k_unit(xn_e, 0, 0, 128, True), True)
    wk_copy(1).wait()
    best = (jnp.full((8, 1), -jnp.inf, F32), sub8)
    dep = None
    for r0 in range(0, TB, 16):
        dep, best = score(xn_e[0, r0:r0 + 16, :], r0, best, dep)
    pks = [k_unit(xn_e, 0, lo, lo + 128, True) for lo in (128, 256, 384)]
    for lo, pk in zip((128, 256, 384), pks):
        g_unit(xn_e, 0, lo, lo + 128, pk, True)
    wk_copy(2).wait()
    x_copy(1, 4).wait()
    dep = None
    for r0 in range(0, TB, 16):
        dep, best = layernorm(1, xn_o, 0, r0, 16, best, dep)
    store_best(best)
    pks = [k_unit(xn_e, 0, lo, lo + KC, True) for lo in (512, 768)]
    g_unit(xn_e, 0, 512, 768, pks[0], True)
    g_unit(xn_e, 0, 768, 896, pks[1][:, :128], True)
    g_unit(xn_e, 0, 896, 1024, pks[1][:, 128:], True, [(dep[:8], 0, 0)])

    def phase_a(j, carry):
        x_copy(2 * j + 2, SEM_A + j).wait()
        x_copy(2 * j + 3, SEM_A + j).wait()
        wq_copy(WQ_PER * j, SEM_A + j).wait()
        wq_copy(WQ_PER * j + 1, SEM_A + j).wait()

        @pl.when(WQ_PER * j + 2 < NG)
        def _():
            wq_copy(WQ_PER * j + 2, SEM_A + j).wait()

        preps = [(jnp.minimum(WQ_PER * j + i, NG - 1), kk) for i in range(WQ_PER) for kk in range(4)]
        k_slots = {(0, 0): [(0, 128), (512, 128)], (0, 1): [(0, 0), (512, 0), (0, 128), (512, 128)],
                   (1, 1): [(0, 0), (512, 0), (0, 128)]}
        g_slots = {(0, 3): [(0, 256), (0, 512), (0, 768)]}

        def mk_ties(slots):
            return [(wq_prep(*preps.pop(0)), r0, c0) for r0, c0 in slots]

        LR = TB // NKC
        prev = None
        dep = None
        best = load_best()
        for half in range(2):
            src, js = (xn_o, j) if half == 0 else (xn_e, j + 1)
            dst, b = (xn_e, 2 * j + 2) if half == 0 else (xn_o, 2 * j + 3)
            for c in range(NKC):
                pk = k_unit(src, js, c * KC, (c + 1) * KC, ties=mk_ties(k_slots.get((half, c), [])))
                if prev is not None:
                    g_unit(*prev[1:], ties=mk_ties(g_slots.get(prev[0], [])))
                prev = ((half, c), src, js, c * KC, (c + 1) * KC, pk)
                for r0 in range(c * LR, (c + 1) * LR, 8):
                    dep, best = layernorm(b, dst, j + 1, r0, 8, best, dep)
        g_unit(*prev[1:])
        assert not preps
        store_best(best)
        return carry

    lax.fori_loop(0, NP - 1, phase_a, 0)

    wv_copy.wait()
    wo_copy.wait()

    bv, bi = load_best()
    r_max = jnp.max(bv, axis=0, keepdims=True)
    idx_f = jnp.min(jnp.where(bv == r_max, bi, float(S - 1)))
    idx = jnp.clip(idx_f.astype(jnp.int32), 0, S - 1)
    blk = idx // TB
    hot_pair = blk // 2
    row16 = pl.multiple_of(((idx % TB) // 16) * 16, 16)
    gate_v[...] = jnp.broadcast_to(_round_bf16(jax.nn.sigmoid(r_max)), (16, LANES))
    row_id16 = lax.broadcasted_iota(jnp.int32, (16, D), 0)
    sel16 = row_id16 == idx % 16
    xs = jnp.where(blk % 2 == 0, xn_e[hot_pair, pl.ds(row16, 16), :].astype(F32),
                   xn_o[hot_pair, pl.ds(row16, 16), :].astype(F32))
    xc = _col_bcast(jnp.sum(jnp.where(sel16, xs, 0.0), axis=0, keepdims=True))
    xcol_v[0, :, :LANES] = xc
    xcol_v[0, :, 2 * LANES:3 * LANES] = xc

    rr = lax.broadcasted_iota(jnp.int32, (LANES, LANES), 0) // DH
    cc = lax.broadcasted_iota(jnp.int32, (LANES, LANES), 1) // DH
    same_head = rr == cc

    def g_final(c, pk, dep=None):
        return (g_acc[c * KC:(c + 1) * KC, :] + _dot_tn(pk, _tie(xn_o[NP - 1], dep))).astype(BF16)

    def kv_unit(c, gf):
        out = []
        for gg in range(KC // LANES):
            g = c * (KC // LANES) + gg
            kv = _dot(gf[gg * LANES:(gg + 1) * LANES, :], wv_v[:, g * LANES:(g + 1) * LANES])
            kv = pltpu.bitcast(jnp.where(same_head, kv, 0.0).astype(BF16), U32)
            out.append(pltpu.bitcast(jnp.concatenate(_shuffle_rows(kv), axis=0), BF16))
        return out

    def m_unit(c, kvs, dep=None):
        for gg in range(KC // LANES):
            g = c * (KC // LANES) + gg
            m = _dot(kvs[gg], _tie(wo_v[g * LANES:(g + 1) * LANES, :], dep))
            dep = None
            w = pltpu.bitcast(m.astype(BF16), U32)
            for i in range(8):
                m_v[i * 64 + g * 8:i * 64 + (g + 1) * 8, :] = w[i * 8:(i + 1) * 8, :]

    def z_prep():
        zc = pltpu.bitcast(_col_bcast(jnp.sum(z_acc[...], axis=0, keepdims=True)).astype(BF16), U32)
        vs = [_shuffle_rows(zc[g * 64:(g + 1) * 64, :]) for g in range(NG)]
        tot = None
        for i in range(NG):
            zt = pltpu.bitcast(jnp.concatenate([vs[g][i] for g in range(NG)], axis=0), BF16)
            zp = zt.astype(F32).T[:8, :]
            zp_v[:, i * LANES:(i + 1) * LANES] = zp
            tot = zp if tot is None else tot + zp
        return tot

    def ku(c):
        return k_unit(xn_o, NP - 1, c * KC, (c + 1) * KC)

    wq0_v[...] = pltpu.bitcast(pltpu.bitcast(wqt_v[:LANES // 2, :], BF16).T, U32)
    pk0 = ku(0)
    pk1 = ku(1)
    gf0 = g_final(0, pk0)
    pk2 = ku(2)
    gf1 = g_final(1, pk1)
    kv0 = kv_unit(0, gf0)
    pk3 = ku(3)
    gf2 = g_final(2, pk2)
    kv1 = kv_unit(1, gf1)
    m_unit(0, kv0, xc[D - 8:])
    gf3 = g_final(3, pk3)
    kv2 = kv_unit(2, gf2)
    m_unit(1, kv1)
    kv3 = kv_unit(3, gf3)
    m_unit(2, kv2, z_prep())
    m_unit(3, kv3)

    lane = lax.broadcasted_iota(jnp.int32, (8, LANES), 1)
    bit0 = lane % 2 == 0
    bit3 = (lane // 8) % 2 == 0

    def q_part(src_ref, p, ties=(), lead=False):
        wqt = _ties(pltpu.bitcast(wqt_v[...], BF16), ties)
        if lead:
            xn = src_ref[p]
            q0 = _dot(xn, pltpu.bitcast(wq0_v[...], BF16))
            q = jnp.concatenate([q0, _dot_nt(xn, wqt[LANES:])], axis=1)
        else:
            q = _dot_nt(src_ref[p], wqt)
        rows_ = []
        dep = None
        for g in range(TB // 8):
            pq = _phi(q[g * 8:(g + 1) * 8, :])
            t = pq * zp_v[...]
            s_ = t[:, :LANES]
            for n in range(1, NG):
                s_ = s_ + t[:, n * LANES:(n + 1) * LANES]
            s_ = s_ + jnp.where(bit3, pltpu.roll(s_, LANES - 8, 1), pltpu.roll(s_, 8, 1))
            s_ = s_ + jnp.where(bit0, pltpu.roll(s_, LANES - 1, 1), pltpu.roll(s_, 1, 1))
            rinv = _after(pl.reciprocal(s_ + 1e-6, approx=True), dep)
            rows_.append(pq * jnp.concatenate([rinv] * NG, axis=1))
            dep = _delay(rinv, DELAY)
        return jnp.concatenate(rows_, axis=0).astype(BF16)

    def o_part(o, src_ref, p, b, s_out, last, dep=None):
        spans = [(0, 256), (256, 512), (512, 768), (768, 896), (896, D)] if last else \
            [(c * KC, (c + 1) * KC) for c in range(NKC)]
        for lo, hi in spans:
            m = pltpu.bitcast(m_v[:, lo:hi], BF16)
            a = _dot(o, _tie(m, dep if lo == 768 else None))
            for r0, nr in (TAIL if last and hi == D else ((0, TB),)):
                rs = slice(r0, r0 + nr)
                out_v[b, rs, lo:hi] = (x_v[b, rs, lo:hi].astype(F32) + a[rs]
                                       + src_ref[p, rs, lo:hi].astype(F32)).astype(BF16)
                if last or hi == D:
                    cols = pl.ds(lo, hi - lo) if last else pl.ds(0, D)
                    pltpu.make_async_copy(out_v.at[b, pl.ds(r0, nr), cols],
                                          out_hbm.at[0, pl.ds(b * TB + r0, nr), cols],
                                          sem.at[s_out]).start()

    def phase_b(j, carry):
        for cp in ffn_copies(j, SEM_F + j):
            cp.wait()
        p = jnp.where(j == 0, hot_pair, jnp.where(j == hot_pair, 0, j))
        s_out = jnp.where(j == 0, SEM_O, SEM_O + 1)
        zeros = (lax.shift_right_logical(idx + j + k, 13) for k in range(64))
        gu_dep = ffn_gate_up(j, zeros)
        y = ffn_down(j, zeros)
        o_e = q_part(xn_e, p, lead=True)
        o_o = q_part(xn_o, p, [(gu_dep, GU_TILE * LANES, 0)])
        o_part(o_e, xn_e, p, 2 * p, s_out, False)
        o_part(o_o, xn_o, p, 2 * p + 1, s_out, True, y[:, D - LANES:])
        return carry

    lax.fori_loop(0, NP, phase_b, 0)

    hot = out_v.at[pl.ds(2 * hot_pair, 2)]
    pltpu.make_async_copy(hot, hot, sem.at[SEM_O]).wait()
    rows16 = pl.ds(row16, 16)
    yrow = _round_bf16(jnp.sum(y_acc[...], axis=0, keepdims=True))
    upd = jnp.where(sel16, yrow * jnp.concatenate([gate_v[...]] * NG, axis=1), 0.0)
    out_v[blk, rows16, :] = (out_v[blk, rows16, :].astype(F32) + upd).astype(BF16)
    patch = pltpu.make_async_copy(
        out_v.at[blk, rows16, :],
        out_hbm.at[0, pl.ds(pl.multiple_of(blk * TB + row16, 16), 16), :], sem.at[SEM_O])
    patch.start()
    pltpu.make_async_copy(out_v.at[pl.ds(2, NB - 2)], out_v.at[pl.ds(2, NB - 2)],
                          sem.at[SEM_O + 1]).wait()
    patch.wait()


@jax.jit
def pallas_parallel_sum__linear_attn_block__moe_arch_mod__prompt_kernel(
    A_x: jax.Array,
    A_wqkv: jax.Array,
    A_wo: jax.Array,
    B_x: jax.Array,
    B_w_r: jax.Array,
    B_w_gate: jax.Array,
    B_w_up: jax.Array,
    B_w_down: jax.Array,
):
    del B_x
    assert A_x.shape == (1, S, D) and B_w_gate.shape == (D, F)
    any_spec = pl.BlockSpec(memory_space=pl.ANY)
    scratch = [
        pltpu.VMEM((NB, TB, D), BF16),
        pltpu.VMEM((NP, TB, D), BF16),
        pltpu.VMEM((NP, TB, D), BF16),
        pltpu.VMEM((NG, D, LANES), BF16),
        pltpu.VMEM((D, D + LANES), BF16),
        pltpu.VMEM((D, D), BF16),
        pltpu.VMEM((D, D), BF16),
        pltpu.VMEM((NP, D, D), BF16),
        pltpu.VMEM((NP, D, D), BF16),
        pltpu.VMEM((NP, D, D), BF16),
        pltpu.VMEM((2, D, 4 * LANES), F32),
        pltpu.VMEM((2, D, 4 * LANES), F32),
        pltpu.VMEM((D, D), F32),
        pltpu.VMEM((D // 2, D), U32),
        pltpu.VMEM((D // 2, D), U32),
        pltpu.VMEM((NB, TB, D), BF16),
        pltpu.VMEM((D // 2, LANES), U32),
        pltpu.VMEM((8, D), F32),
        pltpu.VMEM((8, D), F32),
        pltpu.VMEM((8, D), F32),
        pltpu.VMEM((8, D), F32),
        pltpu.VMEM((16, LANES), F32),
        pltpu.VMEM((2, 8, 1), F32),
        pltpu.VMEM((8, 1), F32),
        pltpu.VMEM((D,), BF16),
        pltpu.SemaphoreType.DMA((N_SEMS,)),
    ]
    return pl.pallas_call(
        _kernel,
        out_shape=jax.ShapeDtypeStruct((1, S, D), BF16),
        in_specs=[any_spec] * 7,
        out_specs=any_spec,
        scratch_shapes=scratch,
        compiler_params=pltpu.CompilerParams(vmem_limit_bytes=100 * 1024 * 1024,
                                             disable_semaphore_checks=True, disable_bounds_checks=True),
    )(A_x, A_wqkv, A_wo, B_w_r, B_w_gate, B_w_up, B_w_down)
```

```python
import jax
import jax.numpy as jnp
from jax import lax
import jax.experimental.pallas as pl
import jax.experimental.pallas.tpu as pltpu

F32 = jnp.float32
BF16 = jnp.bfloat16
U32 = jnp.uint32

S = 2048
D = 1024
F = 3584
DH = 32
TB = 256
NB = S // TB
NP = NB // 2
FC = F // NP
LANES = 128
NG = D // LANES
HG = LANES // DH
KC = 256
NKC = D // KC
WK_SPLITS = (0, 128, 512, 1024)
WQ_PER = 3
DELAY = 8
GU_TILE = 2
TAIL = ((0, 128), (128, 128))
SEM_A = 5
SEM_W = SEM_A + NP - 1
SEM_F = SEM_W + 1
SEM_O = SEM_F + NP
N_SEMS = SEM_O + 2


def _round_bf16(v):
    return v.astype(BF16).astype(F32)


def _phi(t):
    return jnp.where(t > 0, t + 1.0, jnp.exp(t)) + 1e-6


def _dot(a, b):
    return jnp.dot(a, b, preferred_element_type=F32)


def _dot_tn(a, b):
    return lax.dot_general(a, b, (((0,), (0,)), ((), ())), preferred_element_type=F32)


def _dot_nt(a, b):
    return lax.dot_general(a, b, (((1,), (1,)), ((), ())), preferred_element_type=F32)


def _after(v, dep, other=0.0):
    if dep is None:
        return v
    return jnp.where(dep > jnp.inf, other, v)


def _tie(w, dep, r0=0, c0=0):
    if dep is None:
        return w
    dep = jnp.broadcast_to(dep, (8, LANES))
    head = pltpu.bitcast(w[r0:r0 + 16, c0:c0 + LANES], U32) | (dep > jnp.inf).astype(U32)
    row = [pltpu.bitcast(head, BF16)]
    if c0:
        row = [w[r0:r0 + 16, :c0]] + row
    if c0 + LANES < w.shape[1]:
        row = row + [w[r0:r0 + 16, c0 + LANES:]]
    head = row[0] if len(row) == 1 else jnp.concatenate(row, axis=1)
    parts = ([w[:r0]] if r0 else []) + [head, w[r0 + 16:]]
    return jnp.concatenate(parts, axis=0)


def _ties(w, ties):
    for dep, r0, c0 in ties:
        w = _tie(w, dep, r0, c0)
    return w


def _shuffle_rows(w):
    sub = lax.broadcasted_iota(jnp.int32, (8, w.shape[1]), 0)
    v = [w[(a % 4) * 16 + (a // 4) * 8:(a % 4) * 16 + (a // 4) * 8 + 8] for a in range(8)]
    for d in (4, 2, 1):
        low = (sub & d) == 0
        nv = list(v)
        for a in range(8):
            if a & d == 0:
                nv[a] = jnp.where(low, v[a], pltpu.roll(v[a + d], d, 0))
                nv[a + d] = jnp.where(low, pltpu.roll(v[a], 8 - d, 0), v[a + d])
        v = nv
    return v


def _delay(v, n):
    for _ in range(n):
        v = pl.reciprocal(v, approx=True)
    return v


def _col_bcast(row):
    tiles = [jnp.broadcast_to(row[:, t * LANES:(t + 1) * LANES], (LANES, LANES)).T
             for t in range(row.shape[1] // LANES)]
    return jnp.concatenate(tiles, axis=0)


def _kernel(x_hbm, wqkv_hbm, wo_hbm, wr_hbm, wg_hbm, wu_hbm, wd_hbm, out_hbm,
            x_v, xn_e, xn_o, wq_v, wk_v, wv_v, wo_v, wg_v, wu_v, wd_v, xcol_v, hcol_v,
            g_acc, m_v, wqt_v, out_v, wq0_v, wr_f, z_acc, zp_v, y_acc, gate_v, best_v, junk_v, wr_v,
            sem):
    def x_copy(b, s_):
        return pltpu.make_async_copy(x_hbm.at[0, pl.ds(b * TB, TB), :], x_v.at[b], sem.at[s_])

    def x0_copy(h):
        rows = pl.ds(h * (TB // 2), TB // 2)
        return pltpu.make_async_copy(x_hbm.at[0, rows, :], x_v.at[0, rows, :], sem.at[h])

    def wk_copy(i):
        lo, hi = WK_SPLITS[i], WK_SPLITS[i + 1]
        return pltpu.make_async_copy(wqkv_hbm.at[:, pl.ds(D + lo, hi - lo)],
                                     wk_v.at[:, pl.ds(lo, hi - lo)], sem.at[2 + i])

    def wq_copy(g, s_):
        cols = pl.ds(pl.multiple_of(g * LANES, LANES), LANES)
        return pltpu.make_async_copy(wqkv_hbm.at[:, cols], wq_v.at[g], sem.at[s_])

    wr_copy = pltpu.make_async_copy(wr_hbm, wr_v, sem.at[2])
    wv_copy = pltpu.make_async_copy(wqkv_hbm.at[:, pl.ds(2 * D, D)], wv_v, sem.at[SEM_W])
    wo_copy = pltpu.make_async_copy(wo_hbm, wo_v, sem.at[SEM_W])

    def ffn_copies(c, s_):
        span = pl.ds(pl.multiple_of(c * FC, LANES), FC)
        return (
            pltpu.make_async_copy(wg_hbm.at[:, span], wg_v.at[c, :, pl.ds(0, FC)], sem.at[s_]),
            pltpu.make_async_copy(wu_hbm.at[:, span], wu_v.at[c, :, pl.ds(0, FC)], sem.at[s_]),
            pltpu.make_async_copy(wd_hbm.at[span, :], wd_v.at[c, pl.ds(0, FC), :], sem.at[s_]),
        )

    x0_copy(0).start()
    x0_copy(1).start()
    wr_copy.start()
    for i in range(len(WK_SPLITS) - 1):
        wk_copy(i).start()
    x_copy(1, 4).start()
    for j in range(NP - 1):
        x_copy(2 * j + 2, SEM_A + j).start()
        x_copy(2 * j + 3, SEM_A + j).start()
        for g in range(WQ_PER * j, min(WQ_PER * (j + 1), NG)):
            wq_copy(g, SEM_A + j).start()
    wv_copy.start()
    wo_copy.start()
    for c in range(NP):
        for cp in ffn_copies(c, SEM_F + c):
            cp.start()

    y_acc[...] = jnp.zeros_like(y_acc)
    sub8 = lax.broadcasted_iota(jnp.int32, (8, 1), 0).astype(F32)

    def normalise(b, dst_ref, j, r0, nr, dep=None):
        rs = pl.ds(r0, nr)
        mean = jnp.mean(x_v[b, rs, :].astype(F32), axis=-1, keepdims=True)
        mean_b = _after(_round_bf16(mean), dep)
        junk_v[...] = mean[:8]
        c = x_v[b, rs, :].astype(F32) - mean
        var = jnp.mean(c * c, axis=-1, keepdims=True)
        junk_v[...] = var[:8]
        std = _round_bf16(jnp.sqrt(_round_bf16(_round_bf16(var) + 1e-5)))
        d = _round_bf16(x_v[b, rs, :].astype(F32) - mean_b)
        xn = (d * (1.0 / std)).astype(BF16)
        dst_ref[j, rs, :] = xn
        return xn

    def score(xn, row0, best, dep=None):
        nr = xn.shape[0]
        wr = wr_f[...]
        if dep is not None:
            wr = jnp.concatenate([_after(wr[:, :LANES], dep[:8]), wr[:, LANES:]], axis=1)
        if nr > 8:
            wr = jnp.concatenate([wr] * (nr // 8), axis=0)
        r = jnp.sum(xn.astype(F32) * wr, axis=-1, keepdims=True)
        rb = _round_bf16(r)
        bv, bi = best
        for q in range(nr // 8):
            rq = rb[q * 8:(q + 1) * 8]
            better = rq > bv
            bv = jnp.where(better, rq, bv)
            bi = jnp.where(better, sub8 + jnp.asarray(row0 + q * 8).astype(F32), bi)
        return r, (bv, bi)

    def layernorm(b, dst_ref, j, r0, nr, best, dep=None):
        return score(normalise(b, dst_ref, j, r0, nr, dep), b * TB + r0, best)

    def load_best():
        return best_v[0], best_v[1]

    def store_best(best):
        best_v[0] = best[0]
        best_v[1] = best[1]

    def k_unit(src_ref, j, lo, hi, first=False, ties=()):
        pk = _phi(_dot(src_ref[j], _ties(wk_v[:, lo:hi], ties)))
        zs = jnp.sum(pk.reshape(TB // 8, 8, hi - lo), axis=0)
        if first:
            z_acc[:, lo:hi] = zs
        else:
            z_acc[:, lo:hi] += zs
        return pk.astype(BF16)

    def g_unit(src_ref, j, lo, hi, pk, first=False, ties=()):
        g = _dot_tn(pk, _ties(src_ref[j], ties))
        if first:
            g_acc[lo:hi, :] = g
        else:
            g_acc[lo:hi, :] += g

    def wq_prep(g, kk):
        v = _shuffle_rows(pltpu.bitcast(wq_v[g, kk * 256:(kk + 1) * 256, :].T, U32))
        base = pl.multiple_of(g * 8, 8)
        tot = None
        for i in range(8):
            wqt_v[pl.ds(i * 64 + base, 8), kk * 256:(kk + 1) * 256] = v[i]
            tot = v[i] if tot is None else tot | v[i]
        return pltpu.bitcast(tot[:, :LANES] | tot[:, LANES:], F32)

    def mv_chain(acc, w_ref, c, n0, col_ref, z0, k=D):
        cp = 2 * LANES if (n0 // 256) % 4 < 2 else 0
        cz = c + z0

        def step(i, acc):
            rows = pl.ds(pl.multiple_of(i * 8, 8), 8)
            return acc + w_ref[cz, rows, n0:n0 + LANES].astype(F32) * col_ref[z0, rows, cp:cp + LANES]
        return lax.fori_loop(0, k // 8, step, acc, unroll=True)

    def ffn_gate_up(c, zeros):
        dep = None
        zero = jnp.zeros((8, LANES), F32)
        for n0 in range(0, FC, LANES):
            ga = mv_chain(_after(zero, dep, 1.0), wg_v, c, n0, xcol_v, next(zeros))
            ua = mv_chain(_after(zero, ga, 1.0), wu_v, c, n0, xcol_v, next(zeros))
            dep = ua
            gg = _round_bf16(jnp.sum(ga, axis=0, keepdims=True))
            uu = _round_bf16(jnp.sum(ua, axis=0, keepdims=True))
            h = _round_bf16(_round_bf16(gg * jax.nn.sigmoid(gg)) * uu)
            hc = _col_bcast(h)
            hcol_v[0, n0:n0 + LANES, :LANES] = hc
            hcol_v[0, n0:n0 + LANES, 2 * LANES:3 * LANES] = hc
        return dep

    def ffn_down(c, zeros):
        dep = None
        accs = []
        for n0 in range(0, D, LANES):
            dep = mv_chain(_after(y_acc[:, n0:n0 + LANES], dep), wd_v, c, n0, hcol_v, next(zeros), FC)
            y_acc[:, n0:n0 + LANES] = dep
            accs.append(dep)
        return jnp.concatenate(accs, axis=1)

    def first_half():
        x0_copy(0).wait()
        normalise(0, xn_e, 0, 0, TB // 2)
        x0_copy(1).wait()
        normalise(0, xn_e, 0, TB // 2, TB // 2)

        wr_copy.wait()
        wk_copy(0).wait()
        wr_f[...] = jnp.broadcast_to(wr_v[...].astype(F32).reshape(1, D), (8, D))
        g_unit(xn_e, 0, 0, 128, k_unit(xn_e, 0, 0, 128, True), True)
        wk_copy(1).wait()
        best = (jnp.full((8, 1), -jnp.inf, F32), sub8)
        dep = None
        for r0 in range(0, TB, 16):
            dep, best = score(xn_e[0, r0:r0 + 16, :], r0, best, dep)
        pks = [k_unit(xn_e, 0, lo, lo + 128, True) for lo in (128, 256, 384)]
        for lo, pk in zip((128, 256, 384), pks):
            g_unit(xn_e, 0, lo, lo + 128, pk, True)
        wk_copy(2).wait()
        x_copy(1, 4).wait()
        dep = None
        for r0 in range(0, TB, 16):
            dep, best = layernorm(1, xn_o, 0, r0, 16, best, dep)
        store_best(best)
        pks = [k_unit(xn_e, 0, lo, lo + KC, True) for lo in (512, 768)]
        g_unit(xn_e, 0, 512, 768, pks[0], True)
        g_unit(xn_e, 0, 768, 896, pks[1][:, :128], True)
        g_unit(xn_e, 0, 896, 1024, pks[1][:, 128:], True, [(dep[:8], 0, 256)])

        def phase_a(j, carry):
            x_copy(2 * j + 2, SEM_A + j).wait()
            x_copy(2 * j + 3, SEM_A + j).wait()
            wq_copy(WQ_PER * j, SEM_A + j).wait()
            wq_copy(WQ_PER * j + 1, SEM_A + j).wait()

            @pl.when(WQ_PER * j + 2 < NG)
            def _():
                wq_copy(WQ_PER * j + 2, SEM_A + j).wait()

            preps = [(jnp.minimum(WQ_PER * j + i, NG - 1), kk) for i in range(WQ_PER) for kk in range(4)]
            k_slots = {(0, 0): [(0, 128), (512, 128)], (0, 1): [(0, 0), (512, 0), (0, 128), (512, 128)],
                       (1, 1): [(0, 0), (512, 0), (0, 128)]}
            g_slots = {(0, 3): [(0, 256), (0, 512), (0, 768)]}

            def mk_ties(slots):
                return [(wq_prep(*preps.pop(0)), r0, c0) for r0, c0 in slots]

            LR = TB // NKC
            prev = None
            dep = None
            best = load_best()
            for half in range(2):
                src, js = (xn_o, j) if half == 0 else (xn_e, j + 1)
                dst, b = (xn_e, 2 * j + 2) if half == 0 else (xn_o, 2 * j + 3)
                for c in range(NKC):
                    pk = k_unit(src, js, c * KC, (c + 1) * KC, ties=mk_ties(k_slots.get((half, c), [])))
                    if prev is not None:
                        g_unit(*prev[1:], ties=mk_ties(g_slots.get(prev[0], [])))
                    prev = ((half, c), src, js, c * KC, (c + 1) * KC, pk)
                    for r0 in range(c * LR, (c + 1) * LR, 8):
                        dep, best = layernorm(b, dst, j + 1, r0, 8, best, dep)
            g_unit(*prev[1:])
            assert not preps
            store_best(best)
            return carry

        lax.fori_loop(0, NP - 1, phase_a, 0)


    def second_half():
        wv_copy.wait()
        wo_copy.wait()

        bv, bi = load_best()
        r_max = jnp.max(bv, axis=0, keepdims=True)
        idx_f = jnp.min(jnp.where(bv == r_max, bi, float(S - 1)))
        idx = jnp.clip(idx_f.astype(jnp.int32), 0, S - 1)
        blk = idx // TB
        hot_pair = blk // 2
        row16 = pl.multiple_of(((idx % TB) // 16) * 16, 16)
        gate_v[...] = jnp.broadcast_to(_round_bf16(jax.nn.sigmoid(r_max)), (16, LANES))
        row_id16 = lax.broadcasted_iota(jnp.int32, (16, D), 0)
        sel16 = row_id16 == idx % 16
        xs = jnp.where(blk % 2 == 0, xn_e[hot_pair, pl.ds(row16, 16), :].astype(F32),
                       xn_o[hot_pair, pl.ds(row16, 16), :].astype(F32))
        xc = _col_bcast(jnp.sum(jnp.where(sel16, xs, 0.0), axis=0, keepdims=True))
        xcol_v[0, :, :LANES] = xc
        xcol_v[0, :, 2 * LANES:3 * LANES] = xc

        rr = lax.broadcasted_iota(jnp.int32, (LANES, LANES), 0) // DH
        cc = lax.broadcasted_iota(jnp.int32, (LANES, LANES), 1) // DH
        same_head = rr == cc

        def g_final(c, pk, dep=None):
            return (g_acc[c * KC:(c + 1) * KC, :] + _dot_tn(pk, _tie(xn_o[NP - 1], dep))).astype(BF16)

        def kv_unit(c, gf):
            out = []
            for gg in range(KC // LANES):
                g = c * (KC // LANES) + gg
                kv = _dot(gf[gg * LANES:(gg + 1) * LANES, :], wv_v[:, g * LANES:(g + 1) * LANES])
                kv = pltpu.bitcast(jnp.where(same_head, kv, 0.0).astype(BF16), U32)
                out.append(pltpu.bitcast(jnp.concatenate(_shuffle_rows(kv), axis=0), BF16))
            return out

        def m_unit(c, kvs, dep=None):
            for gg in range(KC // LANES):
                g = c * (KC // LANES) + gg
                m = _dot(kvs[gg], _tie(wo_v[g * LANES:(g + 1) * LANES, :], dep))
                dep = None
                w = pltpu.bitcast(m.astype(BF16), U32)
                for i in range(8):
                    m_v[i * 64 + g * 8:i * 64 + (g + 1) * 8, :] = w[i * 8:(i + 1) * 8, :]

        def z_prep():
            zc = pltpu.bitcast(_col_bcast(jnp.sum(z_acc[...], axis=0, keepdims=True)).astype(BF16), U32)
            vs = [_shuffle_rows(zc[g * 64:(g + 1) * 64, :]) for g in range(NG)]
            tot = None
            for i in range(NG):
                zt = pltpu.bitcast(jnp.concatenate([vs[g][i] for g in range(NG)], axis=0), BF16)
                zp = zt.astype(F32).T[:8, :]
                zp_v[:, i * LANES:(i + 1) * LANES] = zp
                tot = zp if tot is None else tot + zp
            return tot

        def ku(c):
            return k_unit(xn_o, NP - 1, c * KC, (c + 1) * KC)

        wq0_v[...] = pltpu.bitcast(pltpu.bitcast(wqt_v[:LANES // 2, :], BF16).T, U32)
        pk0 = ku(0)
        pk1 = ku(1)
        gf0 = g_final(0, pk0)
        pk2 = ku(2)
        gf1 = g_final(1, pk1)
        kv0 = kv_unit(0, gf0)
        pk3 = ku(3)
        gf2 = g_final(2, pk2)
        kv1 = kv_unit(1, gf1)
        m_unit(0, kv0, xc[D - 8:])
        gf3 = g_final(3, pk3)
        kv2 = kv_unit(2, gf2)
        m_unit(1, kv1)
        kv3 = kv_unit(3, gf3)
        m_unit(2, kv2, z_prep())
        m_unit(3, kv3)

        lane = lax.broadcasted_iota(jnp.int32, (8, LANES), 1)
        bit0 = lane % 2 == 0
        bit3 = (lane // 8) % 2 == 0

        def q_part(src_ref, p, ties=(), lead=False):
            wqt = _ties(pltpu.bitcast(wqt_v[...], BF16), ties)
            if lead:
                xn = src_ref[p]
                q0 = _dot(xn, pltpu.bitcast(wq0_v[...], BF16))
                q = jnp.concatenate([q0, _dot_nt(xn, wqt[LANES:])], axis=1)
            else:
                q = _dot_nt(src_ref[p], wqt)
            rows_ = []
            dep = None
            for g in range(TB // 8):
                pq = _phi(q[g * 8:(g + 1) * 8, :])
                t = pq * zp_v[...]
                s_ = t[:, :LANES]
                for n in range(1, NG):
                    s_ = s_ + t[:, n * LANES:(n + 1) * LANES]
                s_ = s_ + jnp.where(bit3, pltpu.roll(s_, LANES - 8, 1), pltpu.roll(s_, 8, 1))
                s_ = s_ + jnp.where(bit0, pltpu.roll(s_, LANES - 1, 1), pltpu.roll(s_, 1, 1))
                rinv = _after(pl.reciprocal(s_ + 1e-6, approx=True), dep)
                rows_.append(pq * jnp.concatenate([rinv] * NG, axis=1))
                dep = _delay(rinv, DELAY)
            return jnp.concatenate(rows_, axis=0).astype(BF16)

        def o_part(o, src_ref, p, b, s_out, last, dep=None):
            spans = [(0, 256), (256, 512), (512, 768), (768, 896), (896, D)] if last else \
                [(c * KC, (c + 1) * KC) for c in range(NKC)]
            for lo, hi in spans:
                m = pltpu.bitcast(m_v[:, lo:hi], BF16)
                a = _dot(o, _tie(m, dep if lo == 768 else None))
                for r0, nr in (TAIL if last and hi == D else ((0, TB),)):
                    rs = slice(r0, r0 + nr)
                    out_v[b, rs, lo:hi] = (x_v[b, rs, lo:hi].astype(F32) + a[rs]
                                           + src_ref[p, rs, lo:hi].astype(F32)).astype(BF16)
                    if last or hi == D:
                        cols = pl.ds(lo, hi - lo) if last else pl.ds(0, D)
                        pltpu.make_async_copy(out_v.at[b, pl.ds(r0, nr), cols],
                                              out_hbm.at[0, pl.ds(b * TB + r0, nr), cols],
                                              sem.at[s_out]).start()

        def phase_b(j, carry):
            for cp in ffn_copies(j, SEM_F + j):
                cp.wait()
            p = jnp.where(j == 0, hot_pair, jnp.where(j == hot_pair, 0, j))
            s_out = jnp.where(j == 0, SEM_O, SEM_O + 1)
            zeros = (lax.shift_right_logical(idx + j + k, 13) for k in range(64))
            gu_dep = ffn_gate_up(j, zeros)
            y = ffn_down(j, zeros)
            o_e = q_part(xn_e, p, lead=True)
            o_o = q_part(xn_o, p, [(gu_dep, GU_TILE * LANES, 0)])
            o_part(o_e, xn_e, p, 2 * p, s_out, False)
            o_part(o_o, xn_o, p, 2 * p + 1, s_out, True, y[:, D - LANES:])
            return carry

        lax.fori_loop(0, NP, phase_b, 0)

        hot = out_v.at[pl.ds(2 * hot_pair, 2)]
        pltpu.make_async_copy(hot, hot, sem.at[SEM_O]).wait()
        rows16 = pl.ds(row16, 16)
        yrow = _round_bf16(jnp.sum(y_acc[...], axis=0, keepdims=True))
        upd = jnp.where(sel16, yrow * jnp.concatenate([gate_v[...]] * NG, axis=1), 0.0)
        out_v[blk, rows16, :] = (out_v[blk, rows16, :].astype(F32) + upd).astype(BF16)
        patch = pltpu.make_async_copy(
            out_v.at[blk, rows16, :],
            out_hbm.at[0, pl.ds(pl.multiple_of(blk * TB + row16, 16), 16), :], sem.at[SEM_O])
        patch.start()
        pltpu.make_async_copy(out_v.at[pl.ds(2, NB - 2)], out_v.at[pl.ds(2, NB - 2)],
                              sem.at[SEM_O + 1]).wait()
        patch.wait()

    def outer(i, carry):
        pl.when(i == 0)(first_half)
        pl.when(i == 1)(second_half)
        return carry

    lax.fori_loop(0, 2, outer, 0)


@jax.jit
def pallas_parallel_sum__linear_attn_block__moe_arch_mod__prompt_kernel(
    A_x: jax.Array,
    A_wqkv: jax.Array,
    A_wo: jax.Array,
    B_x: jax.Array,
    B_w_r: jax.Array,
    B_w_gate: jax.Array,
    B_w_up: jax.Array,
    B_w_down: jax.Array,
):
    del B_x
    assert A_x.shape == (1, S, D) and B_w_gate.shape == (D, F)
    any_spec = pl.BlockSpec(memory_space=pl.ANY)
    scratch = [
        pltpu.VMEM((NB, TB, D), BF16),
        pltpu.VMEM((NP, TB, D), BF16),
        pltpu.VMEM((NP, TB, D), BF16),
        pltpu.VMEM((NG, D, LANES), BF16),
        pltpu.VMEM((D, D + LANES), BF16),
        pltpu.VMEM((D, D), BF16),
        pltpu.VMEM((D, D), BF16),
        pltpu.VMEM((NP, D, D), BF16),
        pltpu.VMEM((NP, D, D), BF16),
        pltpu.VMEM((NP, D, D), BF16),
        pltpu.VMEM((2, D, 4 * LANES), F32),
        pltpu.VMEM((2, D, 4 * LANES), F32),
        pltpu.VMEM((D, D), F32),
        pltpu.VMEM((D // 2, D), U32),
        pltpu.VMEM((D // 2, D), U32),
        pltpu.VMEM((NB, TB, D), BF16),
        pltpu.VMEM((D // 2, LANES), U32),
        pltpu.VMEM((8, D), F32),
        pltpu.VMEM((8, D), F32),
        pltpu.VMEM((8, D), F32),
        pltpu.VMEM((8, D), F32),
        pltpu.VMEM((16, LANES), F32),
        pltpu.VMEM((2, 8, 1), F32),
        pltpu.VMEM((8, 1), F32),
        pltpu.VMEM((D,), BF16),
        pltpu.SemaphoreType.DMA((N_SEMS,)),
    ]
    return pl.pallas_call(
        _kernel,
        out_shape=jax.ShapeDtypeStruct((1, S, D), BF16),
        in_specs=[any_spec] * 7,
        out_specs=any_spec,
        scratch_shapes=scratch,
        compiler_params=pltpu.CompilerParams(vmem_limit_bytes=100 * 1024 * 1024,
                                             disable_semaphore_checks=True, disable_bounds_checks=True),
    )(A_x, A_wqkv, A_wo, B_w_r, B_w_gate, B_w_up, B_w_down)
```

```python
import jax
import jax.numpy as jnp
from jax import lax
import jax.experimental.pallas as pl
import jax.experimental.pallas.tpu as pltpu

F32 = jnp.float32
BF16 = jnp.bfloat16
U32 = jnp.uint32

S = 2048
D = 1024
F = 3584
DH = 32
TB = 256
NB = S // TB
NP = NB // 2
FC = F // NP
LANES = 128
NG = D // LANES
HG = LANES // DH
KC = 256
NKC = D // KC
K_SPLITS = (0, 128, 256, 512, 768, 1024)
X_SPLITS = (0, 128, 256, 512, 1024)
KF = K_SPLITS[-2]
LN0_PACE = 4
PHI_PACE = 1
LEAD = 4
WQ_PER = 3
DELAY = 8
GU_TILE = 2
TAIL = ((0, 128), (128, 128))
SEM_A = 5
SEM_W = SEM_A + NP - 1
SEM_F = SEM_W + 1
SEM_O = SEM_F + NP
N_SEMS = SEM_O + 2


def _round_bf16(v):
    return v.astype(BF16).astype(F32)


def _phi(t):
    return jnp.where(t > 0, t + 1.0, jnp.exp(t)) + 1e-6


def _dot(a, b):
    return jnp.dot(a, b, preferred_element_type=F32)


def _dot_tn(a, b):
    return lax.dot_general(a, b, (((0,), (0,)), ((), ())), preferred_element_type=F32)


def _dot_nt(a, b):
    return lax.dot_general(a, b, (((1,), (1,)), ((), ())), preferred_element_type=F32)


def _after(v, dep, other=0.0):
    if dep is None:
        return v
    return jnp.where(dep > jnp.inf, other, v)


def _tie(w, dep, r0=0, c0=0):
    if dep is None:
        return w
    dep = jnp.broadcast_to(dep, (8, LANES))
    head = pltpu.bitcast(w[r0:r0 + 16, c0:c0 + LANES], U32) | (dep > jnp.inf).astype(U32)
    row = [pltpu.bitcast(head, BF16)]
    if c0:
        row = [w[r0:r0 + 16, :c0]] + row
    if c0 + LANES < w.shape[1]:
        row = row + [w[r0:r0 + 16, c0 + LANES:]]
    head = row[0] if len(row) == 1 else jnp.concatenate(row, axis=1)
    parts = ([w[:r0]] if r0 else []) + [head, w[r0 + 16:]]
    return jnp.concatenate(parts, axis=0)


def _ties(w, ties):
    for dep, r0, c0 in ties:
        w = _tie(w, dep, r0, c0)
    return w


def _shuffle_rows(w):
    sub = lax.broadcasted_iota(jnp.int32, (8, w.shape[1]), 0)
    v = [w[(a % 4) * 16 + (a // 4) * 8:(a % 4) * 16 + (a // 4) * 8 + 8] for a in range(8)]
    for d in (4, 2, 1):
        low = (sub & d) == 0
        nv = list(v)
        for a in range(8):
            if a & d == 0:
                nv[a] = jnp.where(low, v[a], pltpu.roll(v[a + d], d, 0))
                nv[a + d] = jnp.where(low, pltpu.roll(v[a], 8 - d, 0), v[a + d])
        v = nv
    return v


def _delay(v, n):
    for _ in range(n):
        v = pl.reciprocal(v, approx=True)
    return v


def _col_bcast(row):
    tiles = [jnp.broadcast_to(row[:, t * LANES:(t + 1) * LANES], (LANES, LANES)).T
             for t in range(row.shape[1] // LANES)]
    return jnp.concatenate(tiles, axis=0)


def _kernel(x_hbm, wqkv_hbm, wo_hbm, wr_hbm, wg_hbm, wu_hbm, wd_hbm, out_hbm,
            x_v, xn_e, xn_o, wq_v, wk_v, wv_v, wo_v, wg_v, wu_v, wd_v, xcol_v, hcol_v,
            g_acc, m_v, wqt_v, out_v, wq0_v, kraw_v, st_v, cs_v, wr_f, z_acc, zp_v, y_acc, gate_v, best_v, junk_v, wr_v,
            sem):
    def x_copy(b, s_):
        return pltpu.make_async_copy(x_hbm.at[0, pl.ds(b * TB, TB), :], x_v.at[b], sem.at[s_])

    def xs_copies(i):
        cols = pl.ds(X_SPLITS[i], X_SPLITS[i + 1] - X_SPLITS[i])
        return [pltpu.make_async_copy(x_hbm.at[0, pl.ds(b * TB, TB), cols], x_v.at[b, :, cols],
                                      sem.at[i]) for b in (0, NB - 1)]

    def wk_copy(i):
        rows = pl.ds(K_SPLITS[i], K_SPLITS[i + 1] - K_SPLITS[i])
        return pltpu.make_async_copy(wqkv_hbm.at[rows, pl.ds(D, D)], wk_v.at[rows, pl.ds(0, D)],
                                     sem.at[i])

    def wq_copy(g, s_):
        cols = pl.ds(pl.multiple_of(g * LANES, LANES), LANES)
        return pltpu.make_async_copy(wqkv_hbm.at[:, cols], wq_v.at[g], sem.at[s_])

    wr_copy = pltpu.make_async_copy(wr_hbm, wr_v, sem.at[3])
    wv_copy = pltpu.make_async_copy(wqkv_hbm.at[:, pl.ds(2 * D, D)], wv_v, sem.at[SEM_W])
    wo_copy = pltpu.make_async_copy(wo_hbm, wo_v, sem.at[SEM_W])

    def ffn_copies(c, s_):
        span = pl.ds(pl.multiple_of(c * FC, LANES), FC)
        return (
            pltpu.make_async_copy(wg_hbm.at[:, span], wg_v.at[c, :, pl.ds(0, FC)], sem.at[s_]),
            pltpu.make_async_copy(wu_hbm.at[:, span], wu_v.at[c, :, pl.ds(0, FC)], sem.at[s_]),
            pltpu.make_async_copy(wd_hbm.at[span, :], wd_v.at[c, pl.ds(0, FC), :], sem.at[s_]),
        )

    for i in range(len(K_SPLITS) - 1):
        if i < len(X_SPLITS) - 1:
            for cp in xs_copies(i):
                cp.start()
        if i == 3:
            wr_copy.start()
        wk_copy(i).start()
    x_copy(1, 4).start()
    for j in range(NP - 1):
        x_copy(2 * j + 2, SEM_A + j).start()
        if 2 * j + 3 < NB - 1:
            x_copy(2 * j + 3, SEM_A + j).start()
        for g in range(WQ_PER * j, min(WQ_PER * (j + 1), NG)):
            wq_copy(g, SEM_A + j).start()
    wv_copy.start()
    wo_copy.start()
    for c in range(NP):
        for cp in ffn_copies(c, SEM_F + c):
            cp.start()

    y_acc[...] = jnp.zeros_like(y_acc)
    sub8 = lax.broadcasted_iota(jnp.int32, (8, 1), 0).astype(F32)

    def normalise(b, dst_ref, j, r0, nr, dep=None, keep=None):
        rs = pl.ds(r0, nr)
        mean = jnp.mean(x_v[b, rs, :].astype(F32), axis=-1, keepdims=True)
        mean_b = jnp.broadcast_to(_round_bf16(mean), (nr, LANES))
        junk_v[...] = mean[:8]
        c = x_v[b, rs, :].astype(F32) - mean
        var = jnp.mean(c * c, axis=-1, keepdims=True)
        junk_v[...] = var[:8]
        rstd = 1.0 / _round_bf16(jnp.sqrt(_round_bf16(_round_bf16(var) + 1e-5)))
        if keep is not None:
            st_v[keep, 0, rs, :] = mean_b
            st_v[keep, 1, rs, :] = jnp.broadcast_to(rstd, (nr, LANES))
        mean_b = jnp.concatenate([_after(mean_b, dep)] * NG, axis=1)
        xn_f = _round_bf16(x_v[b, rs, :].astype(F32) - mean_b) * rstd
        xn = xn_f.astype(BF16)
        dst_ref[j, rs, :] = xn
        return xn, xn_f

    def score(xn, row0, best, dep=None):
        nr = xn.shape[0]
        wr = wr_f[...]
        if dep is not None:
            wr = jnp.concatenate([_after(wr[:, :LANES], dep[:8]), wr[:, LANES:]], axis=1)
        if nr > 8:
            wr = jnp.concatenate([wr] * (nr // 8), axis=0)
        r = jnp.sum(xn.astype(F32) * wr, axis=-1, keepdims=True)
        rb = _round_bf16(r)
        bv, bi = best
        for q in range(nr // 8):
            rq = rb[q * 8:(q + 1) * 8]
            better = rq > bv
            bv = jnp.where(better, rq, bv)
            bi = jnp.where(better, sub8 + jnp.asarray(row0 + q * 8).astype(F32), bi)
        return r, (bv, bi)

    def layernorm(b, dst_ref, j, r0, nr, best, dep=None, keep=None):
        return score(normalise(b, dst_ref, j, r0, nr, dep, keep)[0], b * TB + r0, best)

    def load_best():
        return best_v[0], best_v[1]

    def store_best(best):
        best_v[0] = best[0]
        best_v[1] = best[1]

    def k_unit(src_ref, j, lo, hi, first=False, ties=()):
        pk = _phi(_dot(src_ref[j], _ties(wk_v[:, lo:hi], ties)))
        zs = jnp.sum(pk.reshape(TB // 8, 8, hi - lo), axis=0)
        if first:
            z_acc[:, lo:hi] = zs
        else:
            z_acc[:, lo:hi] += zs
        return pk.astype(BF16)

    def raw_slice(i):
        lo, hi = K_SPLITS[i], K_SPLITS[i + 1]
        xs = jnp.concatenate([x_v[0, :, lo:hi], x_v[NB - 1, :, lo:hi]], axis=0)
        part = _dot(xs, wk_v[lo:hi, :D])
        if i == 0:
            kraw_v[...] = part
        else:
            kraw_v[...] += part
        if i == 2:
            cs_v[...] = jnp.sum(wk_v[:hi, :D].astype(F32).reshape(hi // 8, 8, D), axis=0)
        elif i > 2:
            cs_v[...] += jnp.sum(wk_v[lo:hi, :D].astype(F32).reshape((hi - lo) // 8, 8, D), axis=0)

    def raw_last(b, c):
        return _dot(x_v[b, :, KF:], wk_v[KF:, c * KC:(c + 1) * KC])

    def raw_finish(slot, c, part, first, paced):
        cs = slice(c * KC, (c + 1) * KC)
        rows_ = []
        dep = None
        zs = None
        for r0 in range(0, TB, 16):
            mean = st_v[slot, 0, r0:r0 + 16, :]
            rstd = _after(st_v[slot, 1, r0:r0 + 16, :], dep)
            mean = jnp.concatenate([mean] * (KC // LANES), axis=1)
            rstd = jnp.concatenate([rstd] * (KC // LANES), axis=1)
            col = jnp.concatenate([cs_v[:, cs]] * 2, axis=0)
            k = (kraw_v[slot * TB + r0:slot * TB + r0 + 16, cs] + part[r0:r0 + 16] - mean * col) * rstd
            pk = _phi(k)
            z2 = pk[:8] + pk[8:]
            zs = z2 if zs is None else zs + z2
            if paced:
                f = _delay(z2[:, :LANES] + z2[:, LANES:], PHI_PACE)
                dep = jnp.concatenate([f, f], axis=0)
            rows_.append(pk.astype(BF16))
        if first:
            z_acc[:, cs] = zs
        else:
            z_acc[:, cs] += zs
        return jnp.concatenate(rows_, axis=0)

    def g_unit(src_ref, j, lo, hi, pk, first=False, ties=()):
        g = _dot_tn(pk, _ties(src_ref[j], ties))
        if first:
            g_acc[lo:hi, :] = g
        else:
            g_acc[lo:hi, :] += g

    def wq_prep(g, kk):
        v = _shuffle_rows(pltpu.bitcast(wq_v[g, kk * 256:(kk + 1) * 256, :].T, U32))
        base = pl.multiple_of(g * 8, 8)
        tot = None
        for i in range(8):
            wqt_v[pl.ds(i * 64 + base, 8), kk * 256:(kk + 1) * 256] = v[i]
            tot = v[i] if tot is None else tot | v[i]
        return pltpu.bitcast(tot[:, :LANES] | tot[:, LANES:], F32)

    def mv_chain(acc, w_ref, c, n0, col_ref, z0, k=D):
        cp = 2 * LANES if (n0 // 256) % 4 < 2 else 0
        cz = c + z0

        def step(i, acc):
            rows = pl.ds(pl.multiple_of(i * 8, 8), 8)
            return acc + w_ref[cz, rows, n0:n0 + LANES].astype(F32) * col_ref[z0, rows, cp:cp + LANES]
        return lax.fori_loop(0, k // 8, step, acc, unroll=True)

    def ffn_gate_up(c, zeros):
        dep = None
        zero = jnp.zeros((8, LANES), F32)
        for n0 in range(0, FC, LANES):
            ga = mv_chain(_after(zero, dep, 1.0), wg_v, c, n0, xcol_v, next(zeros))
            ua = mv_chain(_after(zero, ga, 1.0), wu_v, c, n0, xcol_v, next(zeros))
            dep = ua
            gg = _round_bf16(jnp.sum(ga, axis=0, keepdims=True))
            uu = _round_bf16(jnp.sum(ua, axis=0, keepdims=True))
            h = _round_bf16(_round_bf16(gg * jax.nn.sigmoid(gg)) * uu)
            hc = _col_bcast(h)
            hcol_v[0, n0:n0 + LANES, :LANES] = hc
            hcol_v[0, n0:n0 + LANES, 2 * LANES:3 * LANES] = hc
        return dep

    def ffn_down(c, zeros):
        dep = None
        accs = []
        for n0 in range(0, D, LANES):
            dep = mv_chain(_after(y_acc[:, n0:n0 + LANES], dep), wd_v, c, n0, hcol_v, next(zeros), FC)
            y_acc[:, n0:n0 + LANES] = dep
            accs.append(dep)
        return jnp.concatenate(accs, axis=1)

    def first_half():
        for i in range(4):
            for cp in xs_copies(i):
                cp.wait()
            if i == 3:
                wr_copy.wait()
            wk_copy(i).wait()
            raw_slice(i)
            if i == 3:
                wr_f[...] = jnp.broadcast_to(wr_v[...].astype(F32).reshape(1, D), (8, D))
                dep = None
                for r0 in range(0, TB, 8):
                    _, xn_f = normalise(0, xn_e, 0, r0, 8, dep, keep=0)
                    dep = _delay(xn_f[:, D - LANES:], LN0_PACE)
        wk_copy(4).wait()
        x_copy(1, 4).wait()
        cs = cs_v[...] + jnp.sum(wk_v[KF:, :D].astype(F32).reshape((D - KF) // 8, 8, D), axis=0)
        cs_v[...] = jnp.broadcast_to(jnp.sum(cs, axis=0, keepdims=True), (8, D))
        best = (jnp.full((8, 1), -jnp.inf, F32), sub8)
        dep = None
        for r0 in range(0, TB, 16):
            dep, best = layernorm(1, xn_o, 0, r0, 16, best, dep)
        store_best(best)
        parts = [raw_last(0, c) for c in range(LEAD)]
        for c in range(NKC):
            g_unit(xn_e, 0, c * KC, (c + 1) * KC, raw_finish(0, c, parts[c], True, False), True,
                   [(dep[:8], 0, 512)] if c == NKC - 1 else [])
            if len(parts) < NKC:
                parts.append(raw_last(0, len(parts)))

        def phase_a(j, carry):
            x_copy(2 * j + 2, SEM_A + j).wait()
            wq_copy(WQ_PER * j, SEM_A + j).wait()
            wq_copy(WQ_PER * j + 1, SEM_A + j).wait()

            @pl.when(j < NP - 2)
            def _():
                x_copy(2 * j + 3, SEM_A + j).wait()
                wq_copy(WQ_PER * j + 2, SEM_A + j).wait()

            preps = [(jnp.minimum(WQ_PER * j + i, NG - 1), kk) for i in range(WQ_PER) for kk in range(4)]
            k_slots = {(0, 0): [(0, 128), (512, 128)], (0, 1): [(0, 0), (512, 0), (0, 128), (512, 128)],
                       (1, 1): [(0, 0), (512, 0), (0, 128)]}
            g_slots = {(0, 3): [(0, 256), (0, 512), (0, 768)]}

            def mk_ties(slots):
                return [(wq_prep(*preps.pop(0)), r0, c0) for r0, c0 in slots]

            LR = TB // NKC
            prev = None
            dep = None
            best = load_best()
            for half in range(2):
                src, js = (xn_o, j) if half == 0 else (xn_e, j + 1)
                dst, b = (xn_e, 2 * j + 2) if half == 0 else (xn_o, 2 * j + 3)
                for c in range(NKC):
                    pk = k_unit(src, js, c * KC, (c + 1) * KC, ties=mk_ties(k_slots.get((half, c), [])))
                    if prev is not None:
                        g_unit(*prev[1:], ties=mk_ties(g_slots.get(prev[0], [])))
                    prev = ((half, c), src, js, c * KC, (c + 1) * KC, pk)
                    for r0 in range(c * LR, (c + 1) * LR, 8):
                        dep, best = layernorm(b, dst, j + 1, r0, 8, best, dep, keep=1 if half else None)
            g_unit(*prev[1:])
            assert not preps
            store_best(best)
            return carry

        lax.fori_loop(0, NP - 1, phase_a, 0)


    def second_half():
        wv_copy.wait()
        wo_copy.wait()

        best0 = (jnp.full((8, 1), -jnp.inf, F32), sub8)
        dep = None
        for r0 in range(0, TB, 16):
            dep, best0 = score(xn_e[0, r0:r0 + 16, :], r0, best0, dep)
        bv, bi = load_best()
        first0 = best0[0] >= bv
        bv = jnp.where(first0, best0[0], bv)
        bi = jnp.where(first0, best0[1], bi)
        r_max = jnp.max(bv, axis=0, keepdims=True)
        idx_f = jnp.min(jnp.where(bv == r_max, bi, float(S - 1)))
        idx = jnp.clip(idx_f.astype(jnp.int32), 0, S - 1)
        blk = idx // TB
        hot_pair = blk // 2
        row16 = pl.multiple_of(((idx % TB) // 16) * 16, 16)
        gate_v[...] = jnp.broadcast_to(_round_bf16(jax.nn.sigmoid(r_max)), (16, LANES))
        row_id16 = lax.broadcasted_iota(jnp.int32, (16, D), 0)
        sel16 = row_id16 == idx % 16
        xs = jnp.where(blk % 2 == 0, xn_e[hot_pair, pl.ds(row16, 16), :].astype(F32),
                       xn_o[hot_pair, pl.ds(row16, 16), :].astype(F32))
        xc = _col_bcast(jnp.sum(jnp.where(sel16, xs, 0.0), axis=0, keepdims=True))
        xcol_v[0, :, :LANES] = xc
        xcol_v[0, :, 2 * LANES:3 * LANES] = xc

        rr = lax.broadcasted_iota(jnp.int32, (LANES, LANES), 0) // DH
        cc = lax.broadcasted_iota(jnp.int32, (LANES, LANES), 1) // DH
        same_head = rr == cc

        def g_final(c, pk, dep=None):
            return (g_acc[c * KC:(c + 1) * KC, :] + _dot_tn(pk, _tie(xn_o[NP - 1], dep))).astype(BF16)

        def kv_unit(c, gf):
            out = []
            for gg in range(KC // LANES):
                g = c * (KC // LANES) + gg
                kv = _dot(gf[gg * LANES:(gg + 1) * LANES, :], wv_v[:, g * LANES:(g + 1) * LANES])
                kv = pltpu.bitcast(jnp.where(same_head, kv, 0.0).astype(BF16), U32)
                out.append(pltpu.bitcast(jnp.concatenate(_shuffle_rows(kv), axis=0), BF16))
            return out

        def m_unit(c, kvs, dep=None):
            for gg in range(KC // LANES):
                g = c * (KC // LANES) + gg
                m = _dot(kvs[gg], _tie(wo_v[g * LANES:(g + 1) * LANES, :], dep))
                dep = None
                w = pltpu.bitcast(m.astype(BF16), U32)
                for i in range(8):
                    m_v[i * 64 + g * 8:i * 64 + (g + 1) * 8, :] = w[i * 8:(i + 1) * 8, :]

        def z_prep():
            zc = pltpu.bitcast(_col_bcast(jnp.sum(z_acc[...], axis=0, keepdims=True)).astype(BF16), U32)
            vs = [_shuffle_rows(zc[g * 64:(g + 1) * 64, :]) for g in range(NG)]
            tot = None
            for i in range(NG):
                zt = pltpu.bitcast(jnp.concatenate([vs[g][i] for g in range(NG)], axis=0), BF16)
                zp = zt.astype(F32).T[:8, :]
                zp_v[:, i * LANES:(i + 1) * LANES] = zp
                tot = zp if tot is None else tot + zp
            return tot

        wq0_v[...] = pltpu.bitcast(pltpu.bitcast(wqt_v[:LANES // 2, :], BF16).T, U32)
        parts = [raw_last(NB - 1, c) for c in range(LEAD)]

        def gf(c):
            g = g_final(c, raw_finish(1, c, parts[c], False, False))
            if len(parts) < NKC:
                parts.append(raw_last(NB - 1, len(parts)))
            return g

        gf0 = gf(0)
        gf1 = gf(1)
        kv0 = kv_unit(0, gf0)
        gf2 = gf(2)
        kv1 = kv_unit(1, gf1)
        m_unit(0, kv0)
        gf3 = gf(3)
        kv2 = kv_unit(2, gf2)
        m_unit(1, kv1, xc[D - 8:])
        kv3 = kv_unit(3, gf3)
        m_unit(2, kv2, z_prep())
        m_unit(3, kv3)

        lane = lax.broadcasted_iota(jnp.int32, (8, LANES), 1)
        bit0 = lane % 2 == 0
        bit3 = (lane // 8) % 2 == 0

        def q_part(src_ref, p, ties=(), lead=False):
            wqt = _ties(pltpu.bitcast(wqt_v[...], BF16), ties)
            if lead:
                xn = src_ref[p]
                q0 = _dot(xn, pltpu.bitcast(wq0_v[...], BF16))
                q = jnp.concatenate([q0, _dot_nt(xn, wqt[LANES:])], axis=1)
            else:
                q = _dot_nt(src_ref[p], wqt)
            rows_ = []
            dep = None
            for g in range(TB // 8):
                pq = _phi(q[g * 8:(g + 1) * 8, :])
                t = pq * zp_v[...]
                s_ = t[:, :LANES]
                for n in range(1, NG):
                    s_ = s_ + t[:, n * LANES:(n + 1) * LANES]
                s_ = s_ + jnp.where(bit3, pltpu.roll(s_, LANES - 8, 1), pltpu.roll(s_, 8, 1))
                s_ = s_ + jnp.where(bit0, pltpu.roll(s_, LANES - 1, 1), pltpu.roll(s_, 1, 1))
                rinv = _after(pl.reciprocal(s_ + 1e-6, approx=True), dep)
                rows_.append(pq * jnp.concatenate([rinv] * NG, axis=1))
                dep = _delay(rinv, DELAY)
            return jnp.concatenate(rows_, axis=0).astype(BF16)

        def o_part(o, src_ref, p, b, s_out, last, dep=None):
            spans = [(0, 256), (256, 512), (512, 768), (768, 896), (896, D)] if last else \
                [(c * KC, (c + 1) * KC) for c in range(NKC)]
            for lo, hi in spans:
                m = pltpu.bitcast(m_v[:, lo:hi], BF16)
                a = _dot(o, _tie(m, dep if lo == 768 else None))
                for r0, nr in (TAIL if last and hi == D else ((0, TB),)):
                    rs = slice(r0, r0 + nr)
                    out_v[b, rs, lo:hi] = (x_v[b, rs, lo:hi].astype(F32) + a[rs]
                                           + src_ref[p, rs, lo:hi].astype(F32)).astype(BF16)
                    if last or hi == D:
                        cols = pl.ds(lo, hi - lo) if last else pl.ds(0, D)
                        pltpu.make_async_copy(out_v.at[b, pl.ds(r0, nr), cols],
                                              out_hbm.at[0, pl.ds(b * TB + r0, nr), cols],
                                              sem.at[s_out]).start()

        def phase_b(j, carry):
            for cp in ffn_copies(j, SEM_F + j):
                cp.wait()
            p = jnp.where(j == 0, hot_pair, jnp.where(j == hot_pair, 0, j))
            s_out = jnp.where(j == 0, SEM_O, SEM_O + 1)
            zeros = (lax.shift_right_logical(idx + j + k, 13) for k in range(64))
            gu_dep = ffn_gate_up(j, zeros)
            y = ffn_down(j, zeros)
            o_e = q_part(xn_e, p, lead=True)
            o_o = q_part(xn_o, p, [(gu_dep, GU_TILE * LANES, 0)])
            o_part(o_e, xn_e, p, 2 * p, s_out, False)
            o_part(o_o, xn_o, p, 2 * p + 1, s_out, True, y[:, D - LANES:])
            return carry

        lax.fori_loop(0, NP, phase_b, 0)

        hot = out_v.at[pl.ds(2 * hot_pair, 2)]
        pltpu.make_async_copy(hot, hot, sem.at[SEM_O]).wait()
        rows16 = pl.ds(row16, 16)
        yrow = _round_bf16(jnp.sum(y_acc[...], axis=0, keepdims=True))
        upd = jnp.where(sel16, yrow * jnp.concatenate([gate_v[...]] * NG, axis=1), 0.0)
        out_v[blk, rows16, :] = (out_v[blk, rows16, :].astype(F32) + upd).astype(BF16)
        patch = pltpu.make_async_copy(
            out_v.at[blk, rows16, :],
            out_hbm.at[0, pl.ds(pl.multiple_of(blk * TB + row16, 16), 16), :], sem.at[SEM_O])
        patch.start()
        pltpu.make_async_copy(out_v.at[pl.ds(2, NB - 2)], out_v.at[pl.ds(2, NB - 2)],
                              sem.at[SEM_O + 1]).wait()
        patch.wait()

    def outer(i, carry):
        pl.when(i == 0)(first_half)
        pl.when(i == 1)(second_half)
        return carry

    lax.fori_loop(0, 2, outer, 0)


@jax.jit
def pallas_parallel_sum__linear_attn_block__moe_arch_mod__prompt_kernel(
    A_x: jax.Array,
    A_wqkv: jax.Array,
    A_wo: jax.Array,
    B_x: jax.Array,
    B_w_r: jax.Array,
    B_w_gate: jax.Array,
    B_w_up: jax.Array,
    B_w_down: jax.Array,
):
    del B_x
    assert A_x.shape == (1, S, D) and B_w_gate.shape == (D, F)
    any_spec = pl.BlockSpec(memory_space=pl.ANY)
    scratch = [
        pltpu.VMEM((NB, TB, D), BF16),
        pltpu.VMEM((NP, TB, D), BF16),
        pltpu.VMEM((NP, TB, D), BF16),
        pltpu.VMEM((NG, D, LANES), BF16),
        pltpu.VMEM((D, D + LANES), BF16),
        pltpu.VMEM((D, D), BF16),
        pltpu.VMEM((D, D), BF16),
        pltpu.VMEM((NP, D, D), BF16),
        pltpu.VMEM((NP, D, D), BF16),
        pltpu.VMEM((NP, D, D), BF16),
        pltpu.VMEM((2, D, 4 * LANES), F32),
        pltpu.VMEM((2, D, 4 * LANES), F32),
        pltpu.VMEM((D, D), F32),
        pltpu.VMEM((D // 2, D), U32),
        pltpu.VMEM((D // 2, D), U32),
        pltpu.VMEM((NB, TB, D), BF16),
        pltpu.VMEM((D // 2, LANES), U32),
        pltpu.VMEM((2 * TB, D), F32),
        pltpu.VMEM((2, 2, TB, LANES), F32),
        pltpu.VMEM((8, D), F32),
        pltpu.VMEM((8, D), F32),
        pltpu.VMEM((8, D), F32),
        pltpu.VMEM((8, D), F32),
        pltpu.VMEM((8, D), F32),
        pltpu.VMEM((16, LANES), F32),
        pltpu.VMEM((2, 8, 1), F32),
        pltpu.VMEM((8, 1), F32),
        pltpu.VMEM((D,), BF16),
        pltpu.SemaphoreType.DMA((N_SEMS,)),
    ]
    return pl.pallas_call(
        _kernel,
        out_shape=jax.ShapeDtypeStruct((1, S, D), BF16),
        in_specs=[any_spec] * 7,
        out_specs=any_spec,
        scratch_shapes=scratch,
        compiler_params=pltpu.CompilerParams(vmem_limit_bytes=100 * 1024 * 1024,
                                             disable_semaphore_checks=True, disable_bounds_checks=True),
    )(A_x, A_wqkv, A_wo, B_w_r, B_w_gate, B_w_up, B_w_down)
```

```python
import jax
import jax.numpy as jnp
from jax import lax
import jax.experimental.pallas as pl
import jax.experimental.pallas.tpu as pltpu

F32 = jnp.float32
BF16 = jnp.bfloat16
U32 = jnp.uint32

S = 2048
D = 1024
F = 3584
DH = 32
TB = 256
NB = S // TB
NP = NB // 2
FC = F // NP
LANES = 128
NG = D // LANES
HG = LANES // DH
KC = 256
NKC = D // KC
K_SPLITS = (0, 128, 256, 512, 768, 1024)
X_SPLITS = (0, 128, 256, 512, 1024)
KF = K_SPLITS[-2]
LN0_PACE = 4
PHI_PACE = 1
LEAD = 4
WQ_PER = 3
DELAY = 8
GU_TILE = 2
TAIL = ((0, 128), (128, 128))
SEM_A = 5
SEM_W = SEM_A + NP - 1
SEM_F = SEM_W + 1
SEM_O = SEM_F + NP
N_SEMS = SEM_O + 2


def _round_bf16(v):
    return v.astype(BF16).astype(F32)


def _phi(t):
    return jnp.where(t > 0, t + 1.0, jnp.exp(t)) + 1e-6


def _dot(a, b):
    return jnp.dot(a, b, preferred_element_type=F32)


def _dot_tn(a, b):
    return lax.dot_general(a, b, (((0,), (0,)), ((), ())), preferred_element_type=F32)


def _dot_nt(a, b):
    return lax.dot_general(a, b, (((1,), (1,)), ((), ())), preferred_element_type=F32)


def _after(v, dep, other=0.0):
    if dep is None:
        return v
    return jnp.where(dep > jnp.inf, other, v)


def _tie(w, dep, r0=0, c0=0):
    if dep is None:
        return w
    dep = jnp.broadcast_to(dep, (8, LANES))
    head = pltpu.bitcast(w[r0:r0 + 16, c0:c0 + LANES], U32) | (dep > jnp.inf).astype(U32)
    row = [pltpu.bitcast(head, BF16)]
    if c0:
        row = [w[r0:r0 + 16, :c0]] + row
    if c0 + LANES < w.shape[1]:
        row = row + [w[r0:r0 + 16, c0 + LANES:]]
    head = row[0] if len(row) == 1 else jnp.concatenate(row, axis=1)
    parts = ([w[:r0]] if r0 else []) + [head, w[r0 + 16:]]
    return jnp.concatenate(parts, axis=0)


def _ties(w, ties):
    for dep, r0, c0 in ties:
        w = _tie(w, dep, r0, c0)
    return w


def _shuffle_rows(w):
    sub = lax.broadcasted_iota(jnp.int32, (8, w.shape[1]), 0)
    v = [w[(a % 4) * 16 + (a // 4) * 8:(a % 4) * 16 + (a // 4) * 8 + 8] for a in range(8)]
    for d in (4, 2, 1):
        low = (sub & d) == 0
        nv = list(v)
        for a in range(8):
            if a & d == 0:
                nv[a] = jnp.where(low, v[a], pltpu.roll(v[a + d], d, 0))
                nv[a + d] = jnp.where(low, pltpu.roll(v[a], 8 - d, 0), v[a + d])
        v = nv
    return v


def _delay(v, n):
    for _ in range(n):
        v = pl.reciprocal(v, approx=True)
    return v


def _col_bcast(row):
    tiles = [jnp.broadcast_to(row[:, t * LANES:(t + 1) * LANES], (LANES, LANES)).T
             for t in range(row.shape[1] // LANES)]
    return jnp.concatenate(tiles, axis=0)


def _kernel(x_hbm, wqkv_hbm, wo_hbm, wr_hbm, wg_hbm, wu_hbm, wd_hbm, out_hbm,
            x_v, xn_v, wq_v, wk_v, wv_v, wo_v, wg_v, wu_v, wd_v, xcol_v, hcol_v,
            g_acc, m_v, wqt_v, out_v, wq0_v, kraw_v, st_v, cs_v, wr_f, z_acc, zp_v, y_acc, gate_v, best_v, junk_v, wr_v,
            sem):
    def x_copy(b, s_):
        return pltpu.make_async_copy(x_hbm.at[0, pl.ds(b * TB, TB), :], x_v.at[b], sem.at[s_])

    def xs_copies(i):
        cols = pl.ds(X_SPLITS[i], X_SPLITS[i + 1] - X_SPLITS[i])
        return [pltpu.make_async_copy(x_hbm.at[0, pl.ds(b * TB, TB), cols], x_v.at[b, :, cols],
                                      sem.at[i]) for b in (0, NB - 1)]

    def wk_copy(i):
        rows = pl.ds(K_SPLITS[i], K_SPLITS[i + 1] - K_SPLITS[i])
        return pltpu.make_async_copy(wqkv_hbm.at[rows, pl.ds(D, D)], wk_v.at[rows, pl.ds(0, D)],
                                     sem.at[i])

    def wq_copy(g, s_):
        cols = pl.ds(pl.multiple_of(g * LANES, LANES), LANES)
        return pltpu.make_async_copy(wqkv_hbm.at[:, cols], wq_v.at[g], sem.at[s_])

    wr_copy = pltpu.make_async_copy(wr_hbm, wr_v, sem.at[3])
    wv_copy = pltpu.make_async_copy(wqkv_hbm.at[:, pl.ds(2 * D, D)], wv_v, sem.at[SEM_W])
    wo_copy = pltpu.make_async_copy(wo_hbm, wo_v, sem.at[SEM_W])

    def ffn_copies(c, s_):
        span = pl.ds(pl.multiple_of(c * FC, LANES), FC)
        return (
            pltpu.make_async_copy(wg_hbm.at[:, span], wg_v.at[c, :, pl.ds(0, FC)], sem.at[s_]),
            pltpu.make_async_copy(wu_hbm.at[:, span], wu_v.at[c, :, pl.ds(0, FC)], sem.at[s_]),
            pltpu.make_async_copy(wd_hbm.at[span, :], wd_v.at[c, pl.ds(0, FC), :], sem.at[s_]),
        )

    for i in range(len(K_SPLITS) - 1):
        if i < len(X_SPLITS) - 1:
            for cp in xs_copies(i):
                cp.start()
        if i == 3:
            wr_copy.start()
        wk_copy(i).start()
    x_copy(1, 4).start()
    for j in range(NP - 1):
        x_copy(2 * j + 2, SEM_A + j).start()
        if 2 * j + 3 < NB - 1:
            x_copy(2 * j + 3, SEM_A + j).start()
        for g in range(WQ_PER * j, min(WQ_PER * (j + 1), NG)):
            wq_copy(g, SEM_A + j).start()
    wv_copy.start()
    wo_copy.start()
    for c in range(NP):
        for cp in ffn_copies(c, SEM_F + c):
            cp.start()

    y_acc[...] = jnp.zeros_like(y_acc)
    sub8 = lax.broadcasted_iota(jnp.int32, (8, 1), 0).astype(F32)

    def normalise(b, dst_ref, j, r0, nr, dep=None, keep=None):
        rs = pl.ds(r0, nr)
        mean = jnp.mean(x_v[b, rs, :].astype(F32), axis=-1, keepdims=True)
        mean_b = jnp.broadcast_to(_round_bf16(mean), (nr, LANES))
        junk_v[...] = mean[:8]
        c = x_v[b, rs, :].astype(F32) - mean
        var = jnp.mean(c * c, axis=-1, keepdims=True)
        junk_v[...] = var[:8]
        rstd = 1.0 / _round_bf16(jnp.sqrt(_round_bf16(_round_bf16(var) + 1e-5)))
        if keep is not None:
            st_v[keep, 0, rs, :] = mean_b
            st_v[keep, 1, rs, :] = jnp.broadcast_to(rstd, (nr, LANES))
        mean_b = jnp.concatenate([_after(mean_b, dep)] * NG, axis=1)
        xn_f = _round_bf16(x_v[b, rs, :].astype(F32) - mean_b) * rstd
        xn = xn_f.astype(BF16)
        dst_ref[j, rs, :] = xn
        return xn, xn_f

    def score(xn, row0, best, dep=None):
        nr = xn.shape[0]
        wr = wr_f[...]
        if dep is not None:
            wr = jnp.concatenate([_after(wr[:, :LANES], dep[:8]), wr[:, LANES:]], axis=1)
        if nr > 8:
            wr = jnp.concatenate([wr] * (nr // 8), axis=0)
        r = jnp.sum(xn.astype(F32) * wr, axis=-1, keepdims=True)
        rb = _round_bf16(r)
        bv, bi = best
        for q in range(nr // 8):
            rq = rb[q * 8:(q + 1) * 8]
            better = rq > bv
            bv = jnp.where(better, rq, bv)
            bi = jnp.where(better, sub8 + jnp.asarray(row0 + q * 8).astype(F32), bi)
        return r, (bv, bi)

    def layernorm(b, dst_ref, j, r0, nr, best, dep=None, keep=None):
        return score(normalise(b, dst_ref, j, r0, nr, dep, keep)[0], b * TB + r0, best)

    def load_best():
        return best_v[0], best_v[1]

    def store_best(best):
        best_v[0] = best[0]
        best_v[1] = best[1]

    def k_unit(src_ref, j, lo, hi, first=False, ties=()):
        pk = _phi(_dot(src_ref[j], _ties(wk_v[:, lo:hi], ties)))
        zs = jnp.sum(pk.reshape(TB // 8, 8, hi - lo), axis=0)
        if first:
            z_acc[:, lo:hi] = zs
        else:
            z_acc[:, lo:hi] += zs
        return pk.astype(BF16)

    def raw_slice(i):
        lo, hi = K_SPLITS[i], K_SPLITS[i + 1]
        xs = jnp.concatenate([x_v[0, :, lo:hi], x_v[NB - 1, :, lo:hi]], axis=0)
        part = _dot(xs, wk_v[lo:hi, :D])
        if i == 0:
            kraw_v[...] = part
        else:
            kraw_v[...] += part
        if i == 2:
            cs_v[...] = jnp.sum(wk_v[:hi, :D].astype(F32).reshape(hi // 8, 8, D), axis=0)
        elif i > 2:
            cs_v[...] += jnp.sum(wk_v[lo:hi, :D].astype(F32).reshape((hi - lo) // 8, 8, D), axis=0)

    def raw_last(b, c):
        return _dot(x_v[b, :, KF:], wk_v[KF:, c * KC:(c + 1) * KC])

    def raw_finish(slot, c, part, first, paced):
        cs = slice(c * KC, (c + 1) * KC)
        rows_ = []
        dep = None
        zs = None
        for r0 in range(0, TB, 16):
            mean = st_v[slot, 0, r0:r0 + 16, :]
            rstd = _after(st_v[slot, 1, r0:r0 + 16, :], dep)
            mean = jnp.concatenate([mean] * (KC // LANES), axis=1)
            rstd = jnp.concatenate([rstd] * (KC // LANES), axis=1)
            col = jnp.concatenate([cs_v[:, cs]] * 2, axis=0)
            k = (kraw_v[slot * TB + r0:slot * TB + r0 + 16, cs] + part[r0:r0 + 16] - mean * col) * rstd
            pk = _phi(k)
            z2 = pk[:8] + pk[8:]
            zs = z2 if zs is None else zs + z2
            if paced:
                f = _delay(z2[:, :LANES] + z2[:, LANES:], PHI_PACE)
                dep = jnp.concatenate([f, f], axis=0)
            rows_.append(pk.astype(BF16))
        if first:
            z_acc[:, cs] = zs
        else:
            z_acc[:, cs] += zs
        return jnp.concatenate(rows_, axis=0)

    def g_unit(src_ref, j, lo, hi, pk, first=False, ties=()):
        g = _dot_tn(pk, _ties(src_ref[j], ties))
        if first:
            g_acc[lo:hi, :] = g
        else:
            g_acc[lo:hi, :] += g

    def wq_prep(g, kk):
        v = _shuffle_rows(pltpu.bitcast(wq_v[g, kk * 256:(kk + 1) * 256, :].T, U32))
        base = pl.multiple_of(g * 8, 8)
        tot = None
        for i in range(8):
            wqt_v[pl.ds(i * 64 + base, 8), kk * 256:(kk + 1) * 256] = v[i]
            tot = v[i] if tot is None else tot | v[i]
        return pltpu.bitcast(tot[:, :LANES] | tot[:, LANES:], F32)

    def mv_chain(acc, w_ref, c, n0, col_ref, z0, k=D):
        cp = 2 * LANES if (n0 // 256) % 4 < 2 else 0
        cz = c + z0

        def step(i, acc):
            rows = pl.ds(pl.multiple_of(i * 8, 8), 8)
            return acc + w_ref[cz, rows, n0:n0 + LANES].astype(F32) * col_ref[z0, rows, cp:cp + LANES]
        return lax.fori_loop(0, k // 8, step, acc, unroll=True)

    def ffn_gate_up(c, zeros):
        dep = None
        zero = jnp.zeros((8, LANES), F32)
        for n0 in range(0, FC, LANES):
            ga = mv_chain(_after(zero, dep, 1.0), wg_v, c, n0, xcol_v, next(zeros))
            ua = mv_chain(_after(zero, ga, 1.0), wu_v, c, n0, xcol_v, next(zeros))
            dep = ua
            gg = _round_bf16(jnp.sum(ga, axis=0, keepdims=True))
            uu = _round_bf16(jnp.sum(ua, axis=0, keepdims=True))
            h = _round_bf16(_round_bf16(gg * jax.nn.sigmoid(gg)) * uu)
            hc = _col_bcast(h)
            hcol_v[0, n0:n0 + LANES, :LANES] = hc
            hcol_v[0, n0:n0 + LANES, 2 * LANES:3 * LANES] = hc
        return dep

    def ffn_down(c, zeros):
        dep = None
        accs = []
        for n0 in range(0, D, LANES):
            dep = mv_chain(_after(y_acc[:, n0:n0 + LANES], dep), wd_v, c, n0, hcol_v, next(zeros), FC)
            y_acc[:, n0:n0 + LANES] = dep
            accs.append(dep)
        return jnp.concatenate(accs, axis=1)

    def first_half():
        for i in range(4):
            for cp in xs_copies(i):
                cp.wait()
            if i == 3:
                wr_copy.wait()
            wk_copy(i).wait()
            raw_slice(i)
            if i == 3:
                wr_f[...] = jnp.broadcast_to(wr_v[...].astype(F32).reshape(1, D), (8, D))
                dep = None
                for r0 in range(0, TB, 8):
                    _, xn_f = normalise(0, xn_v, 0, r0, 8, dep, keep=0)
                    dep = _delay(xn_f[:, D - LANES:], LN0_PACE)
        wk_copy(4).wait()
        x_copy(1, 4).wait()
        cs = cs_v[...] + jnp.sum(wk_v[KF:, :D].astype(F32).reshape((D - KF) // 8, 8, D), axis=0)
        cs_v[...] = jnp.broadcast_to(jnp.sum(cs, axis=0, keepdims=True), (8, D))
        best = (jnp.full((8, 1), -jnp.inf, F32), sub8)
        dep = None
        for r0 in range(0, TB, 16):
            dep, best = layernorm(1, xn_v, 1, r0, 16, best, dep)
        store_best(best)
        parts = [raw_last(0, c) for c in range(LEAD)]
        for c in range(NKC):
            g_unit(xn_v, 0, c * KC, (c + 1) * KC, raw_finish(0, c, parts[c], True, False), True,
                   [(dep[:8], 0, 512)] if c == NKC - 1 else [])
            if len(parts) < NKC:
                parts.append(raw_last(0, len(parts)))

        def phase_a(j, carry):
            x_copy(2 * j + 2, SEM_A + j).wait()
            wq_copy(WQ_PER * j, SEM_A + j).wait()
            wq_copy(WQ_PER * j + 1, SEM_A + j).wait()

            @pl.when(j < NP - 2)
            def _():
                x_copy(2 * j + 3, SEM_A + j).wait()
                wq_copy(WQ_PER * j + 2, SEM_A + j).wait()

            preps = [(jnp.minimum(WQ_PER * j + i, NG - 1), kk) for i in range(WQ_PER) for kk in range(4)]
            k_slots = {(0, 0): [(0, 128), (512, 128)], (0, 1): [(0, 0), (512, 0), (0, 128), (512, 128)],
                       (1, 1): [(0, 0), (512, 0)]}
            g_slots = {(0, 3): [(0, 0), (0, 256), (0, 512), (0, 768)]}

            def mk_ties(slots):
                return [(wq_prep(*preps.pop(0)), r0, c0) for r0, c0 in slots]

            LR = TB // NKC
            prev = None
            dep = None
            best = load_best()
            win = xn_v.at[pl.ds(2 * j + 1, 3)]
            for half in range(2):
                src, js = win, half
                dst, b = win, 2 * j + 2 + half
                for c in range(NKC):
                    pk = k_unit(src, js, c * KC, (c + 1) * KC, ties=mk_ties(k_slots.get((half, c), [])))
                    if prev is not None:
                        g_unit(*prev[1:], ties=mk_ties(g_slots.get(prev[0], [])))
                    prev = ((half, c), src, js, c * KC, (c + 1) * KC, pk)
                    for r0 in range(c * LR, (c + 1) * LR, 8):
                        dep, best = layernorm(b, dst, half + 1, r0, 8, best, dep, keep=1 if half else None)
            g_unit(*prev[1:], ties=[(dep, 0, 768)])
            assert not preps
            store_best(best)
            return carry

        lax.fori_loop(0, NP - 1, phase_a, 0)


    def second_half():
        wv_copy.wait()
        wo_copy.wait()

        best0 = (jnp.full((8, 1), -jnp.inf, F32), sub8)
        dep = None
        for r0 in range(0, TB, 16):
            dep, best0 = score(xn_v[0, r0:r0 + 16, :], r0, best0, dep)
        bv, bi = load_best()
        first0 = best0[0] >= bv
        bv = jnp.where(first0, best0[0], bv)
        bi = jnp.where(first0, best0[1], bi)
        r_max = jnp.max(bv, axis=0, keepdims=True)
        idx_f = jnp.min(jnp.where(bv == r_max, bi, float(S - 1)))
        idx = jnp.clip(idx_f.astype(jnp.int32), 0, S - 1)
        blk = idx // TB
        hot_pair = blk // 2
        row16 = pl.multiple_of(((idx % TB) // 16) * 16, 16)
        gate_v[...] = jnp.broadcast_to(_round_bf16(jax.nn.sigmoid(r_max)), (16, LANES))
        row_id16 = lax.broadcasted_iota(jnp.int32, (16, D), 0)
        sel16 = row_id16 == idx % 16
        xs = xn_v[blk, pl.ds(row16, 16), :].astype(F32)
        xc = _col_bcast(jnp.sum(jnp.where(sel16, xs, 0.0), axis=0, keepdims=True))
        xcol_v[0, :, :LANES] = xc
        xcol_v[0, :, 2 * LANES:3 * LANES] = xc

        rr = lax.broadcasted_iota(jnp.int32, (LANES, LANES), 0) // DH
        cc = lax.broadcasted_iota(jnp.int32, (LANES, LANES), 1) // DH
        same_head = rr == cc

        def g_final(c, pk, dep=None):
            return (g_acc[c * KC:(c + 1) * KC, :] + _dot_tn(pk, _tie(xn_v[NB - 1], dep))).astype(BF16)

        def kv_unit(c, gf):
            out = []
            for gg in range(KC // LANES):
                g = c * (KC // LANES) + gg
                kv = _dot(gf[gg * LANES:(gg + 1) * LANES, :], wv_v[:, g * LANES:(g + 1) * LANES])
                kv = pltpu.bitcast(jnp.where(same_head, kv, 0.0).astype(BF16), U32)
                out.append(pltpu.bitcast(jnp.concatenate(_shuffle_rows(kv), axis=0), BF16))
            return out

        def m_unit(c, kvs, dep=None):
            for gg in range(KC // LANES):
                g = c * (KC // LANES) + gg
                m = _dot(kvs[gg], _tie(wo_v[g * LANES:(g + 1) * LANES, :], dep))
                dep = None
                w = pltpu.bitcast(m.astype(BF16), U32)
                for i in range(8):
                    m_v[i * 64 + g * 8:i * 64 + (g + 1) * 8, :] = w[i * 8:(i + 1) * 8, :]

        def z_prep():
            zc = pltpu.bitcast(_col_bcast(jnp.sum(z_acc[...], axis=0, keepdims=True)).astype(BF16), U32)
            vs = [_shuffle_rows(zc[g * 64:(g + 1) * 64, :]) for g in range(NG)]
            tot = None
            for i in range(NG):
                zt = pltpu.bitcast(jnp.concatenate([vs[g][i] for g in range(NG)], axis=0), BF16)
                zp = zt.astype(F32).T[:8, :]
                zp_v[:, i * LANES:(i + 1) * LANES] = zp
                tot = zp if tot is None else tot + zp
            return tot

        wq0_v[...] = pltpu.bitcast(pltpu.bitcast(wqt_v[:LANES // 2, :], BF16).T, U32)
        parts = [raw_last(NB - 1, c) for c in range(LEAD)]

        def gf(c):
            g = g_final(c, raw_finish(1, c, parts[c], False, False))
            if len(parts) < NKC:
                parts.append(raw_last(NB - 1, len(parts)))
            return g

        gf0 = gf(0)
        gf1 = gf(1)
        kv0 = kv_unit(0, gf0)
        gf2 = gf(2)
        kv1 = kv_unit(1, gf1)
        m_unit(0, kv0)
        gf3 = gf(3)
        kv2 = kv_unit(2, gf2)
        m_unit(1, kv1, xc[D - 8:])
        kv3 = kv_unit(3, gf3)
        m_unit(2, kv2, z_prep())
        m_unit(3, kv3)

        lane = lax.broadcasted_iota(jnp.int32, (8, LANES), 1)
        bit0 = lane % 2 == 0
        bit3 = (lane // 8) % 2 == 0

        def q_part(src_ref, p, ties=(), lead=False):
            wqt = _ties(pltpu.bitcast(wqt_v[...], BF16), ties)
            if lead:
                xn = src_ref[p]
                q0 = _dot(xn, pltpu.bitcast(wq0_v[...], BF16))
                q = jnp.concatenate([q0, _dot_nt(xn, wqt[LANES:])], axis=1)
            else:
                q = _dot_nt(src_ref[p], wqt)
            rows_ = []
            dep = None
            for g in range(TB // 8):
                pq = _phi(q[g * 8:(g + 1) * 8, :])
                t = pq * zp_v[...]
                s_ = t[:, :LANES]
                for n in range(1, NG):
                    s_ = s_ + t[:, n * LANES:(n + 1) * LANES]
                s_ = s_ + jnp.where(bit3, pltpu.roll(s_, LANES - 8, 1), pltpu.roll(s_, 8, 1))
                s_ = s_ + jnp.where(bit0, pltpu.roll(s_, LANES - 1, 1), pltpu.roll(s_, 1, 1))
                rinv = _after(pl.reciprocal(s_ + 1e-6, approx=True), dep)
                rows_.append(pq * jnp.concatenate([rinv] * NG, axis=1))
                dep = _delay(rinv, DELAY)
            return jnp.concatenate(rows_, axis=0).astype(BF16)

        def o_part(o, src_ref, p, b, s_out, last, dep=None):
            spans = [(0, 256), (256, 512), (512, 768), (768, 896), (896, D)] if last else \
                [(c * KC, (c + 1) * KC) for c in range(NKC)]
            for lo, hi in spans:
                m = pltpu.bitcast(m_v[:, lo:hi], BF16)
                a = _dot(o, _tie(m, dep if lo == 768 else None))
                for r0, nr in (TAIL if last and hi == D else ((0, TB),)):
                    rs = slice(r0, r0 + nr)
                    out_v[b, rs, lo:hi] = (x_v[b, rs, lo:hi].astype(F32) + a[rs]
                                           + src_ref[p, rs, lo:hi].astype(F32)).astype(BF16)
                    if last or hi == D:
                        cols = pl.ds(lo, hi - lo) if last else pl.ds(0, D)
                        pltpu.make_async_copy(out_v.at[b, pl.ds(r0, nr), cols],
                                              out_hbm.at[0, pl.ds(b * TB + r0, nr), cols],
                                              sem.at[s_out]).start()

        def phase_b(j, carry):
            for cp in ffn_copies(j, SEM_F + j):
                cp.wait()
            p = jnp.where(j == 0, hot_pair, jnp.where(j == hot_pair, 0, j))
            s_out = jnp.where(j == 0, SEM_O, SEM_O + 1)
            zeros = (lax.shift_right_logical(idx + j + k, 13) for k in range(64))
            gu_dep = ffn_gate_up(j, zeros)
            y = ffn_down(j, zeros)
            o_e = q_part(xn_v, 2 * p, lead=True)
            o_o = q_part(xn_v, 2 * p + 1, [(gu_dep, GU_TILE * LANES, 0)])
            o_part(o_e, xn_v, 2 * p, 2 * p, s_out, False)
            o_part(o_o, xn_v, 2 * p + 1, 2 * p + 1, s_out, True, y[:, D - LANES:])
            return carry

        lax.fori_loop(0, NP, phase_b, 0)

        hot = out_v.at[pl.ds(2 * hot_pair, 2)]
        pltpu.make_async_copy(hot, hot, sem.at[SEM_O]).wait()
        rows16 = pl.ds(row16, 16)
        yrow = _round_bf16(jnp.sum(y_acc[...], axis=0, keepdims=True))
        upd = jnp.where(sel16, yrow * jnp.concatenate([gate_v[...]] * NG, axis=1), 0.0)
        out_v[blk, rows16, :] = (out_v[blk, rows16, :].astype(F32) + upd).astype(BF16)
        patch = pltpu.make_async_copy(
            out_v.at[blk, rows16, :],
            out_hbm.at[0, pl.ds(pl.multiple_of(blk * TB + row16, 16), 16), :], sem.at[SEM_O])
        patch.start()
        pltpu.make_async_copy(out_v.at[pl.ds(2, NB - 2)], out_v.at[pl.ds(2, NB - 2)],
                              sem.at[SEM_O + 1]).wait()
        patch.wait()

    def outer(i, carry):
        pl.when(i == 0)(first_half)
        pl.when(i == 1)(second_half)
        return carry

    lax.fori_loop(0, 2, outer, 0)


@jax.jit
def pallas_parallel_sum__linear_attn_block__moe_arch_mod__prompt_kernel(
    A_x: jax.Array,
    A_wqkv: jax.Array,
    A_wo: jax.Array,
    B_x: jax.Array,
    B_w_r: jax.Array,
    B_w_gate: jax.Array,
    B_w_up: jax.Array,
    B_w_down: jax.Array,
):
    del B_x
    assert A_x.shape == (1, S, D) and B_w_gate.shape == (D, F)
    any_spec = pl.BlockSpec(memory_space=pl.ANY)
    scratch = [
        pltpu.VMEM((NB, TB, D), BF16),
        pltpu.VMEM((NB, TB, D), BF16),
        pltpu.VMEM((NG, D, LANES), BF16),
        pltpu.VMEM((D, D + LANES), BF16),
        pltpu.VMEM((D, D), BF16),
        pltpu.VMEM((D, D), BF16),
        pltpu.VMEM((NP, D, D), BF16),
        pltpu.VMEM((NP, D, D), BF16),
        pltpu.VMEM((NP, D, D), BF16),
        pltpu.VMEM((2, D, 4 * LANES), F32),
        pltpu.VMEM((2, D, 4 * LANES), F32),
        pltpu.VMEM((D, D), F32),
        pltpu.VMEM((D // 2, D), U32),
        pltpu.VMEM((D // 2, D), U32),
        pltpu.VMEM((NB, TB, D), BF16),
        pltpu.VMEM((D // 2, LANES), U32),
        pltpu.VMEM((2 * TB, D), F32),
        pltpu.VMEM((2, 2, TB, LANES), F32),
        pltpu.VMEM((8, D), F32),
        pltpu.VMEM((8, D), F32),
        pltpu.VMEM((8, D), F32),
        pltpu.VMEM((8, D), F32),
        pltpu.VMEM((8, D), F32),
        pltpu.VMEM((16, LANES), F32),
        pltpu.VMEM((2, 8, 1), F32),
        pltpu.VMEM((8, 1), F32),
        pltpu.VMEM((D,), BF16),
        pltpu.SemaphoreType.DMA((N_SEMS,)),
    ]
    return pl.pallas_call(
        _kernel,
        out_shape=jax.ShapeDtypeStruct((1, S, D), BF16),
        in_specs=[any_spec] * 7,
        out_specs=any_spec,
        scratch_shapes=scratch,
        compiler_params=pltpu.CompilerParams(vmem_limit_bytes=100 * 1024 * 1024,
                                             disable_semaphore_checks=True, disable_bounds_checks=True),
    )(A_x, A_wqkv, A_wo, B_w_r, B_w_gate, B_w_up, B_w_down)
```

```python
import jax
import jax.numpy as jnp
from jax import lax
import jax.experimental.pallas as pl
import jax.experimental.pallas.tpu as pltpu

F32 = jnp.float32
BF16 = jnp.bfloat16
U32 = jnp.uint32

S = 2048
D = 1024
F = 3584
DH = 32
TB = 256
NB = S // TB
NP = NB // 2
FC = F // NP
LANES = 128
NG = D // LANES
HG = LANES // DH
KC = 256
NKC = D // KC
K_SPLITS = (0, 128, 256, 512, 768, 1024)
X_SPLITS = (0, 128, 256, 512, 1024)
KF = K_SPLITS[-2]
LN0_PACE = 4
PHI_PACE = 1
LEAD = 4
NA = 2
BA = (NB - 2) // NA
WQ_PER = NG // NA
DELAY = 8
GU_TILE = 2
TAIL = ((0, 128), (128, 128))
SEM_A = 5
SEM_W = SEM_A + NA
SEM_F = SEM_W + 1
SEM_O = SEM_F + NP
N_SEMS = SEM_O + 2


def _round_bf16(v):
    return v.astype(BF16).astype(F32)


def _phi(t):
    return jnp.where(t > 0, t + 1.0, jnp.exp(t)) + 1e-6


def _dot(a, b):
    return jnp.dot(a, b, preferred_element_type=F32)


def _dot_tn(a, b):
    return lax.dot_general(a, b, (((0,), (0,)), ((), ())), preferred_element_type=F32)


def _dot_nt(a, b):
    return lax.dot_general(a, b, (((1,), (1,)), ((), ())), preferred_element_type=F32)


def _after(v, dep, other=0.0):
    if dep is None:
        return v
    return jnp.where(dep > jnp.inf, other, v)


def _tie(w, dep, r0=0, c0=0):
    if dep is None:
        return w
    dep = jnp.broadcast_to(dep, (8, LANES))
    head = pltpu.bitcast(w[r0:r0 + 16, c0:c0 + LANES], U32) | (dep > jnp.inf).astype(U32)
    row = [pltpu.bitcast(head, BF16)]
    if c0:
        row = [w[r0:r0 + 16, :c0]] + row
    if c0 + LANES < w.shape[1]:
        row = row + [w[r0:r0 + 16, c0 + LANES:]]
    head = row[0] if len(row) == 1 else jnp.concatenate(row, axis=1)
    parts = ([w[:r0]] if r0 else []) + [head, w[r0 + 16:]]
    return jnp.concatenate(parts, axis=0)


def _ties(w, ties):
    for dep, r0, c0 in ties:
        w = _tie(w, dep, r0, c0)
    return w


def _shuffle_rows(w):
    sub = lax.broadcasted_iota(jnp.int32, (8, w.shape[1]), 0)
    v = [w[(a % 4) * 16 + (a // 4) * 8:(a % 4) * 16 + (a // 4) * 8 + 8] for a in range(8)]
    for d in (4, 2, 1):
        low = (sub & d) == 0
        nv = list(v)
        for a in range(8):
            if a & d == 0:
                nv[a] = jnp.where(low, v[a], pltpu.roll(v[a + d], d, 0))
                nv[a + d] = jnp.where(low, pltpu.roll(v[a], 8 - d, 0), v[a + d])
        v = nv
    return v


def _delay(v, n):
    for _ in range(n):
        v = pl.reciprocal(v, approx=True)
    return v


def _col_bcast(row):
    tiles = [jnp.broadcast_to(row[:, t * LANES:(t + 1) * LANES], (LANES, LANES)).T
             for t in range(row.shape[1] // LANES)]
    return jnp.concatenate(tiles, axis=0)


def _kernel(x_hbm, wqkv_hbm, wo_hbm, wr_hbm, wg_hbm, wu_hbm, wd_hbm, out_hbm,
            x_v, xn_v, wq_v, wk_v, wv_v, wo_v, wg_v, wu_v, wd_v, xcol_v, hcol_v,
            g_acc, m_v, wqt_v, out_v, wq0_v, kraw_v, st_v, cs_v, wr_f, z_acc, zp_v, y_acc, gate_v, best_v, junk_v, wr_v,
            sem):
    def x_copy(b, s_):
        return pltpu.make_async_copy(x_hbm.at[0, pl.ds(b * TB, TB), :], x_v.at[b], sem.at[s_])

    def xs_copies(i):
        cols = pl.ds(X_SPLITS[i], X_SPLITS[i + 1] - X_SPLITS[i])
        return [pltpu.make_async_copy(x_hbm.at[0, pl.ds(b * TB, TB), cols], x_v.at[b, :, cols],
                                      sem.at[i]) for b in (0, NB - 1)]

    def wk_copy(i):
        rows = pl.ds(K_SPLITS[i], K_SPLITS[i + 1] - K_SPLITS[i])
        return pltpu.make_async_copy(wqkv_hbm.at[rows, pl.ds(D, D)], wk_v.at[rows, pl.ds(0, D)],
                                     sem.at[i])

    def wq_copy(g, s_):
        cols = pl.ds(pl.multiple_of(g * LANES, LANES), LANES)
        return pltpu.make_async_copy(wqkv_hbm.at[:, cols], wq_v.at[g], sem.at[s_])

    wr_copy = pltpu.make_async_copy(wr_hbm, wr_v, sem.at[3])
    wv_copy = pltpu.make_async_copy(wqkv_hbm.at[:, pl.ds(2 * D, D)], wv_v, sem.at[SEM_W])
    wo_copy = pltpu.make_async_copy(wo_hbm, wo_v, sem.at[SEM_W])

    def ffn_copies(c, s_):
        span = pl.ds(pl.multiple_of(c * FC, LANES), FC)
        return (
            pltpu.make_async_copy(wg_hbm.at[:, span], wg_v.at[c, :, pl.ds(0, FC)], sem.at[s_]),
            pltpu.make_async_copy(wu_hbm.at[:, span], wu_v.at[c, :, pl.ds(0, FC)], sem.at[s_]),
            pltpu.make_async_copy(wd_hbm.at[span, :], wd_v.at[c, pl.ds(0, FC), :], sem.at[s_]),
        )

    for i in range(len(K_SPLITS) - 1):
        if i < len(X_SPLITS) - 1:
            for cp in xs_copies(i):
                cp.start()
        if i == 3:
            wr_copy.start()
        wk_copy(i).start()
    x_copy(1, 4).start()
    for j in range(NA):
        for b in range(BA * j + 2, min(BA * (j + 1) + 2, NB - 1)):
            x_copy(b, SEM_A + j).start()
        for g in range(WQ_PER * j, WQ_PER * (j + 1)):
            wq_copy(g, SEM_A + j).start()
    wv_copy.start()
    wo_copy.start()
    for c in range(NP):
        for cp in ffn_copies(c, SEM_F + c):
            cp.start()

    y_acc[...] = jnp.zeros_like(y_acc)
    sub8 = lax.broadcasted_iota(jnp.int32, (8, 1), 0).astype(F32)

    def normalise(b, dst_ref, j, r0, nr, dep=None, keep=None):
        rs = pl.ds(r0, nr)
        mean = jnp.mean(x_v[b, rs, :].astype(F32), axis=-1, keepdims=True)
        mean_b = jnp.broadcast_to(_round_bf16(mean), (nr, LANES))
        junk_v[...] = mean[:8]
        c = x_v[b, rs, :].astype(F32) - mean
        var = jnp.mean(c * c, axis=-1, keepdims=True)
        junk_v[...] = var[:8]
        rstd = 1.0 / _round_bf16(jnp.sqrt(_round_bf16(_round_bf16(var) + 1e-5)))
        if keep is not None:
            st_v[keep, 0, rs, :] = mean_b
            st_v[keep, 1, rs, :] = jnp.broadcast_to(rstd, (nr, LANES))
        mean_b = jnp.concatenate([_after(mean_b, dep)] * NG, axis=1)
        xn_f = _round_bf16(x_v[b, rs, :].astype(F32) - mean_b) * rstd
        xn = xn_f.astype(BF16)
        dst_ref[j, rs, :] = xn
        return xn, xn_f

    def score(xn, row0, best, dep=None):
        nr = xn.shape[0]
        wr = wr_f[...]
        if dep is not None:
            wr = jnp.concatenate([_after(wr[:, :LANES], dep[:8]), wr[:, LANES:]], axis=1)
        if nr > 8:
            wr = jnp.concatenate([wr] * (nr // 8), axis=0)
        r = jnp.sum(xn.astype(F32) * wr, axis=-1, keepdims=True)
        rb = _round_bf16(r)
        bv, bi = best
        for q in range(nr // 8):
            rq = rb[q * 8:(q + 1) * 8]
            better = rq > bv
            bv = jnp.where(better, rq, bv)
            bi = jnp.where(better, sub8 + jnp.asarray(row0 + q * 8).astype(F32), bi)
        return r, (bv, bi)

    def layernorm(b, dst_ref, j, r0, nr, best, dep=None, keep=None):
        return score(normalise(b, dst_ref, j, r0, nr, dep, keep)[0], b * TB + r0, best)

    def load_best():
        return best_v[0], best_v[1]

    def store_best(best):
        best_v[0] = best[0]
        best_v[1] = best[1]

    def k_unit(src_ref, j, lo, hi, first=False, ties=()):
        pk = _phi(_dot(src_ref[j], _ties(wk_v[:, lo:hi], ties)))
        zs = jnp.sum(pk.reshape(TB // 8, 8, hi - lo), axis=0)
        if first:
            z_acc[:, lo:hi] = zs
        else:
            z_acc[:, lo:hi] += zs
        return pk.astype(BF16)

    def raw_slice(i):
        lo, hi = K_SPLITS[i], K_SPLITS[i + 1]
        xs = jnp.concatenate([x_v[0, :, lo:hi], x_v[NB - 1, :, lo:hi]], axis=0)
        part = _dot(xs, wk_v[lo:hi, :D])
        if i == 0:
            kraw_v[...] = part
        else:
            kraw_v[...] += part
        if i == 2:
            cs_v[...] = jnp.sum(wk_v[:hi, :D].astype(F32).reshape(hi // 8, 8, D), axis=0)
        elif i > 2:
            cs_v[...] += jnp.sum(wk_v[lo:hi, :D].astype(F32).reshape((hi - lo) // 8, 8, D), axis=0)

    def raw_last(b, c):
        return _dot(x_v[b, :, KF:], wk_v[KF:, c * KC:(c + 1) * KC])

    def raw_finish(slot, c, part, first, paced):
        cs = slice(c * KC, (c + 1) * KC)
        rows_ = []
        dep = None
        zs = None
        for r0 in range(0, TB, 16):
            mean = st_v[slot, 0, r0:r0 + 16, :]
            rstd = _after(st_v[slot, 1, r0:r0 + 16, :], dep)
            mean = jnp.concatenate([mean] * (KC // LANES), axis=1)
            rstd = jnp.concatenate([rstd] * (KC // LANES), axis=1)
            col = jnp.concatenate([cs_v[:, cs]] * 2, axis=0)
            k = (kraw_v[slot * TB + r0:slot * TB + r0 + 16, cs] + part[r0:r0 + 16] - mean * col) * rstd
            pk = _phi(k)
            z2 = pk[:8] + pk[8:]
            zs = z2 if zs is None else zs + z2
            if paced:
                f = _delay(z2[:, :LANES] + z2[:, LANES:], PHI_PACE)
                dep = jnp.concatenate([f, f], axis=0)
            rows_.append(pk.astype(BF16))
        if first:
            z_acc[:, cs] = zs
        else:
            z_acc[:, cs] += zs
        return jnp.concatenate(rows_, axis=0)

    def g_unit(src_ref, j, lo, hi, pk, first=False, ties=()):
        g = _dot_tn(pk, _ties(src_ref[j], ties))
        if first:
            g_acc[lo:hi, :] = g
        else:
            g_acc[lo:hi, :] += g

    def wq_prep(g, kk):
        v = _shuffle_rows(pltpu.bitcast(wq_v[g, kk * 256:(kk + 1) * 256, :].T, U32))
        base = pl.multiple_of(g * 8, 8)
        tot = None
        for i in range(8):
            wqt_v[pl.ds(i * 64 + base, 8), kk * 256:(kk + 1) * 256] = v[i]
            tot = v[i] if tot is None else tot | v[i]
        return pltpu.bitcast(tot[:, :LANES] | tot[:, LANES:], F32)

    def mv_chain(acc, w_ref, c, n0, col_ref, z0, k=D):
        cp = 2 * LANES if (n0 // 256) % 4 < 2 else 0
        cz = c + z0

        def step(i, acc):
            rows = pl.ds(pl.multiple_of(i * 8, 8), 8)
            return acc + w_ref[cz, rows, n0:n0 + LANES].astype(F32) * col_ref[z0, rows, cp:cp + LANES]
        return lax.fori_loop(0, k // 8, step, acc, unroll=True)

    def ffn_gate_up(c, zeros):
        dep = None
        zero = jnp.zeros((8, LANES), F32)
        for n0 in range(0, FC, LANES):
            ga = mv_chain(_after(zero, dep, 1.0), wg_v, c, n0, xcol_v, next(zeros))
            ua = mv_chain(_after(zero, ga, 1.0), wu_v, c, n0, xcol_v, next(zeros))
            dep = ua
            gg = _round_bf16(jnp.sum(ga, axis=0, keepdims=True))
            uu = _round_bf16(jnp.sum(ua, axis=0, keepdims=True))
            h = _round_bf16(_round_bf16(gg * jax.nn.sigmoid(gg)) * uu)
            hc = _col_bcast(h)
            hcol_v[0, n0:n0 + LANES, :LANES] = hc
            hcol_v[0, n0:n0 + LANES, 2 * LANES:3 * LANES] = hc
        return dep

    def ffn_down(c, zeros):
        dep = None
        accs = []
        for n0 in range(0, D, LANES):
            dep = mv_chain(_after(y_acc[:, n0:n0 + LANES], dep), wd_v, c, n0, hcol_v, next(zeros), FC)
            y_acc[:, n0:n0 + LANES] = dep
            accs.append(dep)
        return jnp.concatenate(accs, axis=1)

    def first_half():
        for i in range(4):
            for cp in xs_copies(i):
                cp.wait()
            if i == 3:
                wr_copy.wait()
            wk_copy(i).wait()
            raw_slice(i)
            if i == 3:
                wr_f[...] = jnp.broadcast_to(wr_v[...].astype(F32).reshape(1, D), (8, D))
                dep = None
                for r0 in range(0, TB, 8):
                    _, xn_f = normalise(0, xn_v, 0, r0, 8, dep, keep=0)
                    dep = _delay(xn_f[:, D - LANES:], LN0_PACE)
        wk_copy(4).wait()
        x_copy(1, 4).wait()
        cs = cs_v[...] + jnp.sum(wk_v[KF:, :D].astype(F32).reshape((D - KF) // 8, 8, D), axis=0)
        cs_v[...] = jnp.broadcast_to(jnp.sum(cs, axis=0, keepdims=True), (8, D))
        best = (jnp.full((8, 1), -jnp.inf, F32), sub8)
        dep = None
        for r0 in range(0, TB, 16):
            dep, best = layernorm(1, xn_v, 1, r0, 16, best, dep)
        store_best(best)
        parts = [raw_last(0, c) for c in range(LEAD)]
        for c in range(NKC):
            g_unit(xn_v, 0, c * KC, (c + 1) * KC, raw_finish(0, c, parts[c], True, False), True,
                   [(dep[:8], 0, 512)] if c == NKC - 1 else [])
            if len(parts) < NKC:
                parts.append(raw_last(0, len(parts)))

        def phase_a(j, carry):
            for i in range(BA - 1):
                x_copy(BA * j + 2 + i, SEM_A + j).wait()
            for i in range(WQ_PER):
                wq_copy(WQ_PER * j + i, SEM_A + j).wait()

            @pl.when(j < NA - 1)
            def _():
                x_copy(BA * j + BA + 1, SEM_A + j).wait()

            preps = [(WQ_PER * j + i, kk) for i in range(WQ_PER) for kk in range(4)]
            k_slots = {(0, 0): [(0, 128), (512, 128)], (0, 1): [(0, 0), (512, 0), (0, 128), (512, 128)],
                       (1, 1): [(0, 0)], (2, 1): [(0, 0)]}
            g_slots = {(t, 3): [(0, 0), (0, 256), (0, 512), (0, 768)] for t in range(BA - 1)}

            def mk_ties(slots):
                return [(wq_prep(*preps.pop(0)), r0, c0) for r0, c0 in slots]

            LR = TB // NKC
            prev = None
            dep = None
            best = load_best()
            win = xn_v.at[pl.ds(BA * j + 1, BA + 1)]
            for t in range(BA):
                for c in range(NKC):
                    pk = k_unit(win, t, c * KC, (c + 1) * KC, ties=mk_ties(k_slots.get((t, c), [])))
                    if prev is not None:
                        g_unit(*prev[1:], ties=mk_ties(g_slots.get(prev[0], [])))
                    prev = ((t, c), win, t, c * KC, (c + 1) * KC, pk)
                    for r0 in range(c * LR, (c + 1) * LR, 8):
                        dep, best = layernorm(BA * j + 2 + t, win, t + 1, r0, 8, best, dep,
                                              keep=1 if t == BA - 1 else None)
            g_unit(*prev[1:], ties=[(dep, 0, 768)])
            assert not preps
            store_best(best)
            return carry

        lax.fori_loop(0, NA, phase_a, 0)

    def second_half():
        wv_copy.wait()
        wo_copy.wait()

        best0 = (jnp.full((8, 1), -jnp.inf, F32), sub8)
        dep = None
        for r0 in range(0, TB, 16):
            dep, best0 = score(xn_v[0, r0:r0 + 16, :], r0, best0, dep)
        bv, bi = load_best()
        first0 = best0[0] >= bv
        bv = jnp.where(first0, best0[0], bv)
        bi = jnp.where(first0, best0[1], bi)
        r_max = jnp.max(bv, axis=0, keepdims=True)
        idx_f = jnp.min(jnp.where(bv == r_max, bi, float(S - 1)))
        idx = jnp.clip(idx_f.astype(jnp.int32), 0, S - 1)
        blk = idx // TB
        hot_pair = blk // 2
        row16 = pl.multiple_of(((idx % TB) // 16) * 16, 16)
        gate_v[...] = jnp.broadcast_to(_round_bf16(jax.nn.sigmoid(r_max)), (16, LANES))
        row_id16 = lax.broadcasted_iota(jnp.int32, (16, D), 0)
        sel16 = row_id16 == idx % 16
        xs = xn_v[blk, pl.ds(row16, 16), :].astype(F32)
        xc = _col_bcast(jnp.sum(jnp.where(sel16, xs, 0.0), axis=0, keepdims=True))
        xcol_v[0, :, :LANES] = xc
        xcol_v[0, :, 2 * LANES:3 * LANES] = xc

        rr = lax.broadcasted_iota(jnp.int32, (LANES, LANES), 0) // DH
        cc = lax.broadcasted_iota(jnp.int32, (LANES, LANES), 1) // DH
        same_head = rr == cc

        def g_final(c, pk, dep=None):
            return (g_acc[c * KC:(c + 1) * KC, :] + _dot_tn(pk, _tie(xn_v[NB - 1], dep))).astype(BF16)

        def kv_unit(c, gf):
            out = []
            for gg in range(KC // LANES):
                g = c * (KC // LANES) + gg
                kv = _dot(gf[gg * LANES:(gg + 1) * LANES, :], wv_v[:, g * LANES:(g + 1) * LANES])
                kv = pltpu.bitcast(jnp.where(same_head, kv, 0.0).astype(BF16), U32)
                out.append(pltpu.bitcast(jnp.concatenate(_shuffle_rows(kv), axis=0), BF16))
            return out

        def m_unit(c, kvs, dep=None):
            for gg in range(KC // LANES):
                g = c * (KC // LANES) + gg
                m = _dot(kvs[gg], _tie(wo_v[g * LANES:(g + 1) * LANES, :], dep))
                dep = None
                w = pltpu.bitcast(m.astype(BF16), U32)
                for i in range(8):
                    m_v[i * 64 + g * 8:i * 64 + (g + 1) * 8, :] = w[i * 8:(i + 1) * 8, :]

        def z_prep():
            zc = pltpu.bitcast(_col_bcast(jnp.sum(z_acc[...], axis=0, keepdims=True)).astype(BF16), U32)
            vs = [_shuffle_rows(zc[g * 64:(g + 1) * 64, :]) for g in range(NG)]
            tot = None
            for i in range(NG):
                zt = pltpu.bitcast(jnp.concatenate([vs[g][i] for g in range(NG)], axis=0), BF16)
                zp = zt.astype(F32).T[:8, :]
                zp_v[:, i * LANES:(i + 1) * LANES] = zp
                tot = zp if tot is None else tot + zp
            return tot

        wq0_v[...] = pltpu.bitcast(pltpu.bitcast(wqt_v[:LANES // 2, :], BF16).T, U32)
        parts = [raw_last(NB - 1, c) for c in range(LEAD)]

        def gf(c):
            g = g_final(c, raw_finish(1, c, parts[c], False, False))
            if len(parts) < NKC:
                parts.append(raw_last(NB - 1, len(parts)))
            return g

        gf0 = gf(0)
        gf1 = gf(1)
        kv0 = kv_unit(0, gf0)
        gf2 = gf(2)
        kv1 = kv_unit(1, gf1)
        m_unit(0, kv0)
        gf3 = gf(3)
        kv2 = kv_unit(2, gf2)
        m_unit(1, kv1, xc[D - 8:])
        kv3 = kv_unit(3, gf3)
        m_unit(2, kv2, z_prep())
        m_unit(3, kv3)

        lane = lax.broadcasted_iota(jnp.int32, (8, LANES), 1)
        bit0 = lane % 2 == 0
        bit3 = (lane // 8) % 2 == 0

        def q_part(src_ref, p, ties=(), lead=False):
            wqt = _ties(pltpu.bitcast(wqt_v[...], BF16), ties)
            if lead:
                xn = src_ref[p]
                q0 = _dot(xn, pltpu.bitcast(wq0_v[...], BF16))
                q = jnp.concatenate([q0, _dot_nt(xn, wqt[LANES:])], axis=1)
            else:
                q = _dot_nt(src_ref[p], wqt)
            rows_ = []
            dep = None
            for g in range(TB // 8):
                pq = _phi(q[g * 8:(g + 1) * 8, :])
                t = pq * zp_v[...]
                s_ = t[:, :LANES]
                for n in range(1, NG):
                    s_ = s_ + t[:, n * LANES:(n + 1) * LANES]
                s_ = s_ + jnp.where(bit3, pltpu.roll(s_, LANES - 8, 1), pltpu.roll(s_, 8, 1))
                s_ = s_ + jnp.where(bit0, pltpu.roll(s_, LANES - 1, 1), pltpu.roll(s_, 1, 1))
                rinv = _after(pl.reciprocal(s_ + 1e-6, approx=True), dep)
                rows_.append(pq * jnp.concatenate([rinv] * NG, axis=1))
                dep = _delay(rinv, DELAY)
            return jnp.concatenate(rows_, axis=0).astype(BF16)

        def o_part(o, src_ref, p, b, s_out, last, dep=None):
            spans = [(0, 256), (256, 512), (512, 768), (768, 896), (896, D)] if last else \
                [(c * KC, (c + 1) * KC) for c in range(NKC)]
            for lo, hi in spans:
                m = pltpu.bitcast(m_v[:, lo:hi], BF16)
                a = _dot(o, _tie(m, dep if lo == 768 else None))
                for r0, nr in (TAIL if last and hi == D else ((0, TB),)):
                    rs = slice(r0, r0 + nr)
                    out_v[b, rs, lo:hi] = (x_v[b, rs, lo:hi].astype(F32) + a[rs]
                                           + src_ref[p, rs, lo:hi].astype(F32)).astype(BF16)
                    if last or hi == D:
                        cols = pl.ds(lo, hi - lo) if last else pl.ds(0, D)
                        pltpu.make_async_copy(out_v.at[b, pl.ds(r0, nr), cols],
                                              out_hbm.at[0, pl.ds(b * TB + r0, nr), cols],
                                              sem.at[s_out]).start()

        def phase_b(j, carry):
            for cp in ffn_copies(j, SEM_F + j):
                cp.wait()
            p = jnp.where(j == 0, hot_pair, jnp.where(j == hot_pair, 0, j))
            s_out = jnp.where(j == 0, SEM_O, SEM_O + 1)
            zeros = (lax.shift_right_logical(idx + j + k, 13) for k in range(64))
            gu_dep = ffn_gate_up(j, zeros)
            y = ffn_down(j, zeros)
            o_e = q_part(xn_v, 2 * p, lead=True)
            o_o = q_part(xn_v, 2 * p + 1, [(gu_dep, GU_TILE * LANES, 0)])
            o_part(o_e, xn_v, 2 * p, 2 * p, s_out, False)
            o_part(o_o, xn_v, 2 * p + 1, 2 * p + 1, s_out, True, y[:, D - LANES:])
            return carry

        lax.fori_loop(0, NP, phase_b, 0)

        hot = out_v.at[pl.ds(2 * hot_pair, 2)]
        pltpu.make_async_copy(hot, hot, sem.at[SEM_O]).wait()
        rows16 = pl.ds(row16, 16)
        yrow = _round_bf16(jnp.sum(y_acc[...], axis=0, keepdims=True))
        upd = jnp.where(sel16, yrow * jnp.concatenate([gate_v[...]] * NG, axis=1), 0.0)
        out_v[blk, rows16, :] = (out_v[blk, rows16, :].astype(F32) + upd).astype(BF16)
        patch = pltpu.make_async_copy(
            out_v.at[blk, rows16, :],
            out_hbm.at[0, pl.ds(pl.multiple_of(blk * TB + row16, 16), 16), :], sem.at[SEM_O])
        patch.start()
        pltpu.make_async_copy(out_v.at[pl.ds(2, NB - 2)], out_v.at[pl.ds(2, NB - 2)],
                              sem.at[SEM_O + 1]).wait()
        patch.wait()

    def outer(i, carry):
        pl.when(i == 0)(first_half)
        pl.when(i == 1)(second_half)
        return carry

    lax.fori_loop(0, 2, outer, 0)


@jax.jit
def pallas_parallel_sum__linear_attn_block__moe_arch_mod__prompt_kernel(
    A_x: jax.Array,
    A_wqkv: jax.Array,
    A_wo: jax.Array,
    B_x: jax.Array,
    B_w_r: jax.Array,
    B_w_gate: jax.Array,
    B_w_up: jax.Array,
    B_w_down: jax.Array,
):
    del B_x
    assert A_x.shape == (1, S, D) and B_w_gate.shape == (D, F)
    any_spec = pl.BlockSpec(memory_space=pl.ANY)
    scratch = [
        pltpu.VMEM((NB, TB, D), BF16),
        pltpu.VMEM((NB, TB, D), BF16),
        pltpu.VMEM((NG, D, LANES), BF16),
        pltpu.VMEM((D, D + LANES), BF16),
        pltpu.VMEM((D, D), BF16),
        pltpu.VMEM((D, D), BF16),
        pltpu.VMEM((NP, D, D), BF16),
        pltpu.VMEM((NP, D, D), BF16),
        pltpu.VMEM((NP, D, D), BF16),
        pltpu.VMEM((2, D, 4 * LANES), F32),
        pltpu.VMEM((2, D, 4 * LANES), F32),
        pltpu.VMEM((D, D), F32),
        pltpu.VMEM((D // 2, D), U32),
        pltpu.VMEM((D // 2, D), U32),
        pltpu.VMEM((NB, TB, D), BF16),
        pltpu.VMEM((D // 2, LANES), U32),
        pltpu.VMEM((2 * TB, D), F32),
        pltpu.VMEM((2, 2, TB, LANES), F32),
        pltpu.VMEM((8, D), F32),
        pltpu.VMEM((8, D), F32),
        pltpu.VMEM((8, D), F32),
        pltpu.VMEM((8, D), F32),
        pltpu.VMEM((8, D), F32),
        pltpu.VMEM((16, LANES), F32),
        pltpu.VMEM((2, 8, 1), F32),
        pltpu.VMEM((8, 1), F32),
        pltpu.VMEM((D,), BF16),
        pltpu.SemaphoreType.DMA((N_SEMS,)),
    ]
    return pl.pallas_call(
        _kernel,
        out_shape=jax.ShapeDtypeStruct((1, S, D), BF16),
        in_specs=[any_spec] * 7,
        out_specs=any_spec,
        scratch_shapes=scratch,
        compiler_params=pltpu.CompilerParams(vmem_limit_bytes=100 * 1024 * 1024,
                                             disable_semaphore_checks=True, disable_bounds_checks=True),
    )(A_x, A_wqkv, A_wo, B_w_r, B_w_gate, B_w_up, B_w_down)
```

```python
import jax
import jax.numpy as jnp
from jax import lax
import jax.experimental.pallas as pl
import jax.experimental.pallas.tpu as pltpu

F32 = jnp.float32
BF16 = jnp.bfloat16
U32 = jnp.uint32

S = 2048
D = 1024
F = 3584
DH = 32
TB = 256
NB = S // TB
NP = NB // 2
FC = F // NP
LANES = 128
NG = D // LANES
HG = LANES // DH
KC = 256
NKC = D // KC
K_SPLITS = (0, 128, 256, 512, 768, 1024)
X_SPLITS = (0, 128, 256, 512, 1024)
KF = K_SPLITS[-2]
LN0_PACE = 4
PHI_PACE = 1
LEAD = 4
NA = 2
BA = (NB - 2) // NA
WQ_PER = NG // NA
DELAY = 8
GU_TILE = 2
TAIL = ((0, 128), (128, 128))
SEM_A = 5
SEM_W = SEM_A + NA
SEM_F = SEM_W + 1
SEM_O = SEM_F + NP
N_SEMS = SEM_O + 2


def _round_bf16(v):
    return v.astype(BF16).astype(F32)


def _phi(t):
    return jnp.where(t > 0, t + 1.0, jnp.exp(t)) + 1e-6


def _dot(a, b):
    return jnp.dot(a, b, preferred_element_type=F32)


def _dot_tn(a, b):
    return lax.dot_general(a, b, (((0,), (0,)), ((), ())), preferred_element_type=F32)


def _dot_nt(a, b):
    return lax.dot_general(a, b, (((1,), (1,)), ((), ())), preferred_element_type=F32)


def _after(v, dep, other=0.0):
    if dep is None:
        return v
    return jnp.where(dep > jnp.inf, other, v)


def _tie(w, dep, r0=0, c0=0):
    if dep is None:
        return w
    dep = jnp.broadcast_to(dep, (8, LANES))
    head = pltpu.bitcast(w[r0:r0 + 16, c0:c0 + LANES], U32) | (dep > jnp.inf).astype(U32)
    row = [pltpu.bitcast(head, BF16)]
    if c0:
        row = [w[r0:r0 + 16, :c0]] + row
    if c0 + LANES < w.shape[1]:
        row = row + [w[r0:r0 + 16, c0 + LANES:]]
    head = row[0] if len(row) == 1 else jnp.concatenate(row, axis=1)
    parts = ([w[:r0]] if r0 else []) + [head, w[r0 + 16:]]
    return jnp.concatenate(parts, axis=0)


def _ties(w, ties):
    for dep, r0, c0 in ties:
        w = _tie(w, dep, r0, c0)
    return w


def _shuffle_rows(w):
    sub = lax.broadcasted_iota(jnp.int32, (8, w.shape[1]), 0)
    v = [w[(a % 4) * 16 + (a // 4) * 8:(a % 4) * 16 + (a // 4) * 8 + 8] for a in range(8)]
    for d in (4, 2, 1):
        low = (sub & d) == 0
        nv = list(v)
        for a in range(8):
            if a & d == 0:
                nv[a] = jnp.where(low, v[a], pltpu.roll(v[a + d], d, 0))
                nv[a + d] = jnp.where(low, pltpu.roll(v[a], 8 - d, 0), v[a + d])
        v = nv
    return v


def _delay(v, n):
    for _ in range(n):
        v = pl.reciprocal(v, approx=True)
    return v


def _col_bcast(row):
    tiles = [jnp.broadcast_to(row[:, t * LANES:(t + 1) * LANES], (LANES, LANES)).T
             for t in range(row.shape[1] // LANES)]
    return jnp.concatenate(tiles, axis=0)


def _kernel(x_hbm, wqkv_hbm, wo_hbm, wr_hbm, wg_hbm, wu_hbm, wd_hbm, out_hbm,
            x_v, xn_v, wq_v, wk_v, wv_v, wo_v, wg_v, wu_v, wd_v, xcol_v, hcol_v,
            g_acc, m_v, wqt_v, out_v, wq0_v, kraw_v, st_v, cs_v, wr_f, z_acc, zp_v, y_acc, gate_v, best_v, junk_v, wr_v,
            sem):
    def x_copy(b, s_):
        return pltpu.make_async_copy(x_hbm.at[0, pl.ds(b * TB, TB), :], x_v.at[b], sem.at[s_])

    def xs_copies(i):
        cols = pl.ds(X_SPLITS[i], X_SPLITS[i + 1] - X_SPLITS[i])
        return [pltpu.make_async_copy(x_hbm.at[0, pl.ds(b * TB, TB), cols], x_v.at[b, :, cols],
                                      sem.at[i]) for b in (0, NB - 1)]

    def wk_copy(i):
        rows = pl.ds(K_SPLITS[i], K_SPLITS[i + 1] - K_SPLITS[i])
        return pltpu.make_async_copy(wqkv_hbm.at[rows, pl.ds(D, D)], wk_v.at[rows, pl.ds(0, D)],
                                     sem.at[i])

    def wq_copy(g, s_):
        cols = pl.ds(pl.multiple_of(g * LANES, LANES), LANES)
        return pltpu.make_async_copy(wqkv_hbm.at[:, cols], wq_v.at[g], sem.at[s_])

    wr_copy = pltpu.make_async_copy(wr_hbm, wr_v, sem.at[3])
    wv_copy = pltpu.make_async_copy(wqkv_hbm.at[:, pl.ds(2 * D, D)], wv_v, sem.at[SEM_W])
    wo_copy = pltpu.make_async_copy(wo_hbm, wo_v, sem.at[SEM_W])

    def ffn_copies(c, s_):
        span = pl.ds(pl.multiple_of(c * FC, LANES), FC)
        return (
            pltpu.make_async_copy(wg_hbm.at[:, span], wg_v.at[c, :, pl.ds(0, FC)], sem.at[s_]),
            pltpu.make_async_copy(wu_hbm.at[:, span], wu_v.at[c, :, pl.ds(0, FC)], sem.at[s_]),
            pltpu.make_async_copy(wd_hbm.at[span, :], wd_v.at[c, pl.ds(0, FC), :], sem.at[s_]),
        )

    for i in range(len(K_SPLITS) - 1):
        if i < len(X_SPLITS) - 1:
            for cp in xs_copies(i):
                cp.start()
        if i == 3:
            wr_copy.start()
        wk_copy(i).start()
    x_copy(1, 4).start()
    for j in range(NA):
        for b in range(BA * j + 2, min(BA * (j + 1) + 2, NB - 1)):
            x_copy(b, SEM_A + j).start()
        for g in range(WQ_PER * j, WQ_PER * (j + 1)):
            wq_copy(g, SEM_A + j).start()
    wv_copy.start()
    wo_copy.start()
    for c in range(NP):
        for cp in ffn_copies(c, SEM_F + c):
            cp.start()

    y_acc[...] = jnp.zeros_like(y_acc)
    sub8 = lax.broadcasted_iota(jnp.int32, (8, 1), 0).astype(F32)

    def normalise(b, dst_ref, j, r0, nr, dep=None, keep=None):
        rs = pl.ds(r0, nr)
        mean = jnp.mean(x_v[b, rs, :].astype(F32), axis=-1, keepdims=True)
        mean_b = jnp.broadcast_to(_round_bf16(mean), (nr, LANES))
        junk_v[...] = mean[:8]
        c = x_v[b, rs, :].astype(F32) - mean
        var = jnp.mean(c * c, axis=-1, keepdims=True)
        junk_v[...] = var[:8]
        rstd = 1.0 / _round_bf16(jnp.sqrt(_round_bf16(_round_bf16(var) + 1e-5)))
        if keep is not None:
            st_v[keep, 0, rs, :] = mean_b
            st_v[keep, 1, rs, :] = jnp.broadcast_to(rstd, (nr, LANES))
        mean_b = jnp.concatenate([_after(mean_b, dep)] * NG, axis=1)
        xn_f = _round_bf16(x_v[b, rs, :].astype(F32) - mean_b) * rstd
        xn = xn_f.astype(BF16)
        dst_ref[j, rs, :] = xn
        return xn, xn_f

    def score(xn, row0, best, dep=None):
        nr = xn.shape[0]
        wr = wr_f[...]
        if dep is not None:
            wr = jnp.concatenate([_after(wr[:, :LANES], dep[:8]), wr[:, LANES:]], axis=1)
        if nr > 8:
            wr = jnp.concatenate([wr] * (nr // 8), axis=0)
        r = jnp.sum(xn.astype(F32) * wr, axis=-1, keepdims=True)
        rb = _round_bf16(r)
        bv, bi = best
        for q in range(nr // 8):
            rq = rb[q * 8:(q + 1) * 8]
            better = rq > bv
            bv = jnp.where(better, rq, bv)
            bi = jnp.where(better, sub8 + jnp.asarray(row0 + q * 8).astype(F32), bi)
        return r, (bv, bi)

    def layernorm(b, dst_ref, j, r0, nr, best, dep=None, keep=None):
        return score(normalise(b, dst_ref, j, r0, nr, dep, keep)[0], b * TB + r0, best)

    def load_best():
        return best_v[0], best_v[1]

    def store_best(best):
        best_v[0] = best[0]
        best_v[1] = best[1]

    def k_unit(src_ref, j, lo, hi, first=False, ties=()):
        pk = _phi(_dot(src_ref[j], _ties(wk_v[:, lo:hi], ties)))
        zs = jnp.sum(pk.reshape(TB // 8, 8, hi - lo), axis=0)
        if first:
            z_acc[:, lo:hi] = zs
        else:
            z_acc[:, lo:hi] += zs
        return pk.astype(BF16)

    def raw_slice(i):
        lo, hi = K_SPLITS[i], K_SPLITS[i + 1]
        xs = jnp.concatenate([x_v[0, :, lo:hi], x_v[NB - 1, :, lo:hi]], axis=0)
        part = _dot(xs, wk_v[lo:hi, :D])
        if i == 0:
            kraw_v[...] = part
        else:
            kraw_v[...] += part
        if i == 2:
            cs_v[...] = jnp.sum(wk_v[:hi, :D].astype(F32).reshape(hi // 8, 8, D), axis=0)
        elif i > 2:
            cs_v[...] += jnp.sum(wk_v[lo:hi, :D].astype(F32).reshape((hi - lo) // 8, 8, D), axis=0)

    def raw_last(b, c):
        return _dot(x_v[b, :, KF:], wk_v[KF:, c * KC:(c + 1) * KC])

    def raw_finish(slot, c, part, first, paced):
        cs = slice(c * KC, (c + 1) * KC)
        rows_ = []
        dep = None
        zs = None
        for r0 in range(0, TB, 16):
            mean = st_v[slot, 0, r0:r0 + 16, :]
            rstd = _after(st_v[slot, 1, r0:r0 + 16, :], dep)
            mean = jnp.concatenate([mean] * (KC // LANES), axis=1)
            rstd = jnp.concatenate([rstd] * (KC // LANES), axis=1)
            col = jnp.concatenate([cs_v[:, cs]] * 2, axis=0)
            k = (kraw_v[slot * TB + r0:slot * TB + r0 + 16, cs] + part[r0:r0 + 16] - mean * col) * rstd
            pk = _phi(k)
            z2 = pk[:8] + pk[8:]
            zs = z2 if zs is None else zs + z2
            if paced:
                f = _delay(z2[:, :LANES] + z2[:, LANES:], PHI_PACE)
                dep = jnp.concatenate([f, f], axis=0)
            rows_.append(pk.astype(BF16))
        if first:
            z_acc[:, cs] = zs
        else:
            z_acc[:, cs] += zs
        return jnp.concatenate(rows_, axis=0)

    def g_unit(src_ref, j, lo, hi, pk, first=False, ties=()):
        g = _dot_tn(pk, _ties(src_ref[j], ties))
        if first:
            g_acc[lo:hi, :] = g
        else:
            g_acc[lo:hi, :] += g

    def wq_prep(g, kk):
        v = _shuffle_rows(pltpu.bitcast(wq_v[g, kk * 256:(kk + 1) * 256, :].T, U32))
        base = pl.multiple_of(g * 8, 8)
        tot = None
        for i in range(8):
            wqt_v[pl.ds(i * 64 + base, 8), kk * 256:(kk + 1) * 256] = v[i]
            tot = v[i] if tot is None else tot | v[i]
        return pltpu.bitcast(tot[:, :LANES] | tot[:, LANES:], F32)

    def mv_chain(acc, w_ref, c, n0, col_ref, z0, k=D):
        cp = 2 * LANES if (n0 // 256) % 4 < 2 else 0
        cz = c + z0

        def step(i, acc):
            rows = pl.ds(pl.multiple_of(i * 8, 8), 8)
            return acc + w_ref[cz, rows, n0:n0 + LANES].astype(F32) * col_ref[z0, rows, cp:cp + LANES]
        return lax.fori_loop(0, k // 8, step, acc, unroll=True)

    def ffn_gate_up(c, zeros):
        dep = None
        zero = jnp.zeros((8, LANES), F32)
        for n0 in range(0, FC, LANES):
            ga = mv_chain(_after(zero, dep, 1.0), wg_v, c, n0, xcol_v, next(zeros))
            ua = mv_chain(_after(zero, ga, 1.0), wu_v, c, n0, xcol_v, next(zeros))
            dep = ua
            gg = _round_bf16(jnp.sum(ga, axis=0, keepdims=True))
            uu = _round_bf16(jnp.sum(ua, axis=0, keepdims=True))
            h = _round_bf16(_round_bf16(gg * jax.nn.sigmoid(gg)) * uu)
            hc = _col_bcast(h)
            hcol_v[0, n0:n0 + LANES, :LANES] = hc
            hcol_v[0, n0:n0 + LANES, 2 * LANES:3 * LANES] = hc
        return dep

    def ffn_down(c, zeros):
        dep = None
        accs = []
        for n0 in range(0, D, LANES):
            dep = mv_chain(_after(y_acc[:, n0:n0 + LANES], dep), wd_v, c, n0, hcol_v, next(zeros), FC)
            y_acc[:, n0:n0 + LANES] = dep
            accs.append(dep)
        return jnp.concatenate(accs, axis=1)

    def first_half():
        for i in range(4):
            for cp in xs_copies(i):
                cp.wait()
            if i == 3:
                wr_copy.wait()
            wk_copy(i).wait()
            raw_slice(i)
            if i == 3:
                wr_f[...] = jnp.broadcast_to(wr_v[...].astype(F32).reshape(1, D), (8, D))
                dep = None
                for r0 in range(0, TB, 8):
                    _, xn_f = normalise(0, xn_v, 0, r0, 8, dep, keep=0)
                    dep = _delay(xn_f[:, D - LANES:], LN0_PACE)
        wk_copy(4).wait()
        x_copy(1, 4).wait()
        cs = cs_v[...] + jnp.sum(wk_v[KF:, :D].astype(F32).reshape((D - KF) // 8, 8, D), axis=0)
        cs_v[...] = jnp.broadcast_to(jnp.sum(cs, axis=0, keepdims=True), (8, D))
        best = (jnp.full((8, 1), -jnp.inf, F32), sub8)
        dep = None
        for r0 in range(0, TB, 16):
            dep, best = layernorm(1, xn_v, 1, r0, 16, best, dep)
        store_best(best)
        parts = [raw_last(0, c) for c in range(LEAD)]
        for c in range(NKC):
            g_unit(xn_v, 0, c * KC, (c + 1) * KC, raw_finish(0, c, parts[c], True, False), True,
                   [(dep[:8], 0, 512)] if c == NKC - 1 else [])
            if len(parts) < NKC:
                parts.append(raw_last(0, len(parts)))

        def phase_a(j, carry):
            for i in range(BA - 1):
                x_copy(BA * j + 2 + i, SEM_A + j).wait()
            for i in range(WQ_PER):
                wq_copy(WQ_PER * j + i, SEM_A + j).wait()

            @pl.when(j < NA - 1)
            def _():
                x_copy(BA * j + BA + 1, SEM_A + j).wait()

            preps = [(WQ_PER * j + i, kk) for i in range(WQ_PER) for kk in range(4)]
            k_slots = {(0, 0): [(0, 128), (512, 128)], (0, 1): [(0, 0), (512, 0), (0, 128), (512, 128)],
                       (1, 1): [(0, 0)], (2, 1): [(0, 0)]}
            g_slots = {(t, 3): [(0, 0), (0, 256), (0, 512), (0, 768)] for t in range(BA - 1)}

            def mk_ties(slots):
                return [(wq_prep(*preps.pop(0)), r0, c0) for r0, c0 in slots]

            LR = TB // NKC
            prev = None
            dep = None
            best = load_best()
            win = xn_v.at[pl.ds(BA * j + 1, BA + 1)]
            for t in range(BA):
                for c in range(NKC):
                    pk = k_unit(win, t, c * KC, (c + 1) * KC, ties=mk_ties(k_slots.get((t, c), [])))
                    if prev is not None:
                        g_unit(*prev[1:], ties=mk_ties(g_slots.get(prev[0], [])))
                    prev = ((t, c), win, t, c * KC, (c + 1) * KC, pk)
                    for r0 in range(c * LR, (c + 1) * LR, 8):
                        dep, best = layernorm(BA * j + 2 + t, win, t + 1, r0, 8, best, dep,
                                              keep=1 if t == BA - 1 else None)
            g_unit(*prev[1:], ties=[(dep, 0, 768)])
            assert not preps
            store_best(best)
            return carry

        lax.fori_loop(0, NA, phase_a, 0)

    def second_half():
        wv_copy.wait()
        wo_copy.wait()

        best0 = (jnp.full((8, 1), -jnp.inf, F32), sub8)
        dep = None
        for r0 in range(0, TB, 16):
            dep, best0 = score(xn_v[0, r0:r0 + 16, :], r0, best0, dep)
        bv, bi = load_best()
        first0 = best0[0] >= bv
        bv = jnp.where(first0, best0[0], bv)
        bi = jnp.where(first0, best0[1], bi)
        r_max = jnp.max(bv, axis=0, keepdims=True)
        idx_f = jnp.min(jnp.where(bv == r_max, bi, float(S - 1)))
        idx = jnp.clip(idx_f.astype(jnp.int32), 0, S - 1)
        blk = idx // TB
        hot_pair = blk // 2
        row16 = pl.multiple_of(((idx % TB) // 16) * 16, 16)
        gate_v[...] = jnp.broadcast_to(_round_bf16(jax.nn.sigmoid(r_max)), (16, LANES))
        row_id16 = lax.broadcasted_iota(jnp.int32, (16, D), 0)
        sel16 = row_id16 == idx % 16
        xs = xn_v[blk, pl.ds(row16, 16), :].astype(F32)
        xc = _col_bcast(jnp.sum(jnp.where(sel16, xs, 0.0), axis=0, keepdims=True))
        xcol_v[0, :, :LANES] = xc
        xcol_v[0, :, 2 * LANES:3 * LANES] = xc

        rr = lax.broadcasted_iota(jnp.int32, (LANES, LANES), 0) // DH
        cc = lax.broadcasted_iota(jnp.int32, (LANES, LANES), 1) // DH
        same_head = rr == cc

        def g_final(c, pk, dep=None):
            return (g_acc[c * KC:(c + 1) * KC, :] + _dot_tn(pk, _tie(xn_v[NB - 1], dep))).astype(BF16)

        def kv_unit(c, gf):
            out = []
            for gg in range(KC // LANES):
                g = c * (KC // LANES) + gg
                kv = _dot(gf[gg * LANES:(gg + 1) * LANES, :], wv_v[:, g * LANES:(g + 1) * LANES])
                kv = pltpu.bitcast(jnp.where(same_head, kv, 0.0).astype(BF16), U32)
                out.append(pltpu.bitcast(jnp.concatenate(_shuffle_rows(kv), axis=0), BF16))
            return out

        def m_unit(c, kvs, dep=None):
            for gg in range(KC // LANES):
                g = c * (KC // LANES) + gg
                m = _dot(kvs[gg], _tie(wo_v[g * LANES:(g + 1) * LANES, :], dep))
                dep = None
                w = pltpu.bitcast(m.astype(BF16), U32)
                for i in range(8):
                    m_v[i * 64 + g * 8:i * 64 + (g + 1) * 8, :] = w[i * 8:(i + 1) * 8, :]

        def z_prep():
            zc = pltpu.bitcast(_col_bcast(jnp.sum(z_acc[...], axis=0, keepdims=True)).astype(BF16), U32)
            vs = [_shuffle_rows(zc[g * 64:(g + 1) * 64, :]) for g in range(NG)]
            tot = None
            for i in range(NG):
                zt = pltpu.bitcast(jnp.concatenate([vs[g][i] for g in range(NG)], axis=0), BF16)
                zp = zt.astype(F32).T[:8, :]
                zp_v[:, i * LANES:(i + 1) * LANES] = zp
                tot = zp if tot is None else tot + zp
            return tot

        wq0_v[...] = pltpu.bitcast(pltpu.bitcast(wqt_v[:LANES // 2, :], BF16).T, U32)
        parts = [raw_last(NB - 1, c) for c in range(LEAD)]

        def gf(c):
            g = g_final(c, raw_finish(1, c, parts[c], False, False))
            if len(parts) < NKC:
                parts.append(raw_last(NB - 1, len(parts)))
            return g

        gf0 = gf(0)
        gf1 = gf(1)
        kv0 = kv_unit(0, gf0)
        gf2 = gf(2)
        kv1 = kv_unit(1, gf1)
        m_unit(0, kv0)
        gf3 = gf(3)
        kv2 = kv_unit(2, gf2)
        m_unit(1, kv1, xc[D - 8:])
        kv3 = kv_unit(3, gf3)
        m_unit(2, kv2, z_prep())
        m_unit(3, kv3)

        lane = lax.broadcasted_iota(jnp.int32, (8, LANES), 1)
        bit0 = lane % 2 == 0
        bit3 = (lane // 8) % 2 == 0

        def q_part(src_ref, p, ties=(), lead=False):
            wqt = _ties(pltpu.bitcast(wqt_v[...], BF16), ties)
            if lead:
                xn = src_ref[p]
                q0 = _dot(xn, pltpu.bitcast(wq0_v[...], BF16))
                q = jnp.concatenate([q0, _dot_nt(xn, wqt[LANES:])], axis=1)
            else:
                q = _dot_nt(src_ref[p], wqt)
            rows_ = []
            dep = None
            for g in range(TB // 8):
                pq = _phi(q[g * 8:(g + 1) * 8, :])
                t = pq * zp_v[...]
                s_ = t[:, :LANES]
                for n in range(1, NG):
                    s_ = s_ + t[:, n * LANES:(n + 1) * LANES]
                s_ = s_ + jnp.where(bit3, pltpu.roll(s_, LANES - 8, 1), pltpu.roll(s_, 8, 1))
                s_ = s_ + jnp.where(bit0, pltpu.roll(s_, LANES - 1, 1), pltpu.roll(s_, 1, 1))
                rinv = _after(pl.reciprocal(s_ + 1e-6, approx=True), dep)
                rows_.append(pq * jnp.concatenate([rinv] * NG, axis=1))
                dep = _delay(rinv, DELAY)
            return jnp.concatenate(rows_, axis=0).astype(BF16)

        def o_part(o, b, slot, s_out, last, dep=None):
            spans = [(0, 256), (256, 512), (512, 768), (768, 896), (896, D)] if last else \
                [(c * KC, (c + 1) * KC) for c in range(NKC)]
            for lo, hi in spans:
                m = pltpu.bitcast(m_v[:, lo:hi], BF16)
                a = _dot(o, _tie(m, dep if lo == 768 else None))
                for r0, nr in (TAIL if last and hi == D else ((0, TB),)):
                    rs = slice(r0, r0 + nr)
                    out_v[slot, rs, lo:hi] = (x_v[b, rs, lo:hi].astype(F32) + a[rs]
                                              + xn_v[b, rs, lo:hi].astype(F32)).astype(BF16)
                    if last or hi == D:
                        cols = pl.ds(lo, hi - lo) if last else pl.ds(0, D)
                        pltpu.make_async_copy(out_v.at[slot, pl.ds(r0, nr), cols],
                                              out_hbm.at[0, pl.ds(b * TB + r0, nr), cols],
                                              sem.at[s_out]).start()

        def phase_b(j, carry):
            for cp in ffn_copies(j, SEM_F + j):
                cp.wait()
            p = jnp.where(j == 0, hot_pair, jnp.where(j == hot_pair, 0, j))
            s_out = jnp.where(j == 0, SEM_O, SEM_O + 1)
            zeros = (lax.shift_right_logical(idx + j + k, 13) for k in range(64))
            gu_dep = ffn_gate_up(j, zeros)
            y = ffn_down(j, zeros)
            o_e = q_part(xn_v, 2 * p, lead=True)
            o_o = q_part(xn_v, 2 * p + 1, [(gu_dep, GU_TILE * LANES, 0)])
            o_part(o_e, 2 * p, 2 * j, s_out, False)
            o_part(o_o, 2 * p + 1, 2 * j + 1, s_out, True, y[:, D - LANES:])
            return carry

        lax.fori_loop(0, NP, phase_b, 0)

        hot = out_v.at[pl.ds(0, 2)]
        pltpu.make_async_copy(hot, hot, sem.at[SEM_O]).wait()
        rows16 = pl.ds(row16, 16)
        yrow = _round_bf16(jnp.sum(y_acc[...], axis=0, keepdims=True))
        upd = jnp.where(sel16, yrow * jnp.concatenate([gate_v[...]] * NG, axis=1), 0.0)
        out_v[blk % 2, rows16, :] = (out_v[blk % 2, rows16, :].astype(F32) + upd).astype(BF16)
        patch = pltpu.make_async_copy(
            out_v.at[blk % 2, rows16, :],
            out_hbm.at[0, pl.ds(pl.multiple_of(blk * TB + row16, 16), 16), :], sem.at[SEM_O])
        patch.start()
        pltpu.make_async_copy(out_v.at[pl.ds(2, NB - 2)], out_v.at[pl.ds(2, NB - 2)],
                              sem.at[SEM_O + 1]).wait()
        patch.wait()

    def outer(i, carry):
        pl.when(i == 0)(first_half)
        pl.when(i == 1)(second_half)
        return carry

    lax.fori_loop(0, 2, outer, 0)


@jax.jit
def pallas_parallel_sum__linear_attn_block__moe_arch_mod__prompt_kernel(
    A_x: jax.Array,
    A_wqkv: jax.Array,
    A_wo: jax.Array,
    B_x: jax.Array,
    B_w_r: jax.Array,
    B_w_gate: jax.Array,
    B_w_up: jax.Array,
    B_w_down: jax.Array,
):
    del B_x
    assert A_x.shape == (1, S, D) and B_w_gate.shape == (D, F)
    any_spec = pl.BlockSpec(memory_space=pl.ANY)
    scratch = [
        pltpu.VMEM((NB, TB, D), BF16),
        pltpu.VMEM((NB, TB, D), BF16),
        pltpu.VMEM((NG, D, LANES), BF16),
        pltpu.VMEM((D, D + LANES), BF16),
        pltpu.VMEM((D, D), BF16),
        pltpu.VMEM((D, D), BF16),
        pltpu.VMEM((NP, D, D), BF16),
        pltpu.VMEM((NP, D, D), BF16),
        pltpu.VMEM((NP, D, D), BF16),
        pltpu.VMEM((2, D, 4 * LANES), F32),
        pltpu.VMEM((2, D, 4 * LANES), F32),
        pltpu.VMEM((D, D), F32),
        pltpu.VMEM((D // 2, D), U32),
        pltpu.VMEM((D // 2, D), U32),
        pltpu.VMEM((NB, TB, D), BF16),
        pltpu.VMEM((D // 2, LANES), U32),
        pltpu.VMEM((2 * TB, D), F32),
        pltpu.VMEM((2, 2, TB, LANES), F32),
        pltpu.VMEM((8, D), F32),
        pltpu.VMEM((8, D), F32),
        pltpu.VMEM((8, D), F32),
        pltpu.VMEM((8, D), F32),
        pltpu.VMEM((8, D), F32),
        pltpu.VMEM((16, LANES), F32),
        pltpu.VMEM((2, 8, 1), F32),
        pltpu.VMEM((8, 1), F32),
        pltpu.VMEM((D,), BF16),
        pltpu.SemaphoreType.DMA((N_SEMS,)),
    ]
    return pl.pallas_call(
        _kernel,
        out_shape=jax.ShapeDtypeStruct((1, S, D), BF16),
        in_specs=[any_spec] * 7,
        out_specs=any_spec,
        scratch_shapes=scratch,
        compiler_params=pltpu.CompilerParams(vmem_limit_bytes=100 * 1024 * 1024,
                                             disable_semaphore_checks=True, disable_bounds_checks=True),
    )(A_x, A_wqkv, A_wo, B_w_r, B_w_gate, B_w_up, B_w_down)
```

```python
import jax
import jax.numpy as jnp
from jax import lax
import jax.experimental.pallas as pl
import jax.experimental.pallas.tpu as pltpu

F32 = jnp.float32
BF16 = jnp.bfloat16
U32 = jnp.uint32

S = 2048
D = 1024
F = 3584
DH = 32
TB = 256
NB = S // TB
NP = NB // 2
FC = F // NP
LANES = 128
NG = D // LANES
KC = 256
NKC = D // KC
K_SPLITS = (0, 128, 256, 512, 768, 1024)
X_SPLITS = (0, 128, 256, 512, 1024)
KF = K_SPLITS[-2]
NA = 2
BA = (NB - 2) // NA
WQ_PER = NG // NA
LN0_PACE = 4
DEN_PACE = 8
GU_TILE = 2
TAIL = ((0, 128), (128, 128))
SEM_A = len(K_SPLITS) - 1
SEM_W = SEM_A + NA
SEM_F = SEM_W + 1
SEM_O = SEM_F + NP
N_SEMS = SEM_O + 2


def _round_bf16(v):
    return v.astype(BF16).astype(F32)


def _phi(t):
    return jnp.where(t > 0, t + 1.0, jnp.exp(t)) + 1e-6


def _dot(a, b):
    return jnp.dot(a, b, preferred_element_type=F32)


def _dot_tn(a, b):
    return lax.dot_general(a, b, (((0,), (0,)), ((), ())), preferred_element_type=F32)


def _dot_nt(a, b):
    return lax.dot_general(a, b, (((1,), (1,)), ((), ())), preferred_element_type=F32)


def _after(v, dep, other=0.0):
    if dep is None:
        return v
    return jnp.where(dep > jnp.inf, other, v)


def _tie(w, dep, r0=0, c0=0):
    if dep is None:
        return w
    dep = jnp.broadcast_to(dep, (8, LANES))
    head = pltpu.bitcast(w[r0:r0 + 16, c0:c0 + LANES], U32) | (dep > jnp.inf).astype(U32)
    row = [pltpu.bitcast(head, BF16)]
    if c0:
        row = [w[r0:r0 + 16, :c0]] + row
    if c0 + LANES < w.shape[1]:
        row = row + [w[r0:r0 + 16, c0 + LANES:]]
    head = row[0] if len(row) == 1 else jnp.concatenate(row, axis=1)
    parts = ([w[:r0]] if r0 else []) + [head, w[r0 + 16:]]
    return jnp.concatenate(parts, axis=0)


def _ties(w, ties):
    for dep, r0, c0 in ties:
        w = _tie(w, dep, r0, c0)
    return w


def _shuffle_rows(w):
    sub = lax.broadcasted_iota(jnp.int32, (8, w.shape[1]), 0)
    v = [w[(a % 4) * 16 + (a // 4) * 8:(a % 4) * 16 + (a // 4) * 8 + 8] for a in range(8)]
    for d in (4, 2, 1):
        low = (sub & d) == 0
        nv = list(v)
        for a in range(8):
            if a & d == 0:
                nv[a] = jnp.where(low, v[a], pltpu.roll(v[a + d], d, 0))
                nv[a + d] = jnp.where(low, pltpu.roll(v[a], 8 - d, 0), v[a + d])
        v = nv
    return v


def _delay(v, n):
    for _ in range(n):
        v = pl.reciprocal(v, approx=True)
    return v


def _col_bcast(row):
    tiles = [jnp.broadcast_to(row[:, t * LANES:(t + 1) * LANES], (LANES, LANES)).T
             for t in range(row.shape[1] // LANES)]
    return jnp.concatenate(tiles, axis=0)


def _kernel(x_hbm, wqkv_hbm, wo_hbm, wr_hbm, wg_hbm, wu_hbm, wd_hbm, out_hbm,
            x_v, xn_v, wq_v, wk_v, wv_v, wo_v, wg_v, wu_v, wd_v, xcol_v, hcol_v,
            g_acc, m_v, wqt_v, out_v, wq0_v, kraw_v, st_v, cs_v, wr_f, z_acc, zp_v, y_acc,
            gate_v, best_v, junk_v, wr_v, sem):
    def x_copy(b, s_):
        return pltpu.make_async_copy(x_hbm.at[0, pl.ds(b * TB, TB), :], x_v.at[b], sem.at[s_])

    def xs_copies(i):
        spans = [(NB - 1, K_SPLITS[i], K_SPLITS[i + 1])]
        if i < len(X_SPLITS) - 1:
            spans = [(0, X_SPLITS[i], X_SPLITS[i + 1])] + spans
        return [pltpu.make_async_copy(x_hbm.at[0, pl.ds(b * TB, TB), pl.ds(lo, hi - lo)],
                                      x_v.at[b, :, pl.ds(lo, hi - lo)], sem.at[i])
                for b, lo, hi in spans]

    def wk_copy(i):
        rows = pl.ds(K_SPLITS[i], K_SPLITS[i + 1] - K_SPLITS[i])
        return pltpu.make_async_copy(wqkv_hbm.at[rows, pl.ds(D, D)], wk_v.at[rows, pl.ds(0, D)],
                                     sem.at[i])

    def wq_copy(g, s_):
        cols = pl.ds(pl.multiple_of(g * LANES, LANES), LANES)
        return pltpu.make_async_copy(wqkv_hbm.at[:, cols], wq_v.at[g], sem.at[s_])

    wr_copy = pltpu.make_async_copy(wr_hbm, wr_v, sem.at[3])
    wv_copy = pltpu.make_async_copy(wqkv_hbm.at[:, pl.ds(2 * D, D)], wv_v, sem.at[SEM_W])
    wo_copy = pltpu.make_async_copy(wo_hbm, wo_v, sem.at[SEM_W])

    def ffn_copies(c, s_):
        span = pl.ds(pl.multiple_of(c * FC, LANES), FC)
        return (
            pltpu.make_async_copy(wg_hbm.at[:, span], wg_v.at[c, :, pl.ds(0, FC)], sem.at[s_]),
            pltpu.make_async_copy(wu_hbm.at[:, span], wu_v.at[c, :, pl.ds(0, FC)], sem.at[s_]),
            pltpu.make_async_copy(wd_hbm.at[span, :], wd_v.at[c, pl.ds(0, FC), :], sem.at[s_]),
        )

    for i in range(len(K_SPLITS) - 1):
        for cp in xs_copies(i):
            cp.start()
        if i == 3:
            wr_copy.start()
        wk_copy(i).start()
    x_copy(1, 4).start()
    for j in range(NA):
        for b in range(BA * j + 2, min(BA * (j + 1) + 2, NB - 1)):
            x_copy(b, SEM_A + j).start()
        for g in range(WQ_PER * j, WQ_PER * (j + 1)):
            wq_copy(g, SEM_A + j).start()
    wv_copy.start()
    wo_copy.start()
    for c in range(NP):
        for cp in ffn_copies(c, SEM_F + c):
            cp.start()

    y_acc[...] = jnp.zeros_like(y_acc)
    sub8 = lax.broadcasted_iota(jnp.int32, (8, 1), 0).astype(F32)

    def normalise(b, dst_ref, j, r0, nr, dep=None, keep=None):
        rs = pl.ds(r0, nr)
        mean = jnp.mean(x_v[b, rs, :].astype(F32), axis=-1, keepdims=True)
        mean_b = jnp.broadcast_to(_round_bf16(mean), (nr, LANES))
        junk_v[...] = mean[:8]
        c = x_v[b, rs, :].astype(F32) - mean
        var = jnp.mean(c * c, axis=-1, keepdims=True)
        junk_v[...] = var[:8]
        rstd = 1.0 / _round_bf16(jnp.sqrt(_round_bf16(_round_bf16(var) + 1e-5)))
        if keep is not None:
            st_v[keep, 0, rs, :] = mean_b
            st_v[keep, 1, rs, :] = jnp.broadcast_to(rstd, (nr, LANES))
        mean_b = jnp.concatenate([_after(mean_b, dep)] * NG, axis=1)
        xn_f = _round_bf16(x_v[b, rs, :].astype(F32) - mean_b) * rstd
        xn = xn_f.astype(BF16)
        dst_ref[j, rs, :] = xn
        return xn, xn_f

    def score(xn, row0, best, dep=None):
        nr = xn.shape[0]
        wr = wr_f[...]
        if dep is not None:
            wr = jnp.concatenate([_after(wr[:, :LANES], dep[:8]), wr[:, LANES:]], axis=1)
        if nr > 8:
            wr = jnp.concatenate([wr] * (nr // 8), axis=0)
        r = jnp.sum(xn.astype(F32) * wr, axis=-1, keepdims=True)
        rb = _round_bf16(r)
        bv, bi = best
        for q in range(nr // 8):
            rq = rb[q * 8:(q + 1) * 8]
            better = rq > bv
            bv = jnp.where(better, rq, bv)
            bi = jnp.where(better, sub8 + jnp.asarray(row0 + q * 8).astype(F32), bi)
        return r, (bv, bi)

    def layernorm(b, dst_ref, j, r0, nr, best, dep=None, keep=None):
        return score(normalise(b, dst_ref, j, r0, nr, dep, keep)[0], b * TB + r0, best)

    def load_best():
        return best_v[0], best_v[1]

    def store_best(best):
        best_v[0] = best[0]
        best_v[1] = best[1]

    def k_unit(src_ref, j, lo, hi, ties=()):
        pk = _phi(_dot(src_ref[j], _ties(wk_v[:, lo:hi], ties)))
        z_acc[:, lo:hi] += jnp.sum(pk.reshape(TB // 8, 8, hi - lo), axis=0)
        return pk.astype(BF16)

    def raw_slice(i):
        lo, hi = K_SPLITS[i], K_SPLITS[i + 1]
        xs = jnp.concatenate([x_v[0, :, lo:hi], x_v[NB - 1, :, lo:hi]], axis=0)
        part = _dot(xs, wk_v[lo:hi, :D])
        if i == 0:
            kraw_v[...] = part
        else:
            kraw_v[...] += part
        if i == 2:
            cs_v[...] = jnp.sum(wk_v[:hi, :D].astype(F32).reshape(hi // 8, 8, D), axis=0)
        elif i > 2:
            cs_v[...] += jnp.sum(wk_v[lo:hi, :D].astype(F32).reshape((hi - lo) // 8, 8, D), axis=0)

    def raw_last(b, c):
        return _dot(x_v[b, :, KF:], wk_v[KF:, c * KC:(c + 1) * KC])

    def raw_finish(slot, c, part, first):
        cs = slice(c * KC, (c + 1) * KC)
        rows_ = []
        zs = None
        for r0 in range(0, TB, 16):
            mean = jnp.concatenate([st_v[slot, 0, r0:r0 + 16, :]] * (KC // LANES), axis=1)
            rstd = jnp.concatenate([st_v[slot, 1, r0:r0 + 16, :]] * (KC // LANES), axis=1)
            col = jnp.concatenate([cs_v[:, cs]] * 2, axis=0)
            k = (kraw_v[slot * TB + r0:slot * TB + r0 + 16, cs] + part[r0:r0 + 16] - mean * col) * rstd
            pk = _phi(k)
            z2 = pk[:8] + pk[8:]
            zs = z2 if zs is None else zs + z2
            rows_.append(pk.astype(BF16))
        if first:
            z_acc[:, cs] = zs
        else:
            z_acc[:, cs] += zs
        return jnp.concatenate(rows_, axis=0)

    def g_unit(src_ref, j, lo, hi, pk, first=False, ties=()):
        g = _dot_tn(pk, _ties(src_ref[j], ties))
        if first:
            g_acc[lo:hi, :] = g
        else:
            g_acc[lo:hi, :] += g

    def wq_prep(g, kk):
        v = _shuffle_rows(pltpu.bitcast(wq_v[g, kk * 256:(kk + 1) * 256, :].T, U32))
        base = pl.multiple_of(g * 8, 8)
        tot = None
        for i in range(8):
            wqt_v[pl.ds(i * 64 + base, 8), kk * 256:(kk + 1) * 256] = v[i]
            tot = v[i] if tot is None else tot | v[i]
        return pltpu.bitcast(tot[:, :LANES] | tot[:, LANES:], F32)

    def mv_chain(acc, w_ref, c, n0, col_ref, z0, k=D):
        cp = 2 * LANES if (n0 // 256) % 4 < 2 else 0
        cz = c + z0

        def step(i, acc):
            rows = pl.ds(pl.multiple_of(i * 8, 8), 8)
            return acc + w_ref[cz, rows, n0:n0 + LANES].astype(F32) * col_ref[z0, rows, cp:cp + LANES]
        return lax.fori_loop(0, k // 8, step, acc, unroll=True)

    def ffn_gate_up(c, zeros):
        dep = None
        zero = jnp.zeros((8, LANES), F32)
        for n0 in range(0, FC, LANES):
            ga = mv_chain(_after(zero, dep, 1.0), wg_v, c, n0, xcol_v, next(zeros))
            ua = mv_chain(_after(zero, ga, 1.0), wu_v, c, n0, xcol_v, next(zeros))
            dep = ua
            gg = _round_bf16(jnp.sum(ga, axis=0, keepdims=True))
            uu = _round_bf16(jnp.sum(ua, axis=0, keepdims=True))
            h = _round_bf16(_round_bf16(gg * jax.nn.sigmoid(gg)) * uu)
            hc = _col_bcast(h)
            hcol_v[0, n0:n0 + LANES, :LANES] = hc
            hcol_v[0, n0:n0 + LANES, 2 * LANES:3 * LANES] = hc
        return dep

    def ffn_down(c, zeros):
        dep = None
        accs = []
        for n0 in range(0, D, LANES):
            dep = mv_chain(_after(y_acc[:, n0:n0 + LANES], dep), wd_v, c, n0, hcol_v, next(zeros), FC)
            y_acc[:, n0:n0 + LANES] = dep
            accs.append(dep)
        return jnp.concatenate(accs, axis=1)

    def first_half():
        for i in range(4):
            for cp in xs_copies(i):
                cp.wait()
            if i == 3:
                wr_copy.wait()
            wk_copy(i).wait()
            raw_slice(i)
            if i == 3:
                wr_f[...] = jnp.broadcast_to(wr_v[...].astype(F32).reshape(1, D), (8, D))
                dep = None
                for r0 in range(0, TB, 8):
                    _, xn_f = normalise(0, xn_v, 0, r0, 8, dep, keep=0)
                    dep = _delay(xn_f[:, D - LANES:], LN0_PACE)
        for cp in xs_copies(4):
            cp.wait()
        wk_copy(4).wait()
        x_copy(1, 4).wait()
        cs = cs_v[...] + jnp.sum(wk_v[KF:, :D].astype(F32).reshape((D - KF) // 8, 8, D), axis=0)
        cs_v[...] = jnp.broadcast_to(jnp.sum(cs, axis=0, keepdims=True), (8, D))
        best = (jnp.full((8, 1), -jnp.inf, F32), sub8)
        dep = None
        for r0 in range(0, TB, 16):
            dep, best = layernorm(1, xn_v, 1, r0, 16, best, dep)
        store_best(best)
        parts = [raw_last(0, c) for c in range(NKC)]
        for c in range(NKC):
            g_unit(xn_v, 0, c * KC, (c + 1) * KC, raw_finish(0, c, parts[c], True), True,
                   [(dep[:8], 0, 512)] if c == NKC - 1 else [])

        def phase_a(j, carry):
            for i in range(BA - 1):
                x_copy(BA * j + 2 + i, SEM_A + j).wait()
            for i in range(WQ_PER):
                wq_copy(WQ_PER * j + i, SEM_A + j).wait()

            @pl.when(j < NA - 1)
            def _():
                x_copy(BA * j + BA + 1, SEM_A + j).wait()

            preps = [(WQ_PER * j + i, kk) for i in range(WQ_PER) for kk in range(4)]
            k_slots = {(0, 0): [(0, 128), (512, 128)], (0, 1): [(0, 0), (512, 0), (0, 128), (512, 128)],
                       (1, 1): [(0, 0)], (2, 1): [(0, 0)]}
            g_slots = {(t, 3): [(0, 0), (0, 256), (0, 512), (0, 768)] for t in range(BA - 1)}

            def mk_ties(slots):
                return [(wq_prep(*preps.pop(0)), r0, c0) for r0, c0 in slots]

            LR = TB // NKC
            prev = None
            dep = None
            best = load_best()
            win = xn_v.at[pl.ds(BA * j + 1, BA + 1)]
            for t in range(BA):
                for c in range(NKC):
                    pk = k_unit(win, t, c * KC, (c + 1) * KC, ties=mk_ties(k_slots.get((t, c), [])))
                    if prev is not None:
                        g_unit(*prev[1:], ties=mk_ties(g_slots.get(prev[0], [])))
                    prev = ((t, c), win, t, c * KC, (c + 1) * KC, pk)
                    for r0 in range(c * LR, (c + 1) * LR, 8):
                        dep, best = layernorm(BA * j + 2 + t, win, t + 1, r0, 8, best, dep,
                                              keep=1 if t == BA - 1 else None)
            g_unit(*prev[1:], ties=[(dep, 0, 768)])
            assert not preps
            store_best(best)
            return carry

        lax.fori_loop(0, NA, phase_a, 0)

    def second_half():
        wv_copy.wait()
        wo_copy.wait()

        best0 = (jnp.full((8, 1), -jnp.inf, F32), sub8)
        dep = None
        for r0 in range(0, TB, 16):
            dep, best0 = score(xn_v[0, r0:r0 + 16, :], r0, best0, dep)
        bv, bi = load_best()
        first0 = best0[0] >= bv
        bv = jnp.where(first0, best0[0], bv)
        bi = jnp.where(first0, best0[1], bi)
        r_max = jnp.max(bv, axis=0, keepdims=True)
        idx_f = jnp.min(jnp.where(bv == r_max, bi, float(S - 1)))
        idx = jnp.clip(idx_f.astype(jnp.int32), 0, S - 1)
        blk = idx // TB
        hot_pair = blk // 2
        row16 = pl.multiple_of(((idx % TB) // 16) * 16, 16)
        gate_v[...] = jnp.broadcast_to(_round_bf16(jax.nn.sigmoid(r_max)), (16, LANES))
        sel16 = lax.broadcasted_iota(jnp.int32, (16, D), 0) == idx % 16
        xs = xn_v[blk, pl.ds(row16, 16), :].astype(F32)
        xc = _col_bcast(jnp.sum(jnp.where(sel16, xs, 0.0), axis=0, keepdims=True))
        xcol_v[0, :, :LANES] = xc
        xcol_v[0, :, 2 * LANES:3 * LANES] = xc

        rr = lax.broadcasted_iota(jnp.int32, (LANES, LANES), 0) // DH
        cc = lax.broadcasted_iota(jnp.int32, (LANES, LANES), 1) // DH
        same_head = rr == cc

        def g_final(c, pk):
            return (g_acc[c * KC:(c + 1) * KC, :] + _dot_tn(pk, xn_v[NB - 1])).astype(BF16)

        def kv_unit(c, gf):
            out = []
            for gg in range(KC // LANES):
                g = c * (KC // LANES) + gg
                kv = _dot(gf[gg * LANES:(gg + 1) * LANES, :], wv_v[:, g * LANES:(g + 1) * LANES])
                kv = pltpu.bitcast(jnp.where(same_head, kv, 0.0).astype(BF16), U32)
                out.append(pltpu.bitcast(jnp.concatenate(_shuffle_rows(kv), axis=0), BF16))
            return out

        def m_unit(c, kvs, dep=None):
            for gg in range(KC // LANES):
                g = c * (KC // LANES) + gg
                m = _dot(kvs[gg], _tie(wo_v[g * LANES:(g + 1) * LANES, :], dep))
                dep = None
                w = pltpu.bitcast(m.astype(BF16), U32)
                for i in range(8):
                    m_v[i * 64 + g * 8:i * 64 + (g + 1) * 8, :] = w[i * 8:(i + 1) * 8, :]

        def z_prep():
            zc = pltpu.bitcast(_col_bcast(jnp.sum(z_acc[...], axis=0, keepdims=True)).astype(BF16), U32)
            vs = [_shuffle_rows(zc[g * 64:(g + 1) * 64, :]) for g in range(NG)]
            tot = None
            for i in range(NG):
                zt = pltpu.bitcast(jnp.concatenate([vs[g][i] for g in range(NG)], axis=0), BF16)
                zp = zt.astype(F32).T[:8, :]
                zp_v[:, i * LANES:(i + 1) * LANES] = zp
                tot = zp if tot is None else tot + zp
            return tot

        wq0_v[...] = pltpu.bitcast(pltpu.bitcast(wqt_v[:LANES // 2, :], BF16).T, U32)
        parts = [raw_last(NB - 1, c) for c in range(NKC)]

        def gf(c):
            return g_final(c, raw_finish(1, c, parts[c], False))

        gf0 = gf(0)
        gf1 = gf(1)
        kv0 = kv_unit(0, gf0)
        gf2 = gf(2)
        kv1 = kv_unit(1, gf1)
        m_unit(0, kv0)
        gf3 = gf(3)
        kv2 = kv_unit(2, gf2)
        m_unit(1, kv1, xc[D - 8:])
        kv3 = kv_unit(3, gf3)
        m_unit(2, kv2, z_prep())
        m_unit(3, kv3)

        lane = lax.broadcasted_iota(jnp.int32, (8, LANES), 1)
        bit0 = lane % 2 == 0
        bit3 = (lane // 8) % 2 == 0

        def q_part(src_ref, p, ties=(), lead=False):
            wqt = _ties(pltpu.bitcast(wqt_v[...], BF16), ties)
            if lead:
                xn = src_ref[p]
                q0 = _dot(xn, pltpu.bitcast(wq0_v[...], BF16))
                q = jnp.concatenate([q0, _dot_nt(xn, wqt[LANES:])], axis=1)
            else:
                q = _dot_nt(src_ref[p], wqt)
            rows_ = []
            dep = None
            for g in range(TB // 8):
                pq = _phi(q[g * 8:(g + 1) * 8, :])
                t = pq * zp_v[...]
                s_ = t[:, :LANES]
                for n in range(1, NG):
                    s_ = s_ + t[:, n * LANES:(n + 1) * LANES]
                s_ = s_ + jnp.where(bit3, pltpu.roll(s_, LANES - 8, 1), pltpu.roll(s_, 8, 1))
                s_ = s_ + jnp.where(bit0, pltpu.roll(s_, LANES - 1, 1), pltpu.roll(s_, 1, 1))
                rinv = _after(pl.reciprocal(s_ + 1e-6, approx=True), dep)
                rows_.append(pq * jnp.concatenate([rinv] * NG, axis=1))
                dep = _delay(rinv, DEN_PACE)
            return jnp.concatenate(rows_, axis=0).astype(BF16)

        def o_part(o, b, slot, s_out, last, dep=None):
            spans = [(0, 256), (256, 512), (512, 768), (768, 896), (896, D)] if last else \
                [(c * KC, (c + 1) * KC) for c in range(NKC)]
            for lo, hi in spans:
                m = pltpu.bitcast(m_v[:, lo:hi], BF16)
                a = _dot(o, _tie(m, dep if lo == 768 else None))
                for r0, nr in (TAIL if last and hi == D else ((0, TB),)):
                    rs = slice(r0, r0 + nr)
                    res = x_v[b, rs, lo:hi].astype(F32) + xn_v[b, rs, lo:hi].astype(F32)
                    out_v[slot, rs, lo:hi] = (a[rs] + res).astype(BF16)
                    if last or hi == D:
                        cols = pl.ds(lo, hi - lo) if last else pl.ds(0, D)
                        pltpu.make_async_copy(out_v.at[slot, pl.ds(r0, nr), cols],
                                              out_hbm.at[0, pl.ds(b * TB + r0, nr), cols],
                                              sem.at[s_out]).start()

        def phase_b(j, carry):
            for cp in ffn_copies(j, SEM_F + j):
                cp.wait()
            p = jnp.where(j == 0, hot_pair, jnp.where(j == hot_pair, 0, j))
            s_out = jnp.where(j == 0, SEM_O, SEM_O + 1)
            zeros = (lax.shift_right_logical(idx + j + k, 13) for k in range(64))
            gu_dep = ffn_gate_up(j, zeros)
            y = ffn_down(j, zeros)
            o_e = q_part(xn_v, 2 * p, lead=True)
            o_o = q_part(xn_v, 2 * p + 1, [(gu_dep, GU_TILE * LANES, 0)])
            o_part(o_e, 2 * p, 2 * j, s_out, False)
            o_part(o_o, 2 * p + 1, 2 * j + 1, s_out, True, y[:, D - LANES:])
            return carry

        lax.fori_loop(0, NP, phase_b, 0)

        hot = out_v.at[pl.ds(0, 2)]
        pltpu.make_async_copy(hot, hot, sem.at[SEM_O]).wait()
        rows16 = pl.ds(row16, 16)
        yrow = _round_bf16(jnp.sum(y_acc[...], axis=0, keepdims=True))
        upd = jnp.where(sel16, yrow * jnp.concatenate([gate_v[...]] * NG, axis=1), 0.0)
        out_v[blk % 2, rows16, :] = (out_v[blk % 2, rows16, :].astype(F32) + upd).astype(BF16)
        patch = pltpu.make_async_copy(
            out_v.at[blk % 2, rows16, :],
            out_hbm.at[0, pl.ds(pl.multiple_of(blk * TB + row16, 16), 16), :], sem.at[SEM_O])
        patch.start()
        pltpu.make_async_copy(out_v.at[pl.ds(2, NB - 2)], out_v.at[pl.ds(2, NB - 2)],
                              sem.at[SEM_O + 1]).wait()
        patch.wait()

    def outer(i, carry):
        pl.when(i == 0)(first_half)
        pl.when(i == 1)(second_half)
        return carry

    lax.fori_loop(0, 2, outer, 0)


@jax.jit
def pallas_parallel_sum__linear_attn_block__moe_arch_mod__prompt_kernel(
    A_x: jax.Array,
    A_wqkv: jax.Array,
    A_wo: jax.Array,
    B_x: jax.Array,
    B_w_r: jax.Array,
    B_w_gate: jax.Array,
    B_w_up: jax.Array,
    B_w_down: jax.Array,
):
    del B_x
    assert A_x.shape == (1, S, D) and B_w_gate.shape == (D, F)
    any_spec = pl.BlockSpec(memory_space=pl.ANY)
    scratch = [
        pltpu.VMEM((NB, TB, D), BF16),
        pltpu.VMEM((NB, TB, D), BF16),
        pltpu.VMEM((NG, D, LANES), BF16),
        pltpu.VMEM((D, D + LANES), BF16),
        pltpu.VMEM((D, D), BF16),
        pltpu.VMEM((D, D), BF16),
        pltpu.VMEM((NP, D, D), BF16),
        pltpu.VMEM((NP, D, D), BF16),
        pltpu.VMEM((NP, D, D), BF16),
        pltpu.VMEM((2, D, 4 * LANES), F32),
        pltpu.VMEM((2, D, 4 * LANES), F32),
        pltpu.VMEM((D, D), F32),
        pltpu.VMEM((D // 2, D), U32),
        pltpu.VMEM((D // 2, D), U32),
        pltpu.VMEM((NB, TB, D), BF16),
        pltpu.VMEM((D // 2, LANES), U32),
        pltpu.VMEM((2 * TB, D), F32),
        pltpu.VMEM((2, 2, TB, LANES), F32),
        pltpu.VMEM((8, D), F32),
        pltpu.VMEM((8, D), F32),
        pltpu.VMEM((8, D), F32),
        pltpu.VMEM((8, D), F32),
        pltpu.VMEM((8, D), F32),
        pltpu.VMEM((16, LANES), F32),
        pltpu.VMEM((2, 8, 1), F32),
        pltpu.VMEM((8, 1), F32),
        pltpu.VMEM((D,), BF16),
        pltpu.SemaphoreType.DMA((N_SEMS,)),
    ]
    return pl.pallas_call(
        _kernel,
        out_shape=jax.ShapeDtypeStruct((1, S, D), BF16),
        in_specs=[any_spec] * 7,
        out_specs=any_spec,
        scratch_shapes=scratch,
        compiler_params=pltpu.CompilerParams(vmem_limit_bytes=100 * 1024 * 1024,
                                             disable_semaphore_checks=True, disable_bounds_checks=True),
    )(A_x, A_wqkv, A_wo, B_w_r, B_w_gate, B_w_up, B_w_down)
```

```python
import jax
import jax.numpy as jnp
from jax import lax
import jax.experimental.pallas as pl
import jax.experimental.pallas.tpu as pltpu

F32 = jnp.float32
BF16 = jnp.bfloat16
U32 = jnp.uint32

S = 2048
D = 1024
F = 3584
DH = 32
TB = 256
NB = S // TB
NP = NB // 2
FC = F // NP
LANES = 128
NG = D // LANES
KC = 256
NKC = D // KC
NA = 2
BA = (NB - 2) // NA
WQ_PER = NG // NA
K_SPLITS = (0, 128, 256, 512, D)
RAW_BLOCKS = (0, NB - 1) + tuple(BA * j + 1 for j in range(NA))
RAW_PLAN = (
    ((0, 2, 0, 128),),
    ((0, 2, 128, 256), (2, 3, 0, 256), (3, 4, 0, 128)),
    ((3, 4, 128, 256), (0, 2, 256, 512)),
    ((1, 2, 512, 768),),
)
RAW_DEPTH = tuple(max(hi for step in RAW_PLAN for s0, s1, _, hi in step if s0 <= s < s1)
                  for s in range(len(RAW_BLOCKS)))
SCORE0_EARLY = False
LN_PACE = 6
WQ_SLOTS = (
    ('k', 0, 1, 0, 0), ('k', 0, 1, 512, 128), ('g', 0, 0, 0, 0), ('k', 1, 0, 0, 128),
    ('k', 1, 0, 512, 128), ('g', 0, 3, 0, 0), ('k', 1, 1, 0, 0), ('k', 1, 1, 512, 0),
    ('k', 1, 1, 512, 128), ('k', 2, 0, 0, 128), ('k', 2, 0, 512, 128), ('g', 1, 3, 0, 0),
    ('g', 1, 3, 0, 768), ('k', 2, 1, 0, 0), ('k', 2, 1, 512, 0), ('k', 2, 1, 0, 128),
)
DEN_PACE = 8
GU_TILE = 2
TAIL = ((0, 128), (128, 128))
SEM_X = len(K_SPLITS) - 1
SEM_A = SEM_X + 1
SEM_W = SEM_A + NA
SEM_F = SEM_W + 1
SEM_O = SEM_F + NP
N_SEMS = SEM_O + 2


def _round_bf16(v):
    return v.astype(BF16).astype(F32)


def _phi(t):
    return jnp.where(t > 0, t + 1.0, jnp.exp(t)) + 1e-6


def _dot(a, b):
    return jnp.dot(a, b, preferred_element_type=F32)


def _dot_tn(a, b):
    return lax.dot_general(a, b, (((0,), (0,)), ((), ())), preferred_element_type=F32)


def _dot_nt(a, b):
    return lax.dot_general(a, b, (((1,), (1,)), ((), ())), preferred_element_type=F32)


def _after(v, dep, other=0.0):
    if dep is None:
        return v
    return jnp.where(dep > jnp.inf, other, v)


def _tie(w, dep, r0=0, c0=0):
    if dep is None:
        return w
    dep = jnp.broadcast_to(dep, (8, LANES))
    head = pltpu.bitcast(w[r0:r0 + 16, c0:c0 + LANES], U32) | (dep > jnp.inf).astype(U32)
    row = [pltpu.bitcast(head, BF16)]
    if c0:
        row = [w[r0:r0 + 16, :c0]] + row
    if c0 + LANES < w.shape[1]:
        row = row + [w[r0:r0 + 16, c0 + LANES:]]
    head = row[0] if len(row) == 1 else jnp.concatenate(row, axis=1)
    parts = ([w[:r0]] if r0 else []) + [head, w[r0 + 16:]]
    return jnp.concatenate(parts, axis=0)


def _ties(w, ties):
    for dep, r0, c0 in ties:
        w = _tie(w, dep, r0, c0)
    return w


def _shuffle_rows(w):
    sub = lax.broadcasted_iota(jnp.int32, (8, w.shape[1]), 0)
    v = [w[(a % 4) * 16 + (a // 4) * 8:(a % 4) * 16 + (a // 4) * 8 + 8] for a in range(8)]
    for d in (4, 2, 1):
        low = (sub & d) == 0
        nv = list(v)
        for a in range(8):
            if a & d == 0:
                nv[a] = jnp.where(low, v[a], pltpu.roll(v[a + d], d, 0))
                nv[a + d] = jnp.where(low, pltpu.roll(v[a], 8 - d, 0), v[a + d])
        v = nv
    return v


def _delay(v, n):
    for _ in range(n):
        v = pl.reciprocal(v, approx=True)
    return v


def _col_bcast(row):
    tiles = [jnp.broadcast_to(row[:, t * LANES:(t + 1) * LANES], (LANES, LANES)).T
             for t in range(row.shape[1] // LANES)]
    return jnp.concatenate(tiles, axis=0)


def _kernel(x_hbm, wqkv_hbm, wo_hbm, wr_hbm, wg_hbm, wu_hbm, wd_hbm, out_hbm,
            x_v, xn_v, wq_v, wk_v, wv_v, wo_v, wg_v, wu_v, wd_v, xcol_v, hcol_v,
            g_acc, m_v, wqt_v, out_v, wq0_v, kraw_v, st_v, cs_v, wr_f, z_acc, zp_v, y_acc,
            gate_v, best_v, junk_v, wr_v, sem):
    def x_copy(b, s_):
        return pltpu.make_async_copy(x_hbm.at[0, pl.ds(b * TB, TB), :], x_v.at[b], sem.at[s_])

    have = {b: 0 for b in RAW_BLOCKS}
    x_spans = []
    for i in range(len(RAW_PLAN) + 1):
        need = dict(have)
        if i < len(RAW_PLAN):
            for s0, s1, _, hi in RAW_PLAN[i]:
                for b in RAW_BLOCKS[s0:s1]:
                    need[b] = max(need[b], hi)
        complete = {2: (0,), 3: (1,), len(RAW_PLAN): RAW_BLOCKS}.get(i, ())
        need.update({b: D for b in complete})
        x_spans.append([(b, have[b], need[b]) for b in RAW_BLOCKS if need[b] > have[b]])
        have = need

    def xs_copies(i):
        return [pltpu.make_async_copy(x_hbm.at[0, pl.ds(b * TB, TB), pl.ds(lo, hi - lo)],
                                      x_v.at[b, :, pl.ds(lo, hi - lo)], sem.at[i])
                for b, lo, hi in x_spans[i]]

    def wk_copy(i):
        rows = pl.ds(K_SPLITS[i], K_SPLITS[i + 1] - K_SPLITS[i])
        return pltpu.make_async_copy(wqkv_hbm.at[rows, pl.ds(D, D)], wk_v.at[rows, pl.ds(0, D)],
                                     sem.at[i])

    def wq_copy(g, s_):
        cols = pl.ds(pl.multiple_of(g * LANES, LANES), LANES)
        return pltpu.make_async_copy(wqkv_hbm.at[:, cols], wq_v.at[g], sem.at[s_])

    wr_copy = pltpu.make_async_copy(wr_hbm, wr_v, sem.at[2])
    wv_copy = pltpu.make_async_copy(wqkv_hbm.at[:, pl.ds(2 * D, D)], wv_v, sem.at[SEM_W])
    wo_copy = pltpu.make_async_copy(wo_hbm, wo_v, sem.at[SEM_W])

    def ffn_copies(c, s_):
        span = pl.ds(pl.multiple_of(c * FC, LANES), FC)
        return (
            pltpu.make_async_copy(wg_hbm.at[:, span], wg_v.at[c, :, pl.ds(0, FC)], sem.at[s_]),
            pltpu.make_async_copy(wu_hbm.at[:, span], wu_v.at[c, :, pl.ds(0, FC)], sem.at[s_]),
            pltpu.make_async_copy(wd_hbm.at[span, :], wd_v.at[c, pl.ds(0, FC), :], sem.at[s_]),
        )

    for i in range(len(K_SPLITS) - 1):
        for cp in xs_copies(i):
            cp.start()
        if i == 2:
            wr_copy.start()
        wk_copy(i).start()
    for cp in xs_copies(SEM_X):
        cp.start()
    for j in range(NA):
        for b in range(BA * j + 2, BA * (j + 1) + 1):
            x_copy(b, SEM_A + j).start()
        for g in range(WQ_PER * j, WQ_PER * (j + 1)):
            wq_copy(g, SEM_A + j).start()
    wv_copy.start()
    wo_copy.start()
    for c in range(NP):
        for cp in ffn_copies(c, SEM_F + c):
            cp.start()

    y_acc[...] = jnp.zeros_like(y_acc)
    sub8 = lax.broadcasted_iota(jnp.int32, (8, 1), 0).astype(F32)

    def normalise(b, dst_ref, j, r0, nr, dep=None, keep=None):
        rs = pl.ds(r0, nr)
        mean = jnp.mean(x_v[b, rs, :].astype(F32), axis=-1, keepdims=True)
        mean_b = jnp.broadcast_to(_round_bf16(mean), (nr, LANES))
        junk_v[...] = mean[:8]
        c = x_v[b, rs, :].astype(F32) - mean
        var = jnp.mean(c * c, axis=-1, keepdims=True)
        junk_v[...] = var[:8]
        rstd = 1.0 / _round_bf16(jnp.sqrt(_round_bf16(_round_bf16(var) + 1e-5)))
        if keep is not None:
            st_v[keep, 0, rs, :] = mean_b
            st_v[keep, 1, rs, :] = jnp.broadcast_to(rstd, (nr, LANES))
        mean_b = jnp.concatenate([_after(mean_b, dep)] * NG, axis=1)
        xn_f = _round_bf16(x_v[b, rs, :].astype(F32) - mean_b) * rstd
        xn = xn_f.astype(BF16)
        dst_ref[j, rs, :] = xn
        return xn, xn_f

    def score(xn, row0, best, dep=None):
        nr = xn.shape[0]
        wr = wr_f[...]
        if dep is not None:
            wr = jnp.concatenate([_after(wr[:, :LANES], dep[:8]), wr[:, LANES:]], axis=1)
        if nr > 8:
            wr = jnp.concatenate([wr] * (nr // 8), axis=0)
        r = jnp.sum(xn.astype(F32) * wr, axis=-1, keepdims=True)
        rb = _round_bf16(r)
        bv, bi = best
        for q in range(nr // 8):
            rq = rb[q * 8:(q + 1) * 8]
            better = rq > bv
            bv = jnp.where(better, rq, bv)
            bi = jnp.where(better, sub8 + jnp.asarray(row0 + q * 8).astype(F32), bi)
        return r, (bv, bi)

    def layernorm(b, dst_ref, j, r0, nr, best, dep=None, keep=None):
        return score(normalise(b, dst_ref, j, r0, nr, dep, keep)[0], b * TB + r0, best)

    def load_best():
        return best_v[0], best_v[1]

    def store_best(best):
        best_v[0] = best[0]
        best_v[1] = best[1]

    def k_unit(src_ref, j, lo, hi, ties=()):
        pk = _phi(_dot(src_ref[j], _ties(wk_v[:, lo:hi], ties)))
        z_acc[:, lo:hi] += jnp.sum(pk.reshape(TB // 8, 8, hi - lo), axis=0)
        return pk.astype(BF16)

    def raw_unit(s0, s1, lo, hi):
        xs = jnp.concatenate([x_v[b, :, lo:hi] for b in RAW_BLOCKS[s0:s1]], axis=0)
        part = _dot(xs, wk_v[lo:hi, :D]).reshape(s1 - s0, TB, D)
        if lo == 0:
            kraw_v[s0:s1] = part
        else:
            kraw_v[s0:s1] += part

    def col_sums(lo, hi):
        return jnp.sum(wk_v[lo:hi, :D].astype(F32).reshape((hi - lo) // 8, 8, D), axis=0)

    def raw_rest(b, k0, c, ties=()):
        return _dot(x_v[b, :, k0:], _ties(wk_v[k0:, c * KC:(c + 1) * KC], ties))

    def raw_finish(kslot, slot, c, part, first=False):
        cs = slice(c * KC, (c + 1) * KC)
        rows_ = []
        zs = None
        for r0 in range(0, TB, 16):
            mean = jnp.concatenate([st_v[slot, 0, r0:r0 + 16, :]] * (KC // LANES), axis=1)
            rstd = jnp.concatenate([st_v[slot, 1, r0:r0 + 16, :]] * (KC // LANES), axis=1)
            col = jnp.concatenate([cs_v[:, cs]] * 2, axis=0)
            k = (kraw_v[kslot, r0:r0 + 16, cs] + part[r0:r0 + 16] - mean * col) * rstd
            pk = _phi(k)
            z2 = pk[:8] + pk[8:]
            zs = z2 if zs is None else zs + z2
            rows_.append(pk.astype(BF16))
        if first:
            z_acc[:, cs] = zs
        else:
            z_acc[:, cs] += zs
        return jnp.concatenate(rows_, axis=0)

    def g_unit(src_ref, j, lo, hi, pk, first=False, ties=()):
        g = _dot_tn(pk, _ties(src_ref[j], ties))
        if first:
            g_acc[lo:hi, :] = g
        else:
            g_acc[lo:hi, :] += g

    def wq_prep(g, kk):
        v = _shuffle_rows(pltpu.bitcast(wq_v[g, kk * 256:(kk + 1) * 256, :].T, U32))
        base = pl.multiple_of(g * 8, 8)
        tot = None
        for i in range(8):
            wqt_v[pl.ds(i * 64 + base, 8), kk * 256:(kk + 1) * 256] = v[i]
            tot = v[i] if tot is None else tot | v[i]
        return pltpu.bitcast(tot[:, :LANES] | tot[:, LANES:], F32)

    def mv_chain(acc, w_ref, c, n0, col_ref, z0, k=D):
        cp = 2 * LANES if (n0 // 256) % 4 < 2 else 0
        cz = c + z0

        def step(i, acc):
            rows = pl.ds(pl.multiple_of(i * 8, 8), 8)
            return acc + w_ref[cz, rows, n0:n0 + LANES].astype(F32) * col_ref[z0, rows, cp:cp + LANES]
        return lax.fori_loop(0, k // 8, step, acc, unroll=True)

    def ffn_gate_up(c, zeros):
        dep = None
        zero = jnp.zeros((8, LANES), F32)
        for n0 in range(0, FC, LANES):
            ga = mv_chain(_after(zero, dep, 1.0), wg_v, c, n0, xcol_v, next(zeros))
            ua = mv_chain(_after(zero, ga, 1.0), wu_v, c, n0, xcol_v, next(zeros))
            dep = ua
            gg = _round_bf16(jnp.sum(ga, axis=0, keepdims=True))
            uu = _round_bf16(jnp.sum(ua, axis=0, keepdims=True))
            h = _round_bf16(_round_bf16(gg * jax.nn.sigmoid(gg)) * uu)
            hc = _col_bcast(h)
            hcol_v[0, n0:n0 + LANES, :LANES] = hc
            hcol_v[0, n0:n0 + LANES, 2 * LANES:3 * LANES] = hc
        return dep

    def ffn_down(c, zeros):
        dep = None
        accs = []
        for n0 in range(0, D, LANES):
            dep = mv_chain(_after(y_acc[:, n0:n0 + LANES], dep), wd_v, c, n0, hcol_v, next(zeros), FC)
            y_acc[:, n0:n0 + LANES] = dep
            accs.append(dep)
        return jnp.concatenate(accs, axis=1)

    def first_half():
        def paced_normalise(b, best=None):
            dep = None
            for r0 in range(0, TB, 8):
                xn, xn_f = normalise(b, xn_v, b, r0, 8, dep, keep=b)
                dep = _delay(xn_f[:, 3 * LANES:4 * LANES], LN_PACE)
                if best is not None:
                    _, best = score(xn, b * TB + r0, best)
            return best

        best = (jnp.full((8, 1), -jnp.inf, F32), sub8)
        for i in range(len(RAW_PLAN)):
            for cp in xs_copies(i):
                cp.wait()
            if i == 2:
                wr_copy.wait()
            wk_copy(i).wait()
            if i == 1:
                cs_v[...] = col_sums(0, K_SPLITS[2])
            if i == 2:
                wr_f[...] = jnp.broadcast_to(wr_v[...].astype(F32).reshape(1, D), (8, D))
                if SCORE0_EARLY:
                    best = paced_normalise(0, best)
                else:
                    paced_normalise(0)
                store_best(best)
            if i == 3:
                cs = cs_v[...] + col_sums(K_SPLITS[2], D)
                cs_v[...] = jnp.broadcast_to(jnp.sum(cs, axis=0, keepdims=True), (8, D))
                paced_normalise(1)
                parts = [raw_rest(0, RAW_DEPTH[0], c) for c in range(2)]
                for c in range(NKC):
                    g_unit(xn_v, 0, c * KC, (c + 1) * KC, raw_finish(0, 0, c, parts[c], True), True)
                    if len(parts) < NKC:
                        parts.append(raw_rest(0, RAW_DEPTH[0], len(parts)))
            for unit in RAW_PLAN[i]:
                raw_unit(*unit)
        for cp in xs_copies(SEM_X):
            cp.wait()

        def phase_a(j, carry):
            for i in range(BA - 1):
                x_copy(BA * j + 2 + i, SEM_A + j).wait()
            for i in range(WQ_PER):
                wq_copy(WQ_PER * j + i, SEM_A + j).wait()
            preps = [(WQ_PER * j + i, kk) for i in range(WQ_PER) for kk in range(4)]
            k_slots, g_slots = {}, {}
            for kind, t_, c_, r_, q_ in WQ_SLOTS:
                (k_slots if kind == 'k' else g_slots).setdefault((t_, c_), []).append((r_, q_))

            def mk_ties(slots):
                return [(wq_prep(*preps.pop(0)), r0, c0) for r0, c0 in slots]

            LR = TB // NKC
            prev = None
            dep = None
            best = load_best()
            win = xn_v.at[pl.ds(BA * j + 1, BA + 1)]
            for t in range(BA):
                for c in range(NKC):
                    ties = mk_ties(k_slots.get((t, c), []))
                    if t == 0:
                        pk = raw_finish(2 + j, 1, c, raw_rest(BA * j + 1, RAW_DEPTH[2], c, ties))
                    else:
                        pk = k_unit(win, t, c * KC, (c + 1) * KC, ties)
                    if prev is not None:
                        g_unit(*prev[1:], ties=mk_ties(g_slots.get(prev[0], [])))
                    prev = ((t, c), win, t, c * KC, (c + 1) * KC, pk)
                    for r0 in range(c * LR, (c + 1) * LR, 8):
                        dep, best = layernorm(BA * j + 2 + t, win, t + 1, r0, 8, best, dep,
                                              keep=1 if t == BA - 1 else None)
            g_unit(*prev[1:], ties=[(dep, 0, 768)])
            assert not preps
            store_best(best)
            return carry

        lax.fori_loop(0, NA, phase_a, 0)

    def second_half():
        wv_copy.wait()
        wo_copy.wait()

        best0 = (jnp.full((8, 1), -jnp.inf, F32), sub8)
        dep = None
        for b0 in ((1,) if SCORE0_EARLY else (0, 1)):
            for r0 in range(0, TB, 16):
                dep, best0 = score(xn_v[b0, r0:r0 + 16, :], b0 * TB + r0, best0, dep)
        bv, bi = load_best()
        first0 = (best0[0] > bv) | ((best0[0] == bv) & (best0[1] < bi))
        bv = jnp.where(first0, best0[0], bv)
        bi = jnp.where(first0, best0[1], bi)
        r_max = jnp.max(bv, axis=0, keepdims=True)
        idx_f = jnp.min(jnp.where(bv == r_max, bi, float(S - 1)))
        idx = jnp.clip(idx_f.astype(jnp.int32), 0, S - 1)
        blk = idx // TB
        hot_pair = blk // 2
        row16 = pl.multiple_of(((idx % TB) // 16) * 16, 16)
        gate_v[...] = jnp.broadcast_to(_round_bf16(jax.nn.sigmoid(r_max)), (16, LANES))
        sel16 = lax.broadcasted_iota(jnp.int32, (16, D), 0) == idx % 16
        xs = xn_v[blk, pl.ds(row16, 16), :].astype(F32)
        xc = _col_bcast(jnp.sum(jnp.where(sel16, xs, 0.0), axis=0, keepdims=True))
        xcol_v[0, :, :LANES] = xc
        xcol_v[0, :, 2 * LANES:3 * LANES] = xc

        rr = lax.broadcasted_iota(jnp.int32, (LANES, LANES), 0) // DH
        cc = lax.broadcasted_iota(jnp.int32, (LANES, LANES), 1) // DH
        same_head = rr == cc

        def g_final(c, pk):
            return (g_acc[c * KC:(c + 1) * KC, :] + _dot_tn(pk, xn_v[NB - 1])).astype(BF16)

        def kv_unit(c, gf):
            out = []
            for gg in range(KC // LANES):
                g = c * (KC // LANES) + gg
                kv = _dot(gf[gg * LANES:(gg + 1) * LANES, :], wv_v[:, g * LANES:(g + 1) * LANES])
                kv = pltpu.bitcast(jnp.where(same_head, kv, 0.0).astype(BF16), U32)
                out.append(pltpu.bitcast(jnp.concatenate(_shuffle_rows(kv), axis=0), BF16))
            return out

        def m_unit(c, kvs, dep=None):
            for gg in range(KC // LANES):
                g = c * (KC // LANES) + gg
                m = _dot(kvs[gg], _tie(wo_v[g * LANES:(g + 1) * LANES, :], dep))
                dep = None
                w = pltpu.bitcast(m.astype(BF16), U32)
                for i in range(8):
                    m_v[i * 64 + g * 8:i * 64 + (g + 1) * 8, :] = w[i * 8:(i + 1) * 8, :]

        def z_prep():
            zc = pltpu.bitcast(_col_bcast(jnp.sum(z_acc[...], axis=0, keepdims=True)).astype(BF16), U32)
            vs = [_shuffle_rows(zc[g * 64:(g + 1) * 64, :]) for g in range(NG)]
            tot = None
            for i in range(NG):
                zt = pltpu.bitcast(jnp.concatenate([vs[g][i] for g in range(NG)], axis=0), BF16)
                zp = zt.astype(F32).T[:8, :]
                zp_v[:, i * LANES:(i + 1) * LANES] = zp
                tot = zp if tot is None else tot + zp
            return tot

        wq0_v[...] = pltpu.bitcast(pltpu.bitcast(wqt_v[:LANES // 2, :], BF16).T, U32)
        parts = [raw_rest(NB - 1, RAW_DEPTH[1], c) for c in range(NKC)]

        def gf(c):
            return g_final(c, raw_finish(1, 1, c, parts[c]))

        gf0 = gf(0)
        gf1 = gf(1)
        kv0 = kv_unit(0, gf0)
        gf2 = gf(2)
        kv1 = kv_unit(1, gf1)
        m_unit(0, kv0)
        gf3 = gf(3)
        kv2 = kv_unit(2, gf2)
        m_unit(1, kv1, xc[D - 8:])
        kv3 = kv_unit(3, gf3)
        m_unit(2, kv2, z_prep())
        m_unit(3, kv3)

        lane = lax.broadcasted_iota(jnp.int32, (8, LANES), 1)
        bit0 = lane % 2 == 0
        bit3 = (lane // 8) % 2 == 0

        def q_part(src_ref, p, ties=(), lead=False):
            wqt = _ties(pltpu.bitcast(wqt_v[...], BF16), ties)
            if lead:
                xn = src_ref[p]
                q0 = _dot(xn, pltpu.bitcast(wq0_v[...], BF16))
                q = jnp.concatenate([q0, _dot_nt(xn, wqt[LANES:])], axis=1)
            else:
                q = _dot_nt(src_ref[p], wqt)
            rows_ = []
            dep = None
            for g in range(TB // 8):
                pq = _phi(q[g * 8:(g + 1) * 8, :])
                t = pq * zp_v[...]
                s_ = t[:, :LANES]
                for n in range(1, NG):
                    s_ = s_ + t[:, n * LANES:(n + 1) * LANES]
                s_ = s_ + jnp.where(bit3, pltpu.roll(s_, LANES - 8, 1), pltpu.roll(s_, 8, 1))
                s_ = s_ + jnp.where(bit0, pltpu.roll(s_, LANES - 1, 1), pltpu.roll(s_, 1, 1))
                rinv = _after(pl.reciprocal(s_ + 1e-6, approx=True), dep)
                rows_.append(pq * jnp.concatenate([rinv] * NG, axis=1))
                dep = _delay(rinv, DEN_PACE)
            return jnp.concatenate(rows_, axis=0).astype(BF16)

        def o_part(o, b, slot, s_out, last, dep=None):
            spans = [(0, 256), (256, 512), (512, 768), (768, 896), (896, D)] if last else \
                [(c * KC, (c + 1) * KC) for c in range(NKC)]
            for lo, hi in spans:
                m = pltpu.bitcast(m_v[:, lo:hi], BF16)
                a = _dot(o, _tie(m, dep if lo == 768 else None))
                for r0, nr in (TAIL if last and hi == D else ((0, TB),)):
                    rs = slice(r0, r0 + nr)
                    res = x_v[b, rs, lo:hi].astype(F32) + xn_v[b, rs, lo:hi].astype(F32)
                    out_v[slot, rs, lo:hi] = (a[rs] + res).astype(BF16)
                    if last or hi == D:
                        cols = pl.ds(lo, hi - lo) if last else pl.ds(0, D)
                        pltpu.make_async_copy(out_v.at[slot, pl.ds(r0, nr), cols],
                                              out_hbm.at[0, pl.ds(b * TB + r0, nr), cols],
                                              sem.at[s_out]).start()

        def phase_b(j, carry):
            for cp in ffn_copies(j, SEM_F + j):
                cp.wait()
            p = jnp.where(j == 0, hot_pair, jnp.where(j == hot_pair, 0, j))
            s_out = jnp.where(j == 0, SEM_O, SEM_O + 1)
            zeros = (lax.shift_right_logical(idx + j + k, 13) for k in range(64))
            gu_dep = ffn_gate_up(j, zeros)
            y = ffn_down(j, zeros)
            o_e = q_part(xn_v, 2 * p, lead=True)
            o_o = q_part(xn_v, 2 * p + 1, [(gu_dep, GU_TILE * LANES, 0)])
            o_part(o_e, 2 * p, 2 * j, s_out, False)
            o_part(o_o, 2 * p + 1, 2 * j + 1, s_out, True, y[:, D - LANES:])
            return carry

        lax.fori_loop(0, NP, phase_b, 0)

        hot = out_v.at[pl.ds(0, 2)]
        pltpu.make_async_copy(hot, hot, sem.at[SEM_O]).wait()
        rows16 = pl.ds(row16, 16)
        yrow = _round_bf16(jnp.sum(y_acc[...], axis=0, keepdims=True))
        upd = jnp.where(sel16, yrow * jnp.concatenate([gate_v[...]] * NG, axis=1), 0.0)
        out_v[blk % 2, rows16, :] = (out_v[blk % 2, rows16, :].astype(F32) + upd).astype(BF16)
        patch = pltpu.make_async_copy(
            out_v.at[blk % 2, rows16, :],
            out_hbm.at[0, pl.ds(pl.multiple_of(blk * TB + row16, 16), 16), :], sem.at[SEM_O])
        patch.start()
        pltpu.make_async_copy(out_v.at[pl.ds(2, NB - 2)], out_v.at[pl.ds(2, NB - 2)],
                              sem.at[SEM_O + 1]).wait()
        patch.wait()

    def outer(i, carry):
        pl.when(i == 0)(first_half)
        pl.when(i == 1)(second_half)
        return carry

    lax.fori_loop(0, 2, outer, 0)


@jax.jit
def pallas_parallel_sum__linear_attn_block__moe_arch_mod__prompt_kernel(
    A_x: jax.Array,
    A_wqkv: jax.Array,
    A_wo: jax.Array,
    B_x: jax.Array,
    B_w_r: jax.Array,
    B_w_gate: jax.Array,
    B_w_up: jax.Array,
    B_w_down: jax.Array,
):
    del B_x
    assert A_x.shape == (1, S, D) and B_w_gate.shape == (D, F)
    any_spec = pl.BlockSpec(memory_space=pl.ANY)
    scratch = [
        pltpu.VMEM((NB, TB, D), BF16),
        pltpu.VMEM((NB, TB, D), BF16),
        pltpu.VMEM((NG, D, LANES), BF16),
        pltpu.VMEM((D, D + LANES), BF16),
        pltpu.VMEM((D, D), BF16),
        pltpu.VMEM((D, D), BF16),
        pltpu.VMEM((NP, D, D), BF16),
        pltpu.VMEM((NP, D, D), BF16),
        pltpu.VMEM((NP, D, D), BF16),
        pltpu.VMEM((2, D, 4 * LANES), F32),
        pltpu.VMEM((2, D, 4 * LANES), F32),
        pltpu.VMEM((D, D), F32),
        pltpu.VMEM((D // 2, D), U32),
        pltpu.VMEM((D // 2, D), U32),
        pltpu.VMEM((NB, TB, D), BF16),
        pltpu.VMEM((D // 2, LANES), U32),
        pltpu.VMEM((len(RAW_BLOCKS), TB, D), F32),
        pltpu.VMEM((2, 2, TB, LANES), F32),
        pltpu.VMEM((8, D), F32),
        pltpu.VMEM((8, D), F32),
        pltpu.VMEM((8, D), F32),
        pltpu.VMEM((8, D), F32),
        pltpu.VMEM((8, D), F32),
        pltpu.VMEM((16, LANES), F32),
        pltpu.VMEM((2, 8, 1), F32),
        pltpu.VMEM((8, 1), F32),
        pltpu.VMEM((D,), BF16),
        pltpu.SemaphoreType.DMA((N_SEMS,)),
    ]
    return pl.pallas_call(
        _kernel,
        out_shape=jax.ShapeDtypeStruct((1, S, D), BF16),
        in_specs=[any_spec] * 7,
        out_specs=any_spec,
        scratch_shapes=scratch,
        compiler_params=pltpu.CompilerParams(vmem_limit_bytes=100 * 1024 * 1024,
                                             disable_semaphore_checks=True, disable_bounds_checks=True),
    )(A_x, A_wqkv, A_wo, B_w_r, B_w_gate, B_w_up, B_w_down)
```

```python
import jax
import jax.numpy as jnp
from jax import lax
import jax.experimental.pallas as pl
import jax.experimental.pallas.tpu as pltpu

F32 = jnp.float32
BF16 = jnp.bfloat16
U32 = jnp.uint32

S = 2048
D = 1024
F = 3584
DH = 32
TB = 256
NB = S // TB
NP = NB // 2
FC = F // NP
LANES = 128
NG = D // LANES
KC = 256
NKC = D // KC
NA = 2
BA = (NB - 2) // NA
WQ_PER = NG // NA
K_SPLITS = (0, 128, 256, 512, D)
RAW_BLOCKS = (0, NB - 1) + tuple(BA * j + 1 for j in range(NA))
RAW_PLAN = (
    ((0, 2, 0, 128),),
    ((0, 2, 128, 256), (2, 3, 0, 256), (3, 4, 0, 128)),
    ((3, 4, 128, 256), (0, 2, 256, 512)),
    ((1, 2, 512, 768),),
)
RAW_DEPTH = tuple(max(hi for step in RAW_PLAN for s0, s1, _, hi in step if s0 <= s < s1)
                  for s in range(len(RAW_BLOCKS)))
LN_PACE = 6
WQ_SLOTS = (
    ('k', 0, 1, 0, 0), ('k', 0, 1, 512, 128), ('g', 0, 0, 0, 0), ('k', 1, 0, 0, 128),
    ('k', 1, 0, 512, 128), ('g', 0, 3, 0, 0), ('k', 1, 1, 0, 0), ('k', 1, 1, 512, 0),
    ('k', 1, 1, 512, 128), ('k', 2, 0, 0, 128), ('k', 2, 0, 512, 128), ('g', 1, 3, 0, 0),
    ('g', 1, 3, 0, 768), ('k', 2, 1, 0, 0), ('k', 2, 1, 512, 0), ('k', 2, 1, 0, 128),
)
DEN_PACE = 8
GU_TILE = 2
TAIL = ((0, 128), (128, 128))
SEM_X = len(K_SPLITS) - 1
SEM_A = SEM_X + 1
SEM_W = SEM_A + NA
SEM_F = SEM_W + 1
SEM_O = SEM_F + NP
N_SEMS = SEM_O + 2


def _round_bf16(v):
    return v.astype(BF16).astype(F32)


def _phi(t):
    return jnp.where(t > 0, t + 1.0, jnp.exp(t)) + 1e-6


def _dot(a, b):
    return jnp.dot(a, b, preferred_element_type=F32)


def _dot_tn(a, b):
    return lax.dot_general(a, b, (((0,), (0,)), ((), ())), preferred_element_type=F32)


def _dot_nt(a, b):
    return lax.dot_general(a, b, (((1,), (1,)), ((), ())), preferred_element_type=F32)


def _after(v, dep, other=0.0):
    if dep is None:
        return v
    return jnp.where(dep > jnp.inf, other, v)


def _tie(w, dep, r0=0, c0=0):
    if dep is None:
        return w
    dep = jnp.broadcast_to(dep, (8, LANES))
    head = pltpu.bitcast(w[r0:r0 + 16, c0:c0 + LANES], U32) | (dep > jnp.inf).astype(U32)
    row = [pltpu.bitcast(head, BF16)]
    if c0:
        row = [w[r0:r0 + 16, :c0]] + row
    if c0 + LANES < w.shape[1]:
        row = row + [w[r0:r0 + 16, c0 + LANES:]]
    head = row[0] if len(row) == 1 else jnp.concatenate(row, axis=1)
    parts = ([w[:r0]] if r0 else []) + [head, w[r0 + 16:]]
    return jnp.concatenate(parts, axis=0)


def _ties(w, ties):
    for dep, r0, c0 in ties:
        w = _tie(w, dep, r0, c0)
    return w


def _shuffle_rows(w):
    sub = lax.broadcasted_iota(jnp.int32, (8, w.shape[1]), 0)
    v = [w[(a % 4) * 16 + (a // 4) * 8:(a % 4) * 16 + (a // 4) * 8 + 8] for a in range(8)]
    for d in (4, 2, 1):
        low = (sub & d) == 0
        nv = list(v)
        for a in range(8):
            if a & d == 0:
                nv[a] = jnp.where(low, v[a], pltpu.roll(v[a + d], d, 0))
                nv[a + d] = jnp.where(low, pltpu.roll(v[a], 8 - d, 0), v[a + d])
        v = nv
    return v


def _delay(v, n):
    for _ in range(n):
        v = pl.reciprocal(v, approx=True)
    return v


def _col_bcast(row):
    tiles = [jnp.broadcast_to(row[:, t * LANES:(t + 1) * LANES], (LANES, LANES)).T
             for t in range(row.shape[1] // LANES)]
    return jnp.concatenate(tiles, axis=0)


def _kernel(x_hbm, wqkv_hbm, wo_hbm, wr_hbm, wg_hbm, wu_hbm, wd_hbm, out_hbm,
            x_v, xn_v, wq_v, wk_v, wv_v, wo_v, wg_v, wu_v, wd_v, xcol_v, hcol_v,
            g_acc, m_v, wqt_v, out_v, wq0_v, kraw_v, st_v, cs_v, wr_f, z_acc, zp_v, y_acc,
            gate_v, best_v, junk_v, wr_v, sem):
    def x_copy(b, s_):
        return pltpu.make_async_copy(x_hbm.at[0, pl.ds(b * TB, TB), :], x_v.at[b], sem.at[s_])

    have = {b: 0 for b in RAW_BLOCKS}
    x_spans = []
    for i in range(len(RAW_PLAN) + 1):
        need = dict(have)
        if i < len(RAW_PLAN):
            for s0, s1, _, hi in RAW_PLAN[i]:
                for b in RAW_BLOCKS[s0:s1]:
                    need[b] = max(need[b], hi)
        complete = {2: (0,), 3: (1,), len(RAW_PLAN): RAW_BLOCKS}.get(i, ())
        need.update({b: D for b in complete})
        x_spans.append([(b, have[b], need[b]) for b in RAW_BLOCKS if need[b] > have[b]])
        have = need

    def xs_copies(i):
        return [pltpu.make_async_copy(x_hbm.at[0, pl.ds(b * TB, TB), pl.ds(lo, hi - lo)],
                                      x_v.at[b, :, pl.ds(lo, hi - lo)], sem.at[i])
                for b, lo, hi in x_spans[i]]

    def wk_copy(i):
        rows = pl.ds(K_SPLITS[i], K_SPLITS[i + 1] - K_SPLITS[i])
        return pltpu.make_async_copy(wqkv_hbm.at[rows, pl.ds(D, D)], wk_v.at[rows, pl.ds(0, D)],
                                     sem.at[i])

    def wq_copy(g, s_):
        cols = pl.ds(pl.multiple_of(g * LANES, LANES), LANES)
        return pltpu.make_async_copy(wqkv_hbm.at[:, cols], wq_v.at[g], sem.at[s_])

    wr_copy = pltpu.make_async_copy(wr_hbm, wr_v, sem.at[2])
    wv_copy = pltpu.make_async_copy(wqkv_hbm.at[:, pl.ds(2 * D, D)], wv_v, sem.at[SEM_W])
    wo_copy = pltpu.make_async_copy(wo_hbm, wo_v, sem.at[SEM_W])

    def ffn_copies(c, s_):
        span = pl.ds(pl.multiple_of(c * FC, LANES), FC)
        return (
            pltpu.make_async_copy(wg_hbm.at[:, span], wg_v.at[c, :, pl.ds(0, FC)], sem.at[s_]),
            pltpu.make_async_copy(wu_hbm.at[:, span], wu_v.at[c, :, pl.ds(0, FC)], sem.at[s_]),
            pltpu.make_async_copy(wd_hbm.at[span, :], wd_v.at[c, pl.ds(0, FC), :], sem.at[s_]),
        )

    for i in range(len(K_SPLITS) - 1):
        for cp in xs_copies(i):
            cp.start()
        if i == 2:
            wr_copy.start()
        wk_copy(i).start()
    for cp in xs_copies(SEM_X):
        cp.start()
    for j in range(NA):
        for b in range(BA * j + 2, BA * (j + 1) + 1):
            x_copy(b, SEM_A + j).start()
        for g in range(WQ_PER * j, WQ_PER * (j + 1)):
            wq_copy(g, SEM_A + j).start()
    wv_copy.start()
    wo_copy.start()
    for c in range(NP):
        for cp in ffn_copies(c, SEM_F + c):
            cp.start()

    y_acc[...] = jnp.zeros_like(y_acc)
    sub8 = lax.broadcasted_iota(jnp.int32, (8, 1), 0).astype(F32)

    def normalise(b, dst_ref, j, r0, nr, dep=None, keep=None):
        rs = pl.ds(r0, nr)
        mean = jnp.mean(x_v[b, rs, :].astype(F32), axis=-1, keepdims=True)
        mean_b = jnp.broadcast_to(_round_bf16(mean), (nr, LANES))
        junk_v[...] = mean[:8]
        c = x_v[b, rs, :].astype(F32) - mean
        var = jnp.mean(c * c, axis=-1, keepdims=True)
        junk_v[...] = var[:8]
        rstd = 1.0 / _round_bf16(jnp.sqrt(_round_bf16(_round_bf16(var) + 1e-5)))
        if keep is not None:
            st_v[keep, 0, rs, :] = mean_b
            st_v[keep, 1, rs, :] = jnp.broadcast_to(rstd, (nr, LANES))
        mean_b = jnp.concatenate([_after(mean_b, dep)] * NG, axis=1)
        xn_f = _round_bf16(x_v[b, rs, :].astype(F32) - mean_b) * rstd
        xn = xn_f.astype(BF16)
        dst_ref[j, rs, :] = xn
        return xn, xn_f

    def score(xn, row0, best, dep=None):
        nr = xn.shape[0]
        wr = wr_f[...]
        if dep is not None:
            wr = jnp.concatenate([_after(wr[:, :LANES], dep[:8]), wr[:, LANES:]], axis=1)
        if nr > 8:
            wr = jnp.concatenate([wr] * (nr // 8), axis=0)
        r = jnp.sum(xn.astype(F32) * wr, axis=-1, keepdims=True)
        rb = _round_bf16(r)
        bv, bi = best
        for q in range(nr // 8):
            rq = rb[q * 8:(q + 1) * 8]
            better = rq > bv
            bv = jnp.where(better, rq, bv)
            bi = jnp.where(better, sub8 + jnp.asarray(row0 + q * 8).astype(F32), bi)
        return r, (bv, bi)

    def layernorm(b, dst_ref, j, r0, nr, best, dep=None, keep=None):
        return score(normalise(b, dst_ref, j, r0, nr, dep, keep)[0], b * TB + r0, best)

    def load_best():
        return best_v[0], best_v[1]

    def store_best(best):
        best_v[0] = best[0]
        best_v[1] = best[1]

    def k_unit(src_ref, j, lo, hi, ties=()):
        pk = _phi(_dot(src_ref[j], _ties(wk_v[:, lo:hi], ties)))
        z_acc[:, lo:hi] += jnp.sum(pk.reshape(TB // 8, 8, hi - lo), axis=0)
        return pk.astype(BF16)

    def raw_unit(s0, s1, lo, hi):
        xs = jnp.concatenate([x_v[b, :, lo:hi] for b in RAW_BLOCKS[s0:s1]], axis=0)
        part = _dot(xs, wk_v[lo:hi, :D]).reshape(s1 - s0, TB, D)
        if lo == 0:
            kraw_v[s0:s1] = part
        else:
            kraw_v[s0:s1] += part

    def col_sums(lo, hi):
        return jnp.sum(wk_v[lo:hi, :D].astype(F32).reshape((hi - lo) // 8, 8, D), axis=0)

    def raw_rest(b, k0, c, ties=()):
        return _dot(x_v[b, :, k0:], _ties(wk_v[k0:, c * KC:(c + 1) * KC], ties))

    def raw_finish(kslot, slot, c, part, first=False):
        cs = slice(c * KC, (c + 1) * KC)
        rows_ = []
        zs = None
        for r0 in range(0, TB, 16):
            mean = jnp.concatenate([st_v[slot, 0, r0:r0 + 16, :]] * (KC // LANES), axis=1)
            rstd = jnp.concatenate([st_v[slot, 1, r0:r0 + 16, :]] * (KC // LANES), axis=1)
            col = jnp.concatenate([cs_v[:, cs]] * 2, axis=0)
            k = (kraw_v[kslot, r0:r0 + 16, cs] + part[r0:r0 + 16] - mean * col) * rstd
            pk = _phi(k)
            z2 = pk[:8] + pk[8:]
            zs = z2 if zs is None else zs + z2
            rows_.append(pk.astype(BF16))
        if first:
            z_acc[:, cs] = zs
        else:
            z_acc[:, cs] += zs
        return jnp.concatenate(rows_, axis=0)

    def g_unit(src_ref, j, lo, hi, pk, first=False, ties=()):
        g = _dot_tn(pk, _ties(src_ref[j], ties))
        if first:
            g_acc[lo:hi, :] = g
        else:
            g_acc[lo:hi, :] += g

    def wq_prep(g, kk):
        v = _shuffle_rows(pltpu.bitcast(wq_v[g, kk * 256:(kk + 1) * 256, :].T, U32))
        base = pl.multiple_of(g * 8, 8)
        tot = None
        for i in range(8):
            wqt_v[pl.ds(i * 64 + base, 8), kk * 256:(kk + 1) * 256] = v[i]
            tot = v[i] if tot is None else tot | v[i]
        return pltpu.bitcast(tot[:, :LANES] | tot[:, LANES:], F32)

    def mv_chain(acc, w_ref, c, n0, col_ref, z0, k=D):
        cp = 2 * LANES if (n0 // 256) % 4 < 2 else 0
        cz = c + z0

        def step(i, acc):
            rows = pl.ds(pl.multiple_of(i * 8, 8), 8)
            return acc + w_ref[cz, rows, n0:n0 + LANES].astype(F32) * col_ref[z0, rows, cp:cp + LANES]
        return lax.fori_loop(0, k // 8, step, acc, unroll=True)

    def ffn_gate_up(c, zeros):
        dep = None
        zero = jnp.zeros((8, LANES), F32)
        for n0 in range(0, FC, LANES):
            ga = mv_chain(_after(zero, dep, 1.0), wg_v, c, n0, xcol_v, next(zeros))
            ua = mv_chain(_after(zero, ga, 1.0), wu_v, c, n0, xcol_v, next(zeros))
            dep = ua
            gg = _round_bf16(jnp.sum(ga, axis=0, keepdims=True))
            uu = _round_bf16(jnp.sum(ua, axis=0, keepdims=True))
            h = _round_bf16(_round_bf16(gg * jax.nn.sigmoid(gg)) * uu)
            hc = _col_bcast(h)
            hcol_v[0, n0:n0 + LANES, :LANES] = hc
            hcol_v[0, n0:n0 + LANES, 2 * LANES:3 * LANES] = hc
        return dep

    def ffn_down(c, zeros):
        dep = None
        accs = []
        for n0 in range(0, D, LANES):
            dep = mv_chain(_after(y_acc[:, n0:n0 + LANES], dep), wd_v, c, n0, hcol_v, next(zeros), FC)
            y_acc[:, n0:n0 + LANES] = dep
            accs.append(dep)
        return jnp.concatenate(accs, axis=1)

    def first_half():
        def paced_normalise(b):
            dep = None
            for r0 in range(0, TB, 8):
                _, xn_f = normalise(b, xn_v, b, r0, 8, dep, keep=b)
                dep = _delay(xn_f[:, 3 * LANES:4 * LANES], LN_PACE)

        for i in range(len(RAW_PLAN)):
            for cp in xs_copies(i):
                cp.wait()
            if i == 2:
                wr_copy.wait()
            wk_copy(i).wait()
            if i == 1:
                cs_v[...] = col_sums(0, K_SPLITS[2])
            if i == 2:
                wr_f[...] = jnp.broadcast_to(wr_v[...].astype(F32).reshape(1, D), (8, D))
                paced_normalise(0)
                store_best((jnp.full((8, 1), -jnp.inf, F32), sub8))
            if i == 3:
                cs = cs_v[...] + col_sums(K_SPLITS[2], D)
                cs_v[...] = jnp.broadcast_to(jnp.sum(cs, axis=0, keepdims=True), (8, D))
                paced_normalise(1)
                parts = [raw_rest(0, RAW_DEPTH[0], c) for c in range(2)]
                for c in range(NKC):
                    g_unit(xn_v, 0, c * KC, (c + 1) * KC, raw_finish(0, 0, c, parts[c], True), True)
                    if len(parts) < NKC:
                        parts.append(raw_rest(0, RAW_DEPTH[0], len(parts)))
            for unit in RAW_PLAN[i]:
                raw_unit(*unit)
        for cp in xs_copies(SEM_X):
            cp.wait()

        def phase_a(j, carry):
            for i in range(BA - 1):
                x_copy(BA * j + 2 + i, SEM_A + j).wait()
            for i in range(WQ_PER):
                wq_copy(WQ_PER * j + i, SEM_A + j).wait()
            preps = [(WQ_PER * j + i, kk) for i in range(WQ_PER) for kk in range(4)]
            k_slots, g_slots = {}, {}
            for kind, t_, c_, r_, q_ in WQ_SLOTS:
                (k_slots if kind == 'k' else g_slots).setdefault((t_, c_), []).append((r_, q_))

            def mk_ties(slots):
                return [(wq_prep(*preps.pop(0)), r0, c0) for r0, c0 in slots]

            LR = TB // NKC
            prev = None
            dep = None
            best = load_best()
            win = xn_v.at[pl.ds(BA * j + 1, BA + 1)]
            for t in range(BA):
                for c in range(NKC):
                    ties = mk_ties(k_slots.get((t, c), []))
                    if t == 0:
                        pk = raw_finish(2 + j, 1, c, raw_rest(BA * j + 1, RAW_DEPTH[2], c, ties))
                    else:
                        pk = k_unit(win, t, c * KC, (c + 1) * KC, ties)
                    if prev is not None:
                        g_unit(*prev[1:], ties=mk_ties(g_slots.get(prev[0], [])))
                    prev = ((t, c), win, t, c * KC, (c + 1) * KC, pk)
                    for r0 in range(c * LR, (c + 1) * LR, 8):
                        dep, best = layernorm(BA * j + 2 + t, win, t + 1, r0, 8, best, dep,
                                              keep=1 if t == BA - 1 else None)
            g_unit(*prev[1:], ties=[(dep, 0, 768)])
            assert not preps
            store_best(best)
            return carry

        lax.fori_loop(0, NA, phase_a, 0)

    def second_half():
        wv_copy.wait()
        wo_copy.wait()

        best0 = (jnp.full((8, 1), -jnp.inf, F32), sub8)
        dep = None
        for b0 in range(2):
            for r0 in range(0, TB, 16):
                dep, best0 = score(xn_v[b0, r0:r0 + 16, :], b0 * TB + r0, best0, dep)
        bv, bi = load_best()
        first0 = (best0[0] > bv) | ((best0[0] == bv) & (best0[1] < bi))
        bv = jnp.where(first0, best0[0], bv)
        bi = jnp.where(first0, best0[1], bi)
        r_max = jnp.max(bv, axis=0, keepdims=True)
        idx_f = jnp.min(jnp.where(bv == r_max, bi, float(S - 1)))
        idx = jnp.clip(idx_f.astype(jnp.int32), 0, S - 1)
        blk = idx // TB
        hot_pair = blk // 2
        row16 = pl.multiple_of(((idx % TB) // 16) * 16, 16)
        gate_v[...] = jnp.broadcast_to(_round_bf16(jax.nn.sigmoid(r_max)), (16, LANES))
        sel16 = lax.broadcasted_iota(jnp.int32, (16, D), 0) == idx % 16
        xs = xn_v[blk, pl.ds(row16, 16), :].astype(F32)
        xc = _col_bcast(jnp.sum(jnp.where(sel16, xs, 0.0), axis=0, keepdims=True))
        xcol_v[0, :, :LANES] = xc
        xcol_v[0, :, 2 * LANES:3 * LANES] = xc

        rr = lax.broadcasted_iota(jnp.int32, (LANES, LANES), 0) // DH
        cc = lax.broadcasted_iota(jnp.int32, (LANES, LANES), 1) // DH
        same_head = rr == cc

        def g_final(c, pk):
            return (g_acc[c * KC:(c + 1) * KC, :] + _dot_tn(pk, xn_v[NB - 1])).astype(BF16)

        def kv_unit(c, gf):
            out = []
            for gg in range(KC // LANES):
                g = c * (KC // LANES) + gg
                kv = _dot(gf[gg * LANES:(gg + 1) * LANES, :], wv_v[:, g * LANES:(g + 1) * LANES])
                kv = pltpu.bitcast(jnp.where(same_head, kv, 0.0).astype(BF16), U32)
                out.append(pltpu.bitcast(jnp.concatenate(_shuffle_rows(kv), axis=0), BF16))
            return out

        def m_unit(c, kvs, dep=None):
            for gg in range(KC // LANES):
                g = c * (KC // LANES) + gg
                m = _dot(kvs[gg], _tie(wo_v[g * LANES:(g + 1) * LANES, :], dep))
                dep = None
                w = pltpu.bitcast(m.astype(BF16), U32)
                for i in range(8):
                    m_v[i * 64 + g * 8:i * 64 + (g + 1) * 8, :] = w[i * 8:(i + 1) * 8, :]

        def z_prep():
            zc = pltpu.bitcast(_col_bcast(jnp.sum(z_acc[...], axis=0, keepdims=True)).astype(BF16), U32)
            vs = [_shuffle_rows(zc[g * 64:(g + 1) * 64, :]) for g in range(NG)]
            tot = None
            for i in range(NG):
                zt = pltpu.bitcast(jnp.concatenate([vs[g][i] for g in range(NG)], axis=0), BF16)
                zp = zt.astype(F32).T[:8, :]
                zp_v[:, i * LANES:(i + 1) * LANES] = zp
                tot = zp if tot is None else tot + zp
            return tot

        wq0_v[...] = pltpu.bitcast(pltpu.bitcast(wqt_v[:LANES // 2, :], BF16).T, U32)
        parts = [raw_rest(NB - 1, RAW_DEPTH[1], c) for c in range(NKC)]

        def gf(c):
            return g_final(c, raw_finish(1, 1, c, parts[c]))

        gf0 = gf(0)
        gf1 = gf(1)
        kv0 = kv_unit(0, gf0)
        gf2 = gf(2)
        kv1 = kv_unit(1, gf1)
        m_unit(0, kv0)
        gf3 = gf(3)
        kv2 = kv_unit(2, gf2)
        m_unit(1, kv1)
        kv3 = kv_unit(3, gf3)
        m_unit(2, kv2, z_prep())
        m_unit(3, kv3, xc[D - 8:])

        lane = lax.broadcasted_iota(jnp.int32, (8, LANES), 1)
        bit0 = lane % 2 == 0
        bit3 = (lane // 8) % 2 == 0

        def q_part(src_ref, p, ties=(), lead=False):
            wqt = _ties(pltpu.bitcast(wqt_v[...], BF16), ties)
            if lead:
                xn = src_ref[p]
                q0 = _dot(xn, pltpu.bitcast(wq0_v[...], BF16))
                q = jnp.concatenate([q0, _dot_nt(xn, wqt[LANES:])], axis=1)
            else:
                q = _dot_nt(src_ref[p], wqt)
            rows_ = []
            dep = None
            for g in range(TB // 8):
                pq = _phi(q[g * 8:(g + 1) * 8, :])
                t = pq * zp_v[...]
                s_ = t[:, :LANES]
                for n in range(1, NG):
                    s_ = s_ + t[:, n * LANES:(n + 1) * LANES]
                s_ = s_ + jnp.where(bit3, pltpu.roll(s_, LANES - 8, 1), pltpu.roll(s_, 8, 1))
                s_ = s_ + jnp.where(bit0, pltpu.roll(s_, LANES - 1, 1), pltpu.roll(s_, 1, 1))
                rinv = _after(1.0 / (s_ + 1e-6), dep)
                rows_.append(pq * jnp.concatenate([rinv] * NG, axis=1))
                dep = _delay(rinv, DEN_PACE)
            return jnp.concatenate(rows_, axis=0).astype(BF16)

        def o_part(o, b, slot, s_out, last, dep=None):
            spans = [(0, 256), (256, 512), (512, 768), (768, 896), (896, D)] if last else \
                [(c * KC, (c + 1) * KC) for c in range(NKC)]
            for lo, hi in spans:
                m = pltpu.bitcast(m_v[:, lo:hi], BF16)
                a = _dot(o, _tie(m, dep if lo == 768 else None))
                for r0, nr in (TAIL if last and hi == D else ((0, TB),)):
                    rs = slice(r0, r0 + nr)
                    res = x_v[b, rs, lo:hi].astype(F32) + xn_v[b, rs, lo:hi].astype(F32)
                    out_v[slot, rs, lo:hi] = (a[rs] + res).astype(BF16)
                    if last or hi == D:
                        cols = pl.ds(lo, hi - lo) if last else pl.ds(0, D)
                        pltpu.make_async_copy(out_v.at[slot, pl.ds(r0, nr), cols],
                                              out_hbm.at[0, pl.ds(b * TB + r0, nr), cols],
                                              sem.at[s_out]).start()

        def phase_b(j, carry):
            for cp in ffn_copies(j, SEM_F + j):
                cp.wait()
            p = jnp.where(j == 0, hot_pair, jnp.where(j == hot_pair, 0, j))
            s_out = jnp.where(j == 0, SEM_O, SEM_O + 1)
            zeros = (lax.shift_right_logical(idx + j + k, 13) for k in range(64))
            gu_dep = ffn_gate_up(j, zeros)
            y = ffn_down(j, zeros)
            o_e = q_part(xn_v, 2 * p, lead=True)
            o_o = q_part(xn_v, 2 * p + 1, [(gu_dep, GU_TILE * LANES, 0)])
            o_part(o_e, 2 * p, 2 * j, s_out, False)
            o_part(o_o, 2 * p + 1, 2 * j + 1, s_out, True, y[:, D - LANES:])
            return carry

        lax.fori_loop(0, NP, phase_b, 0)

        hot = out_v.at[pl.ds(0, 2)]
        pltpu.make_async_copy(hot, hot, sem.at[SEM_O]).wait()
        rows16 = pl.ds(row16, 16)
        yrow = _round_bf16(jnp.sum(y_acc[...], axis=0, keepdims=True))
        upd = jnp.where(sel16, yrow * jnp.concatenate([gate_v[...]] * NG, axis=1), 0.0)
        out_v[blk % 2, rows16, :] = (out_v[blk % 2, rows16, :].astype(F32) + upd).astype(BF16)
        patch = pltpu.make_async_copy(
            out_v.at[blk % 2, rows16, :],
            out_hbm.at[0, pl.ds(pl.multiple_of(blk * TB + row16, 16), 16), :], sem.at[SEM_O])
        patch.start()
        pltpu.make_async_copy(out_v.at[pl.ds(2, NB - 2)], out_v.at[pl.ds(2, NB - 2)],
                              sem.at[SEM_O + 1]).wait()
        patch.wait()

    def outer(i, carry):
        pl.when(i == 0)(first_half)
        pl.when(i == 1)(second_half)
        return carry

    lax.fori_loop(0, 2, outer, 0)


@jax.jit
def pallas_parallel_sum__linear_attn_block__moe_arch_mod__prompt_kernel(
    A_x: jax.Array,
    A_wqkv: jax.Array,
    A_wo: jax.Array,
    B_x: jax.Array,
    B_w_r: jax.Array,
    B_w_gate: jax.Array,
    B_w_up: jax.Array,
    B_w_down: jax.Array,
):
    del B_x
    assert A_x.shape == (1, S, D) and B_w_gate.shape == (D, F)
    any_spec = pl.BlockSpec(memory_space=pl.ANY)
    scratch = [
        pltpu.VMEM((NB, TB, D), BF16),
        pltpu.VMEM((NB, TB, D), BF16),
        pltpu.VMEM((NG, D, LANES), BF16),
        pltpu.VMEM((D, D + LANES), BF16),
        pltpu.VMEM((D, D), BF16),
        pltpu.VMEM((D, D), BF16),
        pltpu.VMEM((NP, D, D), BF16),
        pltpu.VMEM((NP, D, D), BF16),
        pltpu.VMEM((NP, D, D), BF16),
        pltpu.VMEM((2, D, 4 * LANES), F32),
        pltpu.VMEM((2, D, 4 * LANES), F32),
        pltpu.VMEM((D, D), F32),
        pltpu.VMEM((D // 2, D), U32),
        pltpu.VMEM((D // 2, D), U32),
        pltpu.VMEM((NB, TB, D), BF16),
        pltpu.VMEM((D // 2, LANES), U32),
        pltpu.VMEM((len(RAW_BLOCKS), TB, D), F32),
        pltpu.VMEM((2, 2, TB, LANES), F32),
        pltpu.VMEM((8, D), F32),
        pltpu.VMEM((8, D), F32),
        pltpu.VMEM((8, D), F32),
        pltpu.VMEM((8, D), F32),
        pltpu.VMEM((8, D), F32),
        pltpu.VMEM((16, LANES), F32),
        pltpu.VMEM((2, 8, 1), F32),
        pltpu.VMEM((8, 1), F32),
        pltpu.VMEM((D,), BF16),
        pltpu.SemaphoreType.DMA((N_SEMS,)),
    ]
    return pl.pallas_call(
        _kernel,
        out_shape=jax.ShapeDtypeStruct((1, S, D), BF16),
        in_specs=[any_spec] * 7,
        out_specs=any_spec,
        scratch_shapes=scratch,
        compiler_params=pltpu.CompilerParams(vmem_limit_bytes=100 * 1024 * 1024,
                                             disable_semaphore_checks=True, disable_bounds_checks=True),
    )(A_x, A_wqkv, A_wo, B_w_r, B_w_gate, B_w_up, B_w_down)
```
